```python
import jax
import jax.numpy as jnp

def _softmax(x, axis=-1):
    return jax.nn.softmax(x, axis=axis)
def _gelu(x):
    return jax.nn.gelu(x, approximate=True)
def _silu(x):
    return jax.nn.silu(x)
def _sigmoid(x):
    return jax.nn.sigmoid(x)
def _layernorm(x, axis=-1, eps=1e-5):
    m = jnp.mean(x, axis=axis, keepdims=True)
    v = jnp.var(x, axis=axis, keepdims=True)
    return (x - m) / jnp.sqrt(v + eps)
def _scatter_add(tgt, idx, src, axis=0):
    return tgt.at[idx].add(src)
def _segment_sum(src, seg, n):
    return jax.ops.segment_sum(src, seg, n)
class _Rng:
    def __init__(self, key):
        self._k = key
    def _next(self):
        self._k, sub = jax.random.split(self._k)
        return sub
    def normal(self, shape):
        return jax.random.normal(self._next(), shape, dtype=jnp.bfloat16)
    def randint(self, lo, hi, shape):
        return jax.random.randint(self._next(), shape, lo, hi, dtype=jnp.int32)
    def uniform(self, shape, lo=0.0, hi=1.0):
        return jax.random.uniform(self._next(), shape, jnp.bfloat16, lo, hi)
    def permutation(self, n):
        return jax.random.permutation(self._next(), n)


kernel_name = 'sequential_preLN__compressed_kv_cla__moe_arch_mod__prompt'

def setup_inputs():
    _rng = _Rng(jax.random.key(int.from_bytes(__import__("os").urandom(4), "little")))
    _w = (lambda a: (lambda t: t.astype(jnp.bfloat16) if jnp.issubdtype(t.dtype, jnp.floating) else t)(jnp.asarray(a)))
    def _A_setup():
        B, H, Sq, Sk, D, M = 1, 32, 2048, 2048, 128, 1024
        Dc = 4 * D
        return {
            "x": _w((lambda *s: _rng.normal(s) * 0.05)(B, Sq, M)),
            "c_kv": _w((lambda *s: _rng.normal(s) * 0.05)(B, Sk, Dc)),
            "w_q": _w((lambda *s: _rng.normal(s) * 0.05)(M, H, D) * (M ** -0.5)),
            "w_uk": _w((lambda *s: _rng.normal(s) * 0.05)(Dc, H, D) * (Dc ** -0.5)),
            "w_uv": _w((lambda *s: _rng.normal(s) * 0.05)(Dc, H, D) * (Dc ** -0.5)),
            "w_o": _w((lambda *s: _rng.normal(s) * 0.05)(H, D, M) * ((H * D) ** -0.5)),
        }
    _A_in = _A_setup()

    def _B_setup():
        B, S, D, F, C = 1, 2048, 1024, 3584, 2
        return {
            "x": _w((lambda *s: _rng.normal(s) * 0.05)(B, S, D)),
            "w_r": _w((lambda *s: _rng.normal(s) * 0.05)(D)),
            "w_gate": _w((lambda *s: _rng.normal(s) * 0.05)(D, F)),
            "w_up": _w((lambda *s: _rng.normal(s) * 0.05)(D, F)),
            "w_down": _w((lambda *s: _rng.normal(s) * 0.05)(F, D)),
        }
    _B_in = _B_setup()

    return {
        "A_x": _A_in["x"],
        "A_c_kv": _A_in["c_kv"],
        "A_w_q": _A_in["w_q"],
        "A_w_uk": _A_in["w_uk"],
        "A_w_uv": _A_in["w_uv"],
        "A_w_o": _A_in["w_o"],
        "B_x": _B_in["x"],
        "B_w_r": _B_in["w_r"],
        "B_w_gate": _B_in["w_gate"],
        "B_w_up": _B_in["w_up"],
        "B_w_down": _B_in["w_down"],
    }

def reference(A_x, A_c_kv, A_w_q, A_w_uk, A_w_uv, A_w_o, B_x, B_w_r, B_w_gate, B_w_up, B_w_down):
    def _A_ref(x, c_kv, w_q, w_uk, w_uv, w_o):
        B, Sq, M = x.shape[0], x.shape[1], x.shape[2]
        Sk = c_kv.shape[1]
        H, D = w_q.shape[1], w_q.shape[2]
        q = jnp.einsum("bqm,mhd->bhqd", x, w_q)
        k = jnp.einsum("bkc,chd->bhkd", c_kv, w_uk)
        v = jnp.einsum("bkc,chd->bhkd", c_kv, w_uv)
        scores = jnp.einsum("bhqd,bhkd->bhqk", q, k) * (D ** -0.5)
        off = Sk - Sq
        qi = jnp.arange(Sq)[:, None]
        kj = jnp.arange(Sk)[None, :]
        cmask = kj <= (qi + off)
        scores = jnp.where(cmask[None, None], scores, -1e9)
        p = _softmax(scores, axis=-1)
        ctx = jnp.einsum("bhqk,bhkd->bhqd", p, v)
        return jnp.einsum("bhqd,hdm->bqm", ctx, w_o)

    def _B_ref(x, w_r, w_gate, w_up, w_down):
        B, S, D = x.shape
        C = 2
        r = x @ w_r
        idx = jnp.argsort(-r, axis=-1)[:, :C]
        idx_e = jnp.repeat(idx.reshape(B, C, 1), D, axis=2)
        x_sel = jnp.take_along_axis(x, idx_e, axis=1)
        g = _silu(x_sel @ w_gate)
        u = x_sel @ w_up
        y = (g * u) @ w_down
        r_sel = _sigmoid(jnp.take_along_axis(r, idx, axis=1))
        y = y * r_sel.reshape(B, C, 1)
        b_off = (jnp.arange(B) * S).reshape(B, 1)
        flat_idx = (idx + b_off).reshape(B * C)
        zero = (x * 0.0).reshape(B * S, D)
        upd = _scatter_add(zero, flat_idx, y.reshape(B * C, D), axis=0)
        return x + upd.reshape(B, S, D)

    x = A_x
    h = x + _A_ref(_layernorm(x, axis=-1), A_c_kv, A_w_q, A_w_uk, A_w_uv, A_w_o)
    h2 = h + _B_ref(_layernorm(h, axis=-1), B_w_r, B_w_gate, B_w_up, B_w_down)
    return h2
```

```python
import jax
import jax.numpy as jnp
from jax import lax
import jax.experimental.pallas as pl
import jax.experimental.pallas.tpu as pltpu

bf16 = jnp.bfloat16
f32 = jnp.float32
u32 = jnp.uint32

T = 128
TQ = 256
HPS = 2
GRP = 8
RB = 256
EPS = 1e-5
NEG = -1e30
LOG2E = 1.4426950408889634
NT = (((1,), (1,)), ((), ()))


def _rnd(x):
    return x.astype(bf16).astype(f32)


def _recip(l):
    r = pl.reciprocal(l, approx=True)
    return r * (2.0 - l * r)


def _make_kernel(S, M, C, H, D, F):
    n_steps = H // HPS
    n_grp = H // GRP
    steps_per_grp = GRP // HPS
    pairs_per_grp = GRP // 2
    nb = S // TQ
    ns = TQ // T
    n_rb = S // RB
    scale = (D ** -0.5) * LOG2E

    def kernel(x_hbm, ckv_hbm, wq_hbm, wk_hbm, wv_hbm, wo_hbm, wr_ref, wg_hbm, wu_hbm, wd_hbm,
               out_hbm,
               x_s, xn_s, ckv_s, wq_raw, wk_raw, wv_raw, uq, uk, uv, k_s, v_s, ctx_s,
               wo_s, wg_s, wu_s, wd_s, attn_s, h_s, hn_s, r_s, out_s,
               sem_in, sem_w, sem_big, sem_out, sem_fix):
        step = pl.program_id(0)

        def w_copies(g):
            return [
                pltpu.make_async_copy(wk_hbm.at[:, pl.ds(g * GRP, GRP), :], wk_raw.at[g], sem_w.at[3 * g]),
                pltpu.make_async_copy(wq_hbm.at[:, pl.ds(g * GRP, GRP), :], wq_raw.at[g], sem_w.at[3 * g + 1]),
                pltpu.make_async_copy(wv_hbm.at[:, pl.ds(g * GRP, GRP), :], wv_raw.at[g], sem_w.at[3 * g + 2]),
            ]

        def big_copies():
            return [
                pltpu.make_async_copy(wo_hbm, wo_s, sem_big.at[0]),
                pltpu.make_async_copy(wg_hbm, wg_s, sem_big.at[1]),
                pltpu.make_async_copy(wu_hbm, wu_s, sem_big.at[2]),
                pltpu.make_async_copy(wd_hbm, wd_s, sem_big.at[3]),
            ]

        @pl.when(step == 0)
        def _():
            cx = pltpu.make_async_copy(x_hbm, x_s, sem_in.at[0])
            cc = pltpu.make_async_copy(ckv_hbm, ckv_s, sem_in.at[1])
            cx.start()
            cc.start()
            for c in w_copies(0):
                c.start()
            cx.wait()

            def ln_body(i, carry):
                r0 = pl.multiple_of(i * 128, 128)
                xf = x_s[pl.ds(r0, 128), :].astype(f32)
                mu = jnp.sum(xf, axis=1, keepdims=True) * (1.0 / M)
                d = xf - mu
                var = jnp.sum(d * d, axis=1, keepdims=True) * (1.0 / M)
                xn_s[pl.ds(r0, 128), :] = (d * lax.rsqrt(var + EPS)).astype(bf16)
                return carry

            lax.fori_loop(0, S // 128, ln_body, 0)
            cc.wait()

        @pl.when(step == 1)
        def _():
            for g in range(1, n_grp):
                for c in w_copies(g):
                    c.start()
            for c in big_copies():
                c.start()

        for g in range(n_grp):
            @pl.when(step == g * steps_per_grp)
            def _(g=g):
                for c in w_copies(g):
                    c.wait()
                uk[...] = pltpu.bitcast(wk_raw[g].reshape(C * GRP, D), u32)
                uq[...] = pltpu.bitcast(wq_raw[g].reshape(M * GRP, D), u32)
                uv[...] = pltpu.bitcast(wv_raw[g].reshape(C * GRP, D), u32)

        pair = step % steps_per_grp

        def unpack_pair(u_ref, rows):
            w = u_ref[pl.ds(pair, rows, stride=pairs_per_grp), :]
            lo = pltpu.bitcast(w << 16, f32).astype(bf16)
            hi = pltpu.bitcast(w & jnp.uint32(0xFFFF0000), f32).astype(bf16)
            return lo, hi

        wk2 = unpack_pair(uk, C)
        wq2 = unpack_pair(uq, M)
        wv2 = unpack_pair(uv, C)

        row = lax.broadcasted_iota(jnp.int32, (T, T), 0)
        col = lax.broadcasted_iota(jnp.int32, (T, T), 1)
        tri = col <= row

        def kproj(hh):
            k_s[hh] = jnp.dot(ckv_s[...], wk2[hh], preferred_element_type=f32).astype(bf16)

        def vproj(hh):
            v_s[hh] = jnp.dot(ckv_s[...], wv2[hh], preferred_element_type=f32).astype(bf16)

        def qk(hh, i):
            L0 = i * TQ
            qf = jnp.dot(xn_s[L0:L0 + TQ, :], wq2[hh], preferred_element_type=f32) * scale
            ss = [lax.dot_general(qf.astype(bf16), k_s[hh, 0:L0 + T, :], NT, preferred_element_type=f32)]
            for j in range(1, ns):
                ss.append(lax.dot_general(qf[j * T:].astype(bf16), k_s[hh, L0 + j * T:L0 + (j + 1) * T, :], NT,
                                          preferred_element_type=f32))
            return ss

        def softmax_pv(hh, i, ss):
            L0 = i * TQ
            p_parts = [[] for _ in range(ns)]
            rl = []
            for r in range(ns):
                pieces = [ss[0][r * T:(r + 1) * T, :]] + [ss[j][(r - j) * T:(r - j + 1) * T, :] for j in range(1, r + 1)]
                last = pieces[-1]
                if r == 0 and L0 > 0:
                    last = jnp.concatenate([last[:, :L0], jnp.where(tri, last[:, L0:], NEG)], axis=1)
                else:
                    last = jnp.where(tri, last, NEG)
                pieces[-1] = last
                s = jnp.concatenate(pieces, axis=1) if len(pieces) > 1 else pieces[0]
                m = jnp.max(s, axis=1, keepdims=True)
                p = jnp.exp2(s - m)
                rl.append(_recip(jnp.sum(p, axis=1, keepdims=True)))
                p_parts[0].append(p[:, :L0 + T])
                for j in range(1, r + 1):
                    p_parts[j].append(p[:, L0 + j * T:L0 + (j + 1) * T])
            o0 = jnp.dot(jnp.concatenate(p_parts[0], axis=0).astype(bf16), v_s[hh, 0:L0 + T, :],
                         preferred_element_type=f32)
            os_ = [o0[r * T:(r + 1) * T] for r in range(ns)]
            for j in range(1, ns):
                oj = jnp.dot(jnp.concatenate(p_parts[j], axis=0).astype(bf16),
                             v_s[hh, L0 + j * T:L0 + (j + 1) * T, :], preferred_element_type=f32)
                for r in range(j, ns):
                    os_[r] = os_[r] + oj[(r - j) * T:(r - j + 1) * T]
            for r in range(ns):
                ctx_s[step, L0 + r * T:L0 + (r + 1) * T, hh * D:(hh + 1) * D] = (os_[r] * rl[r]).astype(bf16)

        order = [(hh, i) for hh in range(HPS) for i in range(nb - 1, -1, -1)]
        kproj(0)
        s_cur = qk(*order[0])
        vproj(0)
        for n, (hh, i) in enumerate(order):
            s_next = None
            if n + 1 < len(order):
                nh, ni = order[n + 1]
                if nh != hh:
                    kproj(nh)
                s_next = qk(nh, ni)
                if nh != hh:
                    vproj(nh)
            softmax_pv(hh, i, s_cur)
            s_cur = s_next

        @pl.when(step == n_steps - 1)
        def _():
            bc = big_copies()
            bc[0].wait()
            wr8 = jnp.broadcast_to(wr_ref[...], (8, M))

            def out_copy(b):
                r0 = pl.multiple_of(b * RB, RB)
                return pltpu.make_async_copy(out_s.at[pl.ds(r0, RB), :], out_hbm.at[pl.ds(r0, RB), :], sem_out.at[b])

            def oproj(b):
                r0 = pl.multiple_of(b * RB, RB)
                lhs = jnp.concatenate([ctx_s[j, pl.ds(r0, RB), :] for j in range(n_steps)], axis=1)
                attn_s[pl.ds(r0, RB), :] = jnp.dot(lhs, wo_s[...], preferred_element_type=f32).astype(bf16)

            def post(b):
                r0 = pl.multiple_of(b * RB, RB)
                h = (x_s[pl.ds(r0, RB), :].astype(f32) + attn_s[pl.ds(r0, RB), :].astype(f32)).astype(bf16)
                hf = h.astype(f32)
                mu = jnp.sum(hf, axis=1, keepdims=True) * (1.0 / M)
                dc = hf - mu
                var = jnp.sum(dc * dc, axis=1, keepdims=True) * (1.0 / M)
                den = _rnd(jnp.sqrt(_rnd(_rnd(var) + _rnd(jnp.full((1, 1), EPS, f32)))))
                hn = (_rnd(hf - _rnd(mu)) / den).astype(bf16)
                h_s[pl.ds(r0, RB), :] = h
                hn_s[pl.ds(r0, RB), :] = hn
                out_s[pl.ds(r0, RB), :] = (hf + hn.astype(f32)).astype(bf16)
                r_s[b] = _rnd(lax.dot_general(wr8, hn, NT, preferred_element_type=f32))
                out_copy(b).start()

            oproj(0)

            def body(b, carry):
                post(b - 1)
                oproj(b)
                return carry

            lax.fori_loop(1, n_rb, body, 0)
            post(n_rb - 1)

            r_all = jnp.concatenate([r_s[b] for b in range(n_rb)], axis=1)
            pos = lax.broadcasted_iota(jnp.int32, (8, S), 1)
            m1 = jnp.max(r_all)
            i1 = jnp.min(jnp.where(r_all == m1, pos, S))
            i1 = jnp.minimum(i1, S - 1)
            rest = jnp.where(pos == i1, -jnp.inf, r_all)
            m2 = jnp.max(rest)
            i2 = jnp.min(jnp.where((rest == m2) & (pos != i1), pos, S))
            i2 = jnp.minimum(i2, S - 1)

            g1 = pl.multiple_of((i1 // 16) * 16, 16)
            g2 = pl.multiple_of((i2 // 16) * 16, 16)
            xs = jnp.concatenate([hn_s[pl.ds(g1, 16), :].astype(f32), hn_s[pl.ds(g2, 16), :].astype(f32)], axis=0)
            hs = jnp.concatenate([h_s[pl.ds(g1, 16), :].astype(f32), h_s[pl.ds(g2, 16), :].astype(f32)], axis=0)
            bc[1].wait()
            bc[2].wait()
            bc[3].wait()
            xb = xs.astype(bf16)
            g = _rnd(jnp.dot(xb, wg_s[...], preferred_element_type=f32))
            u = _rnd(jnp.dot(xb, wu_s[...], preferred_element_type=f32))
            gu = (_rnd(g * jax.nn.sigmoid(g)) * u).astype(bf16)
            y = _rnd(jnp.dot(gu, wd_s[...], preferred_element_type=f32))
            rid = lax.broadcasted_iota(jnp.int32, (32, 1), 0)
            tok = jnp.where(rid < 16, g1 + rid, g2 + rid - 16)
            rsel = jnp.where(tok == i1, m1, m2)
            upd = jnp.where((tok == i1) | (tok == i2), _rnd(y * _rnd(jax.nn.sigmoid(rsel))), 0.0)
            fixed = (hs + _rnd(xs + upd)).astype(bf16)

            for b in range(n_rb):
                out_copy(b).wait()
            out_s[pl.ds(g1, 16), :] = fixed[0:16]
            out_s[pl.ds(g2, 16), :] = fixed[16:32]
            c1 = pltpu.make_async_copy(out_s.at[pl.ds(g1, 16), :], out_hbm.at[pl.ds(g1, 16), :], sem_fix.at[0])
            c2 = pltpu.make_async_copy(out_s.at[pl.ds(g2, 16), :], out_hbm.at[pl.ds(g2, 16), :], sem_fix.at[1])
            c1.start()

            @pl.when(g1 != g2)
            def _():
                c2.start()
                c2.wait()

            c1.wait()

    scratch = [
        pltpu.VMEM((S, M), bf16),
        pltpu.VMEM((S, M), bf16),
        pltpu.VMEM((S, C), bf16),
        pltpu.VMEM((n_grp, M, GRP, D), bf16),
        pltpu.VMEM((n_grp, C, GRP, D), bf16),
        pltpu.VMEM((n_grp, C, GRP, D), bf16),
        pltpu.VMEM((M * GRP // 2, D), u32),
        pltpu.VMEM((C * GRP // 2, D), u32),
        pltpu.VMEM((C * GRP // 2, D), u32),
        pltpu.VMEM((HPS, S, D), bf16),
        pltpu.VMEM((HPS, S, D), bf16),
        pltpu.VMEM((n_steps, S, HPS * D), bf16),
        pltpu.VMEM((H * D, M), bf16),
        pltpu.VMEM((M, F), bf16),
        pltpu.VMEM((M, F), bf16),
        pltpu.VMEM((F, M), bf16),
        pltpu.VMEM((S, M), bf16),
        pltpu.VMEM((S, M), bf16),
        pltpu.VMEM((S, M), bf16),
        pltpu.VMEM((n_rb, 8, RB), f32),
        pltpu.VMEM((S, M), bf16),
        pltpu.SemaphoreType.DMA((2,)),
        pltpu.SemaphoreType.DMA((3 * n_grp,)),
        pltpu.SemaphoreType.DMA((4,)),
        pltpu.SemaphoreType.DMA((n_rb,)),
        pltpu.SemaphoreType.DMA((2,)),
    ]
    return kernel, scratch, n_steps


@jax.jit
def pallas_sequential_preLN__compressed_kv_cla__moe_arch_mod__prompt_kernel(
    A_x: jax.Array,
    A_c_kv: jax.Array,
    A_w_q: jax.Array,
    A_w_uk: jax.Array,
    A_w_uv: jax.Array,
    A_w_o: jax.Array,
    B_x: jax.Array,
    B_w_r: jax.Array,
    B_w_gate: jax.Array,
    B_w_up: jax.Array,
    B_w_down: jax.Array,
):
    B, S, M = A_x.shape
    C = A_c_kv.shape[2]
    H, D = A_w_q.shape[1], A_w_q.shape[2]
    F = B_w_gate.shape[1]
    assert B == 1 and A_c_kv.shape[1] == S

    kernel, scratch, n_steps = _make_kernel(S, M, C, H, D, F)
    any_spec = pl.BlockSpec(memory_space=pl.ANY)
    out = pl.pallas_call(
        kernel,
        grid=(n_steps,),
        in_specs=[any_spec] * 6 + [pl.BlockSpec((1, M), lambda i: (0, 0))] + [any_spec] * 3,
        out_specs=any_spec,
        out_shape=jax.ShapeDtypeStruct((S, M), A_x.dtype),
        scratch_shapes=scratch,
        compiler_params=pltpu.CompilerParams(
            dimension_semantics=("arbitrary",),
            vmem_limit_bytes=120 * 1024 * 1024,
        ),
        name="mla_mod_block",
    )(
        A_x.reshape(S, M), A_c_kv.reshape(S, C), A_w_q, A_w_uk, A_w_uv,
        A_w_o.reshape(H * D, M), B_w_r.reshape(1, M), B_w_gate, B_w_up, B_w_down,
    )
    return out.reshape(B, S, M)
```

```python
import jax
import jax.numpy as jnp
from jax import lax
import jax.experimental.pallas as pl
import jax.experimental.pallas.tpu as pltpu

bf16 = jnp.bfloat16
f32 = jnp.float32
u32 = jnp.uint32

T = 128
TQ = 256
HPS = 1
GRP = 8
RB = 256
XC = 512
EPS = 1e-5
NEG = -1e30
LOG2E = 1.4426950408889634
NT = (((1,), (1,)), ((), ()))


def _rnd(x):
    return x.astype(bf16).astype(f32)


def _recip(l):
    r = pl.reciprocal(l, approx=True)
    return r * (2.0 - l * r)


def _make_kernel(S, M, C, H, D, F):
    n_steps = H // HPS
    n_grp = H // GRP
    steps_per_grp = GRP // HPS
    pairs_per_grp = GRP // 2
    nb = S // TQ
    ns = TQ // T
    n_rb = S // RB
    n_xc = S // XC
    scale = (D ** -0.5) * LOG2E

    def kernel(x_hbm, ckv_hbm, wq_hbm, wk_hbm, wv_hbm, wo_hbm, wr_ref, wg_hbm, wu_hbm, wd_hbm,
               out_hbm,
               x_s, xn_s, ckv_s, wq_raw, wk_raw, wv_raw, uq, uk, uv, k_s, v_s, ctx_s,
               wo_s, wg_s, wu_s, wd_s, attn_s, h_s, hn_s, r_s, out_s,
               sem_in, sem_x, sem_w, sem_big, sem_out, sem_fix):
        def w_copies(g):
            return [
                pltpu.make_async_copy(wk_hbm.at[:, pl.ds(g * GRP, GRP), :], wk_raw.at[g], sem_w.at[3 * g]),
                pltpu.make_async_copy(wq_hbm.at[:, pl.ds(g * GRP, GRP), :], wq_raw.at[g], sem_w.at[3 * g + 1]),
                pltpu.make_async_copy(wv_hbm.at[:, pl.ds(g * GRP, GRP), :], wv_raw.at[g], sem_w.at[3 * g + 2]),
            ]

        big_copies = [
            pltpu.make_async_copy(wo_hbm, wo_s, sem_big.at[0]),
            pltpu.make_async_copy(wg_hbm, wg_s, sem_big.at[1]),
            pltpu.make_async_copy(wu_hbm, wu_s, sem_big.at[2]),
            pltpu.make_async_copy(wd_hbm, wd_s, sem_big.at[3]),
        ]

        def x_copy(i):
            r0 = pl.multiple_of(i * XC, XC)
            return pltpu.make_async_copy(x_hbm.at[pl.ds(r0, XC), :], x_s.at[pl.ds(r0, XC), :], sem_x.at[i])

        with jax.named_scope("prologue"):
            cc = pltpu.make_async_copy(ckv_hbm, ckv_s, sem_in.at[0])
            for i in range(n_xc):
                x_copy(i).start()
            cc.start()
            for c in w_copies(0):
                c.start()

            def ln_body(i, carry):
                x_copy(i).wait()
                for k in range(XC // 128):
                    r0 = pl.multiple_of(i * XC + k * 128, 128)
                    xf = x_s[pl.ds(r0, 128), :].astype(f32)
                    mu = jnp.sum(xf, axis=1, keepdims=True) * (1.0 / M)
                    d = xf - mu
                    var = jnp.sum(d * d, axis=1, keepdims=True) * (1.0 / M)
                    xn_s[pl.ds(r0, 128), :] = (d * lax.rsqrt(var + EPS)).astype(bf16)
                return carry

            lax.fori_loop(0, n_xc, ln_body, 0)
            cc.wait()

        row = lax.broadcasted_iota(jnp.int32, (T, T), 0)
        col = lax.broadcasted_iota(jnp.int32, (T, T), 1)

        def attn_step(g, t):
            step = g * steps_per_grp + t
            tri = col <= row

            @pl.when(t == 1)
            def _():
                for gg in range(4):
                    @pl.when(g == gg)
                    def _():
                        big_copies[gg].start()

            if HPS == 2:
                def unpack(u_ref, rows):
                    w = u_ref[pl.ds(t, rows, stride=pairs_per_grp), :]
                    lo = pltpu.bitcast(w << 16, f32).astype(bf16)
                    hi = pltpu.bitcast(w & jnp.uint32(0xFFFF0000), f32).astype(bf16)
                    return lo, hi
            else:
                def unpack(u_ref, rows):
                    w = u_ref[pl.ds(t // 2, rows, stride=pairs_per_grp), :]
                    sh = (16 * (1 - t % 2)).astype(u32)
                    return (pltpu.bitcast((w << sh) & jnp.uint32(0xFFFF0000), f32).astype(bf16),)

            wk2 = unpack(uk, C)
            wq2 = unpack(uq, M)
            wv2 = unpack(uv, C)

            def kproj(hh):
                k_s[hh] = jnp.dot(ckv_s[...], wk2[hh], preferred_element_type=f32).astype(bf16)

            def vproj(hh):
                v_s[hh] = jnp.dot(ckv_s[...], wv2[hh], preferred_element_type=f32).astype(bf16)

            def qproj(hh, i):
                L0 = i * TQ
                return jnp.dot(xn_s[L0:L0 + TQ, :], wq2[hh], preferred_element_type=f32) * scale

            def qk(hh, i, qf):
                L0 = i * TQ
                ss = [lax.dot_general(qf.astype(bf16), k_s[hh, 0:L0 + T, :], NT, preferred_element_type=f32)]
                for j in range(1, ns):
                    ss.append(lax.dot_general(qf[j * T:].astype(bf16), k_s[hh, L0 + j * T:L0 + (j + 1) * T, :], NT,
                                              preferred_element_type=f32))
                return ss

            def softmax_pv(hh, i, ss):
                L0 = i * TQ
                p_parts = [[] for _ in range(ns)]
                rl = []
                for r in range(ns):
                    pieces = [ss[0][r * T:(r + 1) * T, :]] + [ss[j][(r - j) * T:(r - j + 1) * T, :]
                                                              for j in range(1, r + 1)]
                    last = pieces[-1]
                    if r == 0 and L0 > 0:
                        last = jnp.concatenate([last[:, :L0], jnp.where(tri, last[:, L0:], NEG)], axis=1)
                    else:
                        last = jnp.where(tri, last, NEG)
                    pieces[-1] = last
                    s = jnp.concatenate(pieces, axis=1) if len(pieces) > 1 else pieces[0]
                    m = jnp.max(s, axis=1, keepdims=True)
                    p = jnp.exp2(s - m)
                    rl.append(_recip(jnp.sum(p, axis=1, keepdims=True)))
                    p_parts[0].append(p[:, :L0 + T])
                    for j in range(1, r + 1):
                        p_parts[j].append(p[:, L0 + j * T:L0 + (j + 1) * T])
                o0 = jnp.dot(jnp.concatenate(p_parts[0], axis=0).astype(bf16), v_s[hh, 0:L0 + T, :],
                             preferred_element_type=f32)
                os_ = [o0[r * T:(r + 1) * T] for r in range(ns)]
                for j in range(1, ns):
                    oj = jnp.dot(jnp.concatenate(p_parts[j], axis=0).astype(bf16),
                                 v_s[hh, L0 + j * T:L0 + (j + 1) * T, :], preferred_element_type=f32)
                    for r in range(j, ns):
                        os_[r] = os_[r] + oj[(r - j) * T:(r - j + 1) * T]
                for r in range(ns):
                    ctx_s[step, L0 + r * T:L0 + (r + 1) * T, hh * D:(hh + 1) * D] = (os_[r] * rl[r]).astype(bf16)

            order = [(hh, i) for hh in range(HPS) for i in range(nb - 1, -1, -1)]
            n_o = len(order)
            qs, ss = {}, {}

            def do_q(n):
                if n < n_o:
                    if order[n][1] == nb - 1:
                        kproj(order[n][0])
                    qs[n] = qproj(*order[n])

            def do_qk(n):
                if n < n_o:
                    ss[n] = qk(*order[n], qs.pop(n))
                    if order[n][1] == nb - 1:
                        vproj(order[n][0])

            do_q(0)
            do_q(1)
            do_qk(0)
            for n in range(n_o):
                do_q(n + 2)
                do_qk(n + 1)
                softmax_pv(*order[n], ss.pop(n))

        def group_body(g, carry):
            with jax.named_scope("stage1"):
                for c in w_copies(g):
                    c.wait()

                @pl.when(g + 1 < n_grp)
                def _():
                    for c in w_copies(jnp.minimum(g + 1, n_grp - 1)):
                        c.start()

                uk[...] = pltpu.bitcast(wk_raw[g].reshape(C * GRP, D), u32)
                uq[...] = pltpu.bitcast(wq_raw[g].reshape(M * GRP, D), u32)
                uv[...] = pltpu.bitcast(wv_raw[g].reshape(C * GRP, D), u32)

            def body(t, c2):
                with jax.named_scope("main"):
                    attn_step(g, t)
                return c2

            lax.fori_loop(0, steps_per_grp, body, 0)
            return carry

        lax.fori_loop(0, n_grp, group_body, 0)

        big_copies[0].wait()
        wr8 = jnp.broadcast_to(wr_ref[...], (8, M))

        def out_copy(b):
            r0 = pl.multiple_of(b * RB, RB)
            return pltpu.make_async_copy(out_s.at[pl.ds(r0, RB), :], out_hbm.at[pl.ds(r0, RB), :], sem_out.at[b])

        def oproj(b):
            r0 = pl.multiple_of(b * RB, RB)
            lhs = jnp.concatenate([ctx_s[j, pl.ds(r0, RB), :] for j in range(n_steps)], axis=1)
            attn_s[pl.ds(r0, RB), :] = jnp.dot(lhs, wo_s[...], preferred_element_type=f32).astype(bf16)

        def post(b):
            r0 = pl.multiple_of(b * RB, RB)
            h = (x_s[pl.ds(r0, RB), :].astype(f32) + attn_s[pl.ds(r0, RB), :].astype(f32)).astype(bf16)
            hf = h.astype(f32)
            mu = jnp.sum(hf, axis=1, keepdims=True) * (1.0 / M)
            dc = hf - mu
            var = jnp.sum(dc * dc, axis=1, keepdims=True) * (1.0 / M)
            den = _rnd(jnp.sqrt(_rnd(_rnd(var) + _rnd(jnp.full((1, 1), EPS, f32)))))
            hn = (_rnd(hf - _rnd(mu)) * (1.0 / den)).astype(bf16)
            h_s[pl.ds(r0, RB), :] = h
            hn_s[pl.ds(r0, RB), :] = hn
            out_s[pl.ds(r0, RB), :] = (hf + hn.astype(f32)).astype(bf16)
            return hn

        def router(b, hn):
            r_s[b] = _rnd(lax.dot_general(wr8, hn, NT, preferred_element_type=f32))
            out_copy(b).start()

        with jax.named_scope("oproj0"):
            oproj(0)

        def body(b, carry):
            with jax.named_scope("oloop"):
                hn = post(b - 1)
                oproj(b)
                router(b - 1, hn)
            return carry

        lax.fori_loop(1, n_rb, body, 0)
        with jax.named_scope("tail"):
            router(n_rb - 1, post(n_rb - 1))

            r_all = jnp.concatenate([r_s[b] for b in range(n_rb)], axis=1)
            pos = lax.broadcasted_iota(jnp.int32, (8, S), 1)
            m1 = jnp.max(r_all)
            i1 = jnp.min(jnp.where(r_all == m1, pos, S))
            i1 = jnp.minimum(i1, S - 1)
            rest = jnp.where(pos == i1, -jnp.inf, r_all)
            m2 = jnp.max(rest)
            i2 = jnp.min(jnp.where((rest == m2) & (pos != i1), pos, S))
            i2 = jnp.minimum(i2, S - 1)

            g1 = pl.multiple_of((i1 // 16) * 16, 16)
            g2 = pl.multiple_of((i2 // 16) * 16, 16)
            xs = jnp.concatenate([hn_s[pl.ds(g1, 16), :].astype(f32), hn_s[pl.ds(g2, 16), :].astype(f32)], axis=0)
            hs = jnp.concatenate([h_s[pl.ds(g1, 16), :].astype(f32), h_s[pl.ds(g2, 16), :].astype(f32)], axis=0)
            big_copies[1].wait()
            big_copies[2].wait()
            big_copies[3].wait()
            xb = xs.astype(bf16)
            g = _rnd(jnp.dot(xb, wg_s[...], preferred_element_type=f32))
            u = _rnd(jnp.dot(xb, wu_s[...], preferred_element_type=f32))
            gu = (_rnd(g * jax.nn.sigmoid(g)) * u).astype(bf16)
            y = _rnd(jnp.dot(gu, wd_s[...], preferred_element_type=f32))
            rid = lax.broadcasted_iota(jnp.int32, (32, 1), 0)
            tok = jnp.where(rid < 16, g1 + rid, g2 + rid - 16)
            rsel = jnp.where(tok == i1, m1, m2)
            upd = jnp.where((tok == i1) | (tok == i2), _rnd(y * _rnd(jax.nn.sigmoid(rsel))), 0.0)
            fixed = (hs + _rnd(xs + upd)).astype(bf16)

            for b in range(n_rb):
                out_copy(b).wait()
            out_s[pl.ds(g1, 16), :] = fixed[0:16]
            out_s[pl.ds(g2, 16), :] = fixed[16:32]
            c1 = pltpu.make_async_copy(out_s.at[pl.ds(g1, 16), :], out_hbm.at[pl.ds(g1, 16), :], sem_fix.at[0])
            c2 = pltpu.make_async_copy(out_s.at[pl.ds(g2, 16), :], out_hbm.at[pl.ds(g2, 16), :], sem_fix.at[1])
            c1.start()

            @pl.when(g1 != g2)
            def _():
                c2.start()
                c2.wait()

            c1.wait()

    scratch = [
        pltpu.VMEM((S, M), bf16),
        pltpu.VMEM((S, M), bf16),
        pltpu.VMEM((S, C), bf16),
        pltpu.VMEM((n_grp, M, GRP, D), bf16),
        pltpu.VMEM((n_grp, C, GRP, D), bf16),
        pltpu.VMEM((n_grp, C, GRP, D), bf16),
        pltpu.VMEM((M * GRP // 2, D), u32),
        pltpu.VMEM((C * GRP // 2, D), u32),
        pltpu.VMEM((C * GRP // 2, D), u32),
        pltpu.VMEM((HPS, S, D), bf16),
        pltpu.VMEM((HPS, S, D), bf16),
        pltpu.VMEM((n_steps, S, HPS * D), bf16),
        pltpu.VMEM((H * D, M), bf16),
        pltpu.VMEM((M, F), bf16),
        pltpu.VMEM((M, F), bf16),
        pltpu.VMEM((F, M), bf16),
        pltpu.VMEM((S, M), bf16),
        pltpu.VMEM((S, M), bf16),
        pltpu.VMEM((S, M), bf16),
        pltpu.VMEM((n_rb, 8, RB), f32),
        pltpu.VMEM((S, M), bf16),
        pltpu.SemaphoreType.DMA((1,)),
        pltpu.SemaphoreType.DMA((n_xc,)),
        pltpu.SemaphoreType.DMA((3 * n_grp,)),
        pltpu.SemaphoreType.DMA((4,)),
        pltpu.SemaphoreType.DMA((n_rb,)),
        pltpu.SemaphoreType.DMA((2,)),
    ]
    return kernel, scratch, n_steps


@jax.jit
def pallas_sequential_preLN__compressed_kv_cla__moe_arch_mod__prompt_kernel(
    A_x: jax.Array,
    A_c_kv: jax.Array,
    A_w_q: jax.Array,
    A_w_uk: jax.Array,
    A_w_uv: jax.Array,
    A_w_o: jax.Array,
    B_x: jax.Array,
    B_w_r: jax.Array,
    B_w_gate: jax.Array,
    B_w_up: jax.Array,
    B_w_down: jax.Array,
):
    B, S, M = A_x.shape
    C = A_c_kv.shape[2]
    H, D = A_w_q.shape[1], A_w_q.shape[2]
    F = B_w_gate.shape[1]
    assert B == 1 and A_c_kv.shape[1] == S

    kernel, scratch, n_steps = _make_kernel(S, M, C, H, D, F)
    any_spec = pl.BlockSpec(memory_space=pl.ANY)
    out = pl.pallas_call(
        kernel,
        in_specs=[any_spec] * 6 + [pl.BlockSpec(memory_space=pltpu.VMEM)] + [any_spec] * 3,
        out_specs=any_spec,
        out_shape=jax.ShapeDtypeStruct((S, M), A_x.dtype),
        scratch_shapes=scratch,
        compiler_params=pltpu.CompilerParams(
            vmem_limit_bytes=120 * 1024 * 1024,
        ),
        name="mla_mod_block",
    )(
        A_x.reshape(S, M), A_c_kv.reshape(S, C), A_w_q, A_w_uk, A_w_uv,
        A_w_o.reshape(H * D, M), B_w_r.reshape(1, M), B_w_gate, B_w_up, B_w_down,
    )
    return out.reshape(B, S, M)
```

```python
import jax
import jax.numpy as jnp
from jax import lax
import jax.experimental.pallas as pl
import jax.experimental.pallas.tpu as pltpu

bf16 = jnp.bfloat16
f32 = jnp.float32
u32 = jnp.uint32

T = 128
AHEAD = 3
QAHEAD = 1
WB = 4
RB = 256
NP = 16
XC = 256
WD_PAD = 128
EPS = 1e-5
NEG = -1e30
LOG2E = 1.4426950408889634
NT = (((1,), (1,)), ((), ()))


def _rnd(x):
    return x.astype(bf16).astype(f32)


def _recip(l):
    r = pl.reciprocal(l, approx=True)
    return r * (2.0 - l * r)


def _make_kernel(S, M, C, H, D, F):
    n_pair = H // 2
    nb = S // T
    n_rb = S // RB
    n_xc = S // XC
    PR = RB // NP
    qa, ka = M // WB, C // WB
    scale = (D ** -0.5) * LOG2E

    def kernel(x_hbm, ckv_hbm, wq_hbm, wk_hbm, wv_hbm, wo_hbm, wr_ref, wg_hbm, wu_hbm, wd_hbm,
               out_hbm,
               x_s, xn_s, ckv_s, w_s, ctx_s,
               wo_s, wg_s, wu_s, wd_s, attn_s, h_s, hn_s, out_s,
               sem_in, sem_x, sem_w, sem_big, sem_out, sem_fix):

        def w_start(p, slot):
            for hbm, r0, n in ((wk_hbm, qa, ka), (wq_hbm, 0, qa), (wv_hbm, qa + ka, ka)):
                for b in range(WB):
                    pltpu.make_async_copy(hbm.at[:, b, p], w_s.at[slot, pl.ds(r0, n), pl.ds(2 * b, 2), :],
                                          sem_w.at[slot]).start()

        def w_wait(slot):
            pltpu.make_async_copy(w_s.at[slot], w_s.at[slot], sem_w.at[slot]).wait()

        big_copies = [
            pltpu.make_async_copy(wo_hbm, wo_s.at[:, pl.ds(0, M)], sem_big.at[0]),
            pltpu.make_async_copy(wg_hbm, wg_s, sem_big.at[1]),
            pltpu.make_async_copy(wu_hbm, wu_s, sem_big.at[2]),
            pltpu.make_async_copy(wd_hbm, wd_s.at[:, pl.ds(0, M)], sem_big.at[3]),
        ]

        def x_copy(i):
            r0 = pl.multiple_of(i * XC, XC)
            return pltpu.make_async_copy(x_hbm.at[pl.ds(r0, XC), :], x_s.at[pl.ds(r0, XC), :], sem_x.at[i])

        with jax.named_scope("prologue"):
            cc = pltpu.make_async_copy(ckv_hbm, ckv_s, sem_in.at[0])
            for i in range(n_xc):
                x_copy(i).start()
            cc.start()
            w_start(0, 0)

            def ln_body(i, carry):
                x_copy(i).wait()
                for k in range(XC // 128):
                    r0 = pl.multiple_of(i * XC + k * 128, 128)
                    xf = x_s[pl.ds(r0, 128), :].astype(f32)
                    mu = jnp.sum(xf, axis=1, keepdims=True) * (1.0 / M)
                    d = xf - mu
                    var = jnp.sum(d * d, axis=1, keepdims=True) * (1.0 / M)
                    xn_s[pl.ds(pl.multiple_of(r0 // 2, 64), 64), :] = pltpu.bitcast((d * lax.rsqrt(var + EPS)).astype(bf16), u32)
                return carry

            lax.fori_loop(0, n_xc, ln_body, 0)
            cc.wait()

        row = lax.broadcasted_iota(jnp.int32, (T, T), 0)
        col = lax.broadcasted_iota(jnp.int32, (T, T), 1)

        def head_step(p, slot, e):
            @pl.when(e == 0)
            def _():
                w_wait(slot)

            tri = col <= row
            sh = (16 * (1 - e)).astype(u32)

            def unpack(r0, n):
                w = pltpu.bitcast(w_s[slot, r0:r0 + n].reshape(n * 2 * WB, D), u32)
                return pltpu.bitcast((w << sh) & jnp.uint32(0xFFFF0000), f32).astype(bf16)

            wk = unpack(qa, ka)
            wq = unpack(0, qa)
            wv = unpack(qa + ka, ka)

            @pl.when((e == 0) & (p + 1 < n_pair))
            def _():
                w_start(jnp.minimum(p + 1, n_pair - 1), 1 - slot)

            for j in range(4):
                @pl.when((e == 1) & (p == 2 * j))
                def _():
                    big_copies[j].start()

            def qproj(i):
                xn = pltpu.bitcast(xn_s[i * T // 2:(i + 1) * T // 2, :], bf16)
                q = jnp.dot(xn, wq, preferred_element_type=f32)
                return (q * scale).astype(bf16)

            def qk(i, q):
                return lax.dot_general(q, kv[0][0:(i + 1) * T, :], NT, preferred_element_type=f32)

            def softmax_pv(i, s):
                diag = jnp.where(tri, s[:, i * T:], NEG)
                s = jnp.concatenate([s[:, :i * T], diag], axis=1) if i > 0 else diag
                m = jnp.max(s, axis=1, keepdims=True)
                pb = jnp.exp2(s - m).astype(bf16)
                l = jnp.sum(pb.astype(f32), axis=1, keepdims=True)
                o = jnp.dot(pb, kv[1][0:(i + 1) * T, :], preferred_element_type=f32)
                ctx_s[2 * p + e, i * T // 2:(i + 1) * T // 2, :] = pltpu.bitcast((o * _recip(l)).astype(bf16), u32)

            order = list(range(nb - 1, -1, -1))
            qs, ss = {}, {}

            def do_q(n):
                if n < nb:
                    qs[n] = qproj(order[n])

            def do_qk(n):
                if n < nb:
                    ss[n] = qk(order[n], qs.pop(n))

            kv = [jnp.dot(ckv_s[...], wk, preferred_element_type=f32).astype(bf16)]
            for n in range(AHEAD + QAHEAD):
                do_q(n)
                if n >= QAHEAD:
                    do_qk(n - QAHEAD)
                if n == QAHEAD:
                    kv.append(jnp.dot(ckv_s[...], wv, preferred_element_type=f32).astype(bf16))
            for n in range(nb):
                do_q(n + AHEAD + QAHEAD)
                do_qk(n + AHEAD)
                softmax_pv(order[n], ss.pop(n))

        def head_body(h, carry):
            with jax.named_scope("main"):
                head_step(h >> 1, (h >> 1) & 1, h & 1)
            return carry

        lax.fori_loop(0, H, head_body, 0)

        for c in big_copies:
            c.wait()
        wr = wr_ref[...].astype(f32)

        def out_copy(b):
            r0 = pl.multiple_of(b * RB, RB)
            return pltpu.make_async_copy(out_s.at[pl.ds(r0, RB), :], out_hbm.at[pl.ds(r0, RB), :], sem_out.at[b])

        def oproj(b):
            r0 = pl.multiple_of(b * (RB // 2), RB // 2)
            lhs = pltpu.bitcast(jnp.concatenate([ctx_s[j, pl.ds(r0, RB // 2), :] for j in range(H)], axis=1), bf16)
            o = jnp.dot(lhs, wo_s[:, 0:M], preferred_element_type=f32)
            attn_s[...] = pltpu.bitcast(o.astype(bf16), u32)

        def post(b, top, chain):
            for n in range(NP):
                r0 = pl.multiple_of(b * RB + n * PR, PR)
                xf = x_s[pl.ds(r0, PR), :].astype(f32)
                if chain and n > 0:
                    xf = jnp.where(r * r < 0.0, 0.0, xf)
                h = (xf + pltpu.bitcast(attn_s[n * PR // 2:(n + 1) * PR // 2, :], bf16).astype(f32)).astype(bf16)
                hf = h.astype(f32)
                mu = jnp.sum(hf, axis=1, keepdims=True) * (1.0 / M)
                dc = hf - mu
                var = jnp.sum(dc * dc, axis=1, keepdims=True) * (1.0 / M)
                den = _rnd(jnp.sqrt(_rnd(_rnd(var) + _rnd(jnp.full((1, 1), EPS, f32)))))
                hn = (_rnd(hf - _rnd(mu)) * (1.0 / den)).astype(bf16)
                hnf = hn.astype(f32)
                h_s[pl.ds(r0, PR), :] = h
                hn_s[pl.ds(r0, PR), :] = hn
                out_s[pl.ds(r0, PR), :] = (hf + hnf).astype(bf16)
                r = _rnd(jnp.sum(hnf * wr, axis=1, keepdims=True))
                m1, i1, m2, i2 = top
                idx = r0 + lax.broadcasted_iota(jnp.int32, (PR, 1), 0)
                g1, g2 = r > m1, r > m2
                top = (jnp.where(g1, r, m1), jnp.where(g1, idx, i1),
                       jnp.where(g1, m1, jnp.where(g2, r, m2)), jnp.where(g1, i1, jnp.where(g2, idx, i2)))
            return top

        with jax.named_scope("oproj0"):
            oproj(0)

        def body(b, top):
            with jax.named_scope("oloop"):
                top = post(b - 1, top, True)
                oproj(b)
                out_copy(b - 1).start()
            return top

        slot_id = lax.broadcasted_iota(jnp.int32, (PR, 1), 0)
        ninf = jnp.full((PR, 1), -jnp.inf, f32)
        top = lax.fori_loop(1, n_rb, body, (ninf, slot_id, ninf, slot_id + PR))
        with jax.named_scope("tail"):
            top = post(n_rb - 1, top, False)
            out_copy(n_rb - 1).start()

            val = jnp.concatenate([top[0], top[2]], axis=0)
            pos = jnp.concatenate([top[1], top[3]], axis=0).astype(f32)
            m1 = jnp.max(val, axis=0, keepdims=True)
            p1 = jnp.min(jnp.where(val == m1, pos, float(S)), axis=0, keepdims=True)
            rest = jnp.where(pos == p1, -jnp.inf, val)
            m2 = jnp.max(rest, axis=0, keepdims=True)
            p2 = jnp.min(jnp.where((rest == m2) & (pos != p1), pos, float(S)), axis=0, keepdims=True)
            i1 = jnp.clip(p1.astype(jnp.int32)[0, 0], 0, S - 1)
            i2 = jnp.clip(p2.astype(jnp.int32)[0, 0], 0, S - 1)

            g1 = pl.multiple_of((i1 // 16) * 16, 16)
            g2 = pl.multiple_of((i2 // 16) * 16, 16)
            xs = jnp.concatenate([hn_s[pl.ds(g1, 16), :].astype(f32), hn_s[pl.ds(g2, 16), :].astype(f32)], axis=0)
            hs = jnp.concatenate([h_s[pl.ds(g1, 16), :].astype(f32), h_s[pl.ds(g2, 16), :].astype(f32)], axis=0)
            xb = xs.astype(bf16)
            g = _rnd(jnp.dot(xb, wg_s[...], preferred_element_type=f32))
            u = _rnd(jnp.dot(xb, wu_s[...], preferred_element_type=f32))
            gu = (_rnd(g * jax.nn.sigmoid(g)) * u).astype(bf16)
            y = _rnd(jnp.dot(gu, wd_s[:, 0:M], preferred_element_type=f32))
            rid = lax.broadcasted_iota(jnp.int32, (32, 1), 0)
            tok = jnp.where(rid < 16, g1 + rid, g2 + rid - 16)
            rsel = jnp.where(tok == i1, m1, m2)
            upd = jnp.where((tok == i1) | (tok == i2), _rnd(y * _rnd(jax.nn.sigmoid(rsel))), 0.0)
            fixed = (hs + _rnd(xs + upd)).astype(bf16)

            for b in range(n_rb):
                out_copy(b).wait()
            out_s[pl.ds(g1, 16), :] = fixed[0:16]
            out_s[pl.ds(g2, 16), :] = fixed[16:32]
            c1 = pltpu.make_async_copy(out_s.at[pl.ds(g1, 16), :], out_hbm.at[pl.ds(g1, 16), :], sem_fix.at[0])
            c2 = pltpu.make_async_copy(out_s.at[pl.ds(g2, 16), :], out_hbm.at[pl.ds(g2, 16), :], sem_fix.at[1])
            c1.start()

            @pl.when(g1 != g2)
            def _():
                c2.start()
                c2.wait()

            c1.wait()

    scratch = [
        pltpu.VMEM((S, M), bf16),
        pltpu.VMEM((S // 2, M), u32),
        pltpu.VMEM((S, C), bf16),
        pltpu.VMEM((2, qa + 2 * ka, 2 * WB, D), bf16),
        pltpu.VMEM((H, S // 2, D), u32),
        pltpu.VMEM((H * D, M + WD_PAD), bf16),
        pltpu.VMEM((M, F), bf16),
        pltpu.VMEM((M, F), bf16),
        pltpu.VMEM((F, M + WD_PAD), bf16),
        pltpu.VMEM((RB // 2, M), u32),
        pltpu.VMEM((S, M), bf16),
        pltpu.VMEM((S, M), bf16),
        pltpu.VMEM((S, M), bf16),
        pltpu.SemaphoreType.DMA((1,)),
        pltpu.SemaphoreType.DMA((n_xc,)),
        pltpu.SemaphoreType.DMA((2,)),
        pltpu.SemaphoreType.DMA((4,)),
        pltpu.SemaphoreType.DMA((n_rb,)),
        pltpu.SemaphoreType.DMA((2,)),
    ]
    return kernel, scratch


@jax.jit
def pallas_sequential_preLN__compressed_kv_cla__moe_arch_mod__prompt_kernel(
    A_x: jax.Array,
    A_c_kv: jax.Array,
    A_w_q: jax.Array,
    A_w_uk: jax.Array,
    A_w_uv: jax.Array,
    A_w_o: jax.Array,
    B_x: jax.Array,
    B_w_r: jax.Array,
    B_w_gate: jax.Array,
    B_w_up: jax.Array,
    B_w_down: jax.Array,
):
    B, S, M = A_x.shape
    C = A_c_kv.shape[2]
    H, D = A_w_q.shape[1], A_w_q.shape[2]
    F = B_w_gate.shape[1]
    assert B == 1 and A_c_kv.shape[1] == S

    kernel, scratch = _make_kernel(S, M, C, H, D, F)
    any_spec = pl.BlockSpec(memory_space=pl.ANY)
    out = pl.pallas_call(
        kernel,
        in_specs=[any_spec] * 6 + [pl.BlockSpec(memory_space=pltpu.VMEM)] + [any_spec] * 3,
        out_specs=any_spec,
        out_shape=jax.ShapeDtypeStruct((S, M), A_x.dtype),
        scratch_shapes=scratch,
        compiler_params=pltpu.CompilerParams(
            vmem_limit_bytes=120 * 1024 * 1024,
            disable_bounds_checks=True,
        ),
        name="mla_mod_block",
    )(
        A_x.reshape(S, M), A_c_kv.reshape(S, C),
        A_w_q.reshape(M // WB, WB, H // 2, 2, D),
        A_w_uk.reshape(C // WB, WB, H // 2, 2, D),
        A_w_uv.reshape(C // WB, WB, H // 2, 2, D),
        A_w_o.reshape(H * D, M), B_w_r.reshape(1, M), B_w_gate, B_w_up, B_w_down,
    )
    return out.reshape(B, S, M)
```

```python
import jax
import jax.numpy as jnp
from jax import lax
import jax.experimental.pallas as pl
import jax.experimental.pallas.tpu as pltpu

bf16 = jnp.bfloat16
f32 = jnp.float32
u32 = jnp.uint32

T = 128
AHEAD = 3
QAHEAD = 1
WB = 4
RB = 256
NP = 16
LP = 32
XC = 256
WD_PAD = 128
EPS = 1e-5
NEG = -1e30
LOG2E = 1.4426950408889634
NT = (((1,), (1,)), ((), ()))


def _rnd(x):
    return x.astype(bf16).astype(f32)


def _recip(l):
    r = pl.reciprocal(l, approx=True)
    return r * (2.0 - l * r)


def _make_kernel(S, M, C, H, D, F):
    n_pair = H // 2
    nb = S // T
    n_rb = S // RB
    n_xc = S // XC
    PR = RB // NP
    qa, ka = M // WB, C // WB
    scale = (D ** -0.5) * LOG2E

    def kernel(x_hbm, ckv_hbm, wq_hbm, wk_hbm, wv_hbm, wo_hbm, wr_ref, wg_hbm, wu_hbm, wd_hbm,
               out_hbm,
               x_s, xn_s, ckv_s, w_s, kv_s, ctx_s,
               wo_s, wg_s, wu_s, wd_s, attn_s, h_s, hn_s, out_s,
               sem_in, sem_x, sem_w, sem_kv, sem_big, sem_out, sem_fix, sem_reg):

        w_parts = {"q": (wq_hbm, 0, qa), "k": (wk_hbm, qa, ka), "v": (wv_hbm, qa + ka, ka)}

        def w_start(p, slot, parts, sem):
            for name in parts:
                hbm, r0, n = w_parts[name]
                for b in range(WB):
                    pltpu.make_async_copy(hbm.at[:, b, p], w_s.at[slot, pl.ds(r0, n), pl.ds(2 * b, 2), :],
                                          sem).start()

        def w_wait(slot, r0, n, sem):
            view = w_s.at[slot, pl.ds(r0, n)]
            pltpu.make_async_copy(view, view, sem).wait()

        def unpack(slot, name, e):
            _, r0, n = w_parts[name]
            w = pltpu.bitcast(w_s[slot, r0:r0 + n].reshape(n * 2 * WB, D), u32)
            if isinstance(e, int):
                w = (w << 16) if e == 0 else (w & jnp.uint32(0xFFFF0000))
            else:
                w = (w << (16 * (1 - e)).astype(u32)) & jnp.uint32(0xFFFF0000)
            return pltpu.bitcast(w, f32).astype(bf16)

        big_copies = [
            pltpu.make_async_copy(wo_hbm, wo_s.at[:, pl.ds(0, M)], sem_big.at[0]),
            pltpu.make_async_copy(wg_hbm, wg_s, sem_big.at[1]),
            pltpu.make_async_copy(wu_hbm, wu_s, sem_big.at[2]),
            pltpu.make_async_copy(wd_hbm, wd_s.at[:, pl.ds(0, M)], sem_big.at[3]),
        ]

        def x_copy(i):
            return pltpu.make_async_copy(x_hbm.at[pl.ds(i * XC, XC), :], x_s.at[pl.ds(i * XC, XC), :], sem_x.at[i])

        def ckv_copy(i):
            rows = pl.ds(i * (S // 2), S // 2)
            return pltpu.make_async_copy(ckv_hbm.at[rows, :], ckv_s.at[rows, :], sem_in.at[i])

        def layernorm_x(c0, c1):
            mu = None
            for r0 in range(c0 * XC, c1 * XC, LP):
                xf = x_s[r0:r0 + LP, :].astype(f32)
                if mu is not None:
                    xf = jnp.where(mu * mu < 0.0, 0.0, xf)
                mu = jnp.sum(xf, axis=1, keepdims=True) * (1.0 / M)
                d = xf - mu
                var = jnp.sum(d * d, axis=1, keepdims=True) * (1.0 / M)
                xn_s[r0 // 2:(r0 + LP) // 2, :] = pltpu.bitcast((d * lax.rsqrt(var + EPS)).astype(bf16), u32)

        def kv_pre(pair, names, r0, r1):
            for j, name in names:
                for e in range(2):
                    y = jnp.dot(ckv_s[r0:r1, :], unpack(pair, name, e), preferred_element_type=f32)
                    kv_s[2 * pair + e, j, r0 // 2:r1 // 2, :] = pltpu.bitcast(y.astype(bf16), u32)

        with jax.named_scope("prologue"):
            def fence():
                pl.semaphore_signal(sem_reg, 1)
                pl.semaphore_wait(sem_reg, 1)

            w_start(0, 0, "kv", sem_kv.at[0])
            fence()
            ckv_copy(0).start()
            ckv_copy(1).start()
            fence()
            for i in range(4):
                x_copy(i).start()
            fence()
            w_start(1, 1, "kv", sem_kv.at[1])
            fence()
            for i in range(4, n_xc):
                x_copy(i).start()
            fence()
            w_start(0, 0, "q", sem_w.at[0])
            w_start(1, 1, "q", sem_w.at[1])

            both = ((0, "k"), (1, "v"))
            with jax.named_scope("w1"):
                w_wait(0, qa, 2 * ka, sem_kv.at[0])
                ckv_copy(0).wait()
            with jax.named_scope("r1"):
                kv_pre(0, both, 0, S // 2)

            with jax.named_scope("w2"):
                ckv_copy(1).wait()
                for i in range(0, 2):
                    x_copy(i).wait()
            with jax.named_scope("r2"):
                layernorm_x(0, 2)
                kv_pre(0, both, S // 2, S)

            with jax.named_scope("w3"):
                w_wait(1, qa, 2 * ka, sem_kv.at[1])
                for i in range(2, 5):
                    x_copy(i).wait()
            with jax.named_scope("r3"):
                layernorm_x(2, 5)
                kv_pre(1, both[:1], 0, S)

            with jax.named_scope("w4"):
                for i in range(5, n_xc):
                    x_copy(i).wait()
            with jax.named_scope("r4"):
                layernorm_x(5, n_xc)
                kv_pre(1, both[1:], 0, S)
            with jax.named_scope("w5"):
                w_wait(0, 0, qa, sem_w.at[0])
                w_wait(1, 0, qa, sem_w.at[1])

        row = lax.broadcasted_iota(jnp.int32, (T, T), 0)
        col = lax.broadcasted_iota(jnp.int32, (T, T), 1)

        def head_step(h, have_kv):
            p = h >> 1
            slot = p & 1
            e = h & 1
            if not have_kv:
                @pl.when(e == 0)
                def _():
                    w_wait(slot, 0, qa + 2 * ka, sem_w.at[slot])

            tri = col <= row
            wq = unpack(slot, "q", e)
            if have_kv:
                @pl.when(h == 2)
                def _():
                    w_start(2, 0, "kqv", sem_w.at[0])
            else:
                wk = unpack(slot, "k", e)
                wv = unpack(slot, "v", e)

                @pl.when((e == 0) & (p + 1 < n_pair))
                def _():
                    w_start(jnp.minimum(p + 1, n_pair - 1), 1 - slot, "kqv", sem_w.at[1 - slot])

                for j in range(4):
                    @pl.when((e == 1) & (p == 2 * j + 2))
                    def _():
                        big_copies[j].start()

            def qproj(i):
                xn = pltpu.bitcast(xn_s[i * T // 2:(i + 1) * T // 2, :], bf16)
                q = jnp.dot(xn, wq, preferred_element_type=f32)
                return (q * scale).astype(bf16)

            def qk(i, q):
                return lax.dot_general(q, kv[0][0:(i + 1) * T, :], NT, preferred_element_type=f32)

            def softmax_pv(i, s):
                diag = jnp.where(tri, s[:, i * T:], NEG)
                s = jnp.concatenate([s[:, :i * T], diag], axis=1) if i > 0 else diag
                m = jnp.max(s, axis=1, keepdims=True)
                pb = jnp.exp2(s - m).astype(bf16)
                l = jnp.sum(pb.astype(f32), axis=1, keepdims=True)
                o = jnp.dot(pb, kv[1][0:(i + 1) * T, :], preferred_element_type=f32)
                ctx_s[h, i * T // 2:(i + 1) * T // 2, :] = pltpu.bitcast((o * _recip(l)).astype(bf16), u32)

            order = list(range(nb - 1, -1, -1))
            qs, ss = {}, {}

            def do_q(n):
                if n < nb:
                    qs[n] = qproj(order[n])

            def do_qk(n):
                if n < nb:
                    ss[n] = qk(order[n], qs.pop(n))

            if have_kv:
                kv = [pltpu.bitcast(kv_s[h, j], bf16) for j in range(2)]
            else:
                kv = [jnp.dot(ckv_s[...], wk, preferred_element_type=f32).astype(bf16)]
            for n in range(AHEAD + QAHEAD):
                do_q(n)
                if n >= QAHEAD:
                    do_qk(n - QAHEAD)
                if n == QAHEAD and not have_kv:
                    kv.append(jnp.dot(ckv_s[...], wv, preferred_element_type=f32).astype(bf16))
            for n in range(nb):
                do_q(n + AHEAD + QAHEAD)
                do_qk(n + AHEAD)
                softmax_pv(order[n], ss.pop(n))

        def first_body(h, carry):
            with jax.named_scope("first"):
                head_step(h, True)
            return carry

        def head_body(h, carry):
            with jax.named_scope("main"):
                head_step(h, False)
            return carry

        lax.fori_loop(0, 4, first_body, 0)
        lax.fori_loop(4, H, head_body, 0)

        for c in big_copies:
            c.wait()
        wr = wr_ref[...].astype(f32)

        def out_copy(b):
            r0 = pl.multiple_of(b * RB, RB)
            return pltpu.make_async_copy(out_s.at[pl.ds(r0, RB), :], out_hbm.at[pl.ds(r0, RB), :], sem_out.at[b])

        def oproj(b):
            r0 = pl.multiple_of(b * (RB // 2), RB // 2)
            lhs = pltpu.bitcast(jnp.concatenate([ctx_s[j, pl.ds(r0, RB // 2), :] for j in range(H)], axis=1), bf16)
            o = jnp.dot(lhs, wo_s[:, 0:M], preferred_element_type=f32)
            attn_s[...] = pltpu.bitcast(o.astype(bf16), u32)

        def post(b, top, chain):
            for n in range(NP):
                r0 = pl.multiple_of(b * RB + n * PR, PR)
                xf = x_s[pl.ds(r0, PR), :].astype(f32)
                if chain and n > 0:
                    xf = jnp.where(r * r < 0.0, 0.0, xf)
                h = (xf + pltpu.bitcast(attn_s[n * PR // 2:(n + 1) * PR // 2, :], bf16).astype(f32)).astype(bf16)
                hf = h.astype(f32)
                mu = jnp.sum(hf, axis=1, keepdims=True) * (1.0 / M)
                dc = hf - mu
                var = jnp.sum(dc * dc, axis=1, keepdims=True) * (1.0 / M)
                den = _rnd(jnp.sqrt(_rnd(_rnd(var) + _rnd(jnp.full((1, 1), EPS, f32)))))
                hn = (_rnd(hf - _rnd(mu)) * (1.0 / den)).astype(bf16)
                hnf = hn.astype(f32)
                h_s[pl.ds(r0, PR), :] = h
                hn_s[pl.ds(r0, PR), :] = hn
                out_s[pl.ds(r0, PR), :] = (hf + hnf).astype(bf16)
                r = _rnd(jnp.sum(hnf * wr, axis=1, keepdims=True))
                m1, i1, m2, i2 = top
                idx = r0 + lax.broadcasted_iota(jnp.int32, (PR, 1), 0)
                g1, g2 = r > m1, r > m2
                top = (jnp.where(g1, r, m1), jnp.where(g1, idx, i1),
                       jnp.where(g1, m1, jnp.where(g2, r, m2)), jnp.where(g1, i1, jnp.where(g2, idx, i2)))
            return top

        with jax.named_scope("oproj0"):
            oproj(0)

        def body(b, top):
            with jax.named_scope("oloop"):
                top = post(b - 1, top, True)
                oproj(b)
                out_copy(b - 1).start()
            return top

        slot_id = lax.broadcasted_iota(jnp.int32, (PR, 1), 0)
        ninf = jnp.full((PR, 1), -jnp.inf, f32)
        top = lax.fori_loop(1, n_rb, body, (ninf, slot_id, ninf, slot_id + PR))
        with jax.named_scope("tail"):
            top = post(n_rb - 1, top, False)
            out_copy(n_rb - 1).start()

            val = jnp.concatenate([top[0], top[2]], axis=0)
            pos = jnp.concatenate([top[1], top[3]], axis=0).astype(f32)
            m1 = jnp.max(val, axis=0, keepdims=True)
            p1 = jnp.min(jnp.where(val == m1, pos, float(S)), axis=0, keepdims=True)
            rest = jnp.where(pos == p1, -jnp.inf, val)
            m2 = jnp.max(rest, axis=0, keepdims=True)
            p2 = jnp.min(jnp.where((rest == m2) & (pos != p1), pos, float(S)), axis=0, keepdims=True)
            i1 = jnp.clip(p1.astype(jnp.int32)[0, 0], 0, S - 1)
            i2 = jnp.clip(p2.astype(jnp.int32)[0, 0], 0, S - 1)

            g1 = pl.multiple_of((i1 // 16) * 16, 16)
            g2 = pl.multiple_of((i2 // 16) * 16, 16)
            xs = jnp.concatenate([hn_s[pl.ds(g1, 16), :].astype(f32), hn_s[pl.ds(g2, 16), :].astype(f32)], axis=0)
            hs = jnp.concatenate([h_s[pl.ds(g1, 16), :].astype(f32), h_s[pl.ds(g2, 16), :].astype(f32)], axis=0)
            xb = xs.astype(bf16)
            g = _rnd(jnp.dot(xb, wg_s[...], preferred_element_type=f32))
            u = _rnd(jnp.dot(xb, wu_s[...], preferred_element_type=f32))
            gu = (_rnd(g * jax.nn.sigmoid(g)) * u).astype(bf16)
            y = _rnd(jnp.dot(gu, wd_s[:, 0:M], preferred_element_type=f32))
            rid = lax.broadcasted_iota(jnp.int32, (32, 1), 0)
            tok = jnp.where(rid < 16, g1 + rid, g2 + rid - 16)
            rsel = jnp.where(tok == i1, m1, m2)
            upd = jnp.where((tok == i1) | (tok == i2), _rnd(y * _rnd(jax.nn.sigmoid(rsel))), 0.0)
            fixed = (hs + _rnd(xs + upd)).astype(bf16)

            for b in range(n_rb):
                out_copy(b).wait()
            out_s[pl.ds(g1, 16), :] = fixed[0:16]
            out_s[pl.ds(g2, 16), :] = fixed[16:32]
            c1 = pltpu.make_async_copy(out_s.at[pl.ds(g1, 16), :], out_hbm.at[pl.ds(g1, 16), :], sem_fix.at[0])
            c2 = pltpu.make_async_copy(out_s.at[pl.ds(g2, 16), :], out_hbm.at[pl.ds(g2, 16), :], sem_fix.at[1])
            c1.start()

            @pl.when(g1 != g2)
            def _():
                c2.start()
                c2.wait()

            c1.wait()

    scratch = [
        pltpu.VMEM((S, M), bf16),
        pltpu.VMEM((S // 2, M), u32),
        pltpu.VMEM((S, C), bf16),
        pltpu.VMEM((2, qa + 2 * ka, 2 * WB, D), bf16),
        pltpu.VMEM((4, 2, S // 2, D), u32),
        pltpu.VMEM((H, S // 2, D), u32),
        pltpu.VMEM((H * D, M + WD_PAD), bf16),
        pltpu.VMEM((M, F), bf16),
        pltpu.VMEM((M, F), bf16),
        pltpu.VMEM((F, M + WD_PAD), bf16),
        pltpu.VMEM((RB // 2, M), u32),
        pltpu.VMEM((S, M), bf16),
        pltpu.VMEM((S, M), bf16),
        pltpu.VMEM((S, M), bf16),
        pltpu.SemaphoreType.DMA((2,)),
        pltpu.SemaphoreType.DMA((n_xc,)),
        pltpu.SemaphoreType.DMA((2,)),
        pltpu.SemaphoreType.DMA((2,)),
        pltpu.SemaphoreType.DMA((4,)),
        pltpu.SemaphoreType.DMA((n_rb,)),
        pltpu.SemaphoreType.DMA((2,)),
        pltpu.SemaphoreType.REGULAR,
    ]
    return kernel, scratch


@jax.jit
def pallas_sequential_preLN__compressed_kv_cla__moe_arch_mod__prompt_kernel(
    A_x: jax.Array,
    A_c_kv: jax.Array,
    A_w_q: jax.Array,
    A_w_uk: jax.Array,
    A_w_uv: jax.Array,
    A_w_o: jax.Array,
    B_x: jax.Array,
    B_w_r: jax.Array,
    B_w_gate: jax.Array,
    B_w_up: jax.Array,
    B_w_down: jax.Array,
):
    B, S, M = A_x.shape
    C = A_c_kv.shape[2]
    H, D = A_w_q.shape[1], A_w_q.shape[2]
    F = B_w_gate.shape[1]
    assert B == 1 and A_c_kv.shape[1] == S

    kernel, scratch = _make_kernel(S, M, C, H, D, F)
    any_spec = pl.BlockSpec(memory_space=pl.ANY)
    out = pl.pallas_call(
        kernel,
        in_specs=[any_spec] * 6 + [pl.BlockSpec(memory_space=pltpu.VMEM)] + [any_spec] * 3,
        out_specs=any_spec,
        out_shape=jax.ShapeDtypeStruct((S, M), A_x.dtype),
        scratch_shapes=scratch,
        compiler_params=pltpu.CompilerParams(
            vmem_limit_bytes=120 * 1024 * 1024,
            disable_bounds_checks=True,
        ),
        name="mla_mod_block",
    )(
        A_x.reshape(S, M), A_c_kv.reshape(S, C),
        A_w_q.reshape(M // WB, WB, H // 2, 2, D),
        A_w_uk.reshape(C // WB, WB, H // 2, 2, D),
        A_w_uv.reshape(C // WB, WB, H // 2, 2, D),
        A_w_o.reshape(H * D, M), B_w_r.reshape(1, M), B_w_gate, B_w_up, B_w_down,
    )
    return out.reshape(B, S, M)
```

```python
import jax
import jax.numpy as jnp
from jax import lax
import jax.experimental.pallas as pl
import jax.experimental.pallas.tpu as pltpu

bf16 = jnp.bfloat16
f32 = jnp.float32
u32 = jnp.uint32

T = 128
AHEAD = 3
QAHEAD = 2
WB = 4
BLKS = (256,) * 7 + (128, 64, 64)
PR = 16
LCH = 4
LP = 16
XC = 256
WD_PAD = 128
EPS = 1e-5
NEG = -1e30
LOG2E = 1.4426950408889634
NT = (((1,), (1,)), ((), ()))


def _rnd(x):
    return x.astype(bf16).astype(f32)


def _recip(l):
    r = pl.reciprocal(l, approx=True)
    return r * (2.0 - l * r)


def _make_kernel(S, M, C, H, D, F):
    n_pair = H // 2
    nb = S // T
    offs = [sum(BLKS[:b]) for b in range(len(BLKS))]
    assert sum(BLKS) == S
    n_xc = S // XC
    qa, ka = M // WB, C // WB
    scale = (D ** -0.5) * LOG2E

    def kernel(x_hbm, ckv_hbm, wq_hbm, wk_hbm, wv_hbm, wo_hbm, wr_hbm, wg_hbm, wu_hbm, wd_hbm,
               out_hbm,
               x_s, xn_s, ckv_s, w_s, kv_s, ctx_s,
               wo_s, wr_s, wg_s, wu_s, wd_s, h_s, hn_s, out_s,
               sem_in, sem_x, sem_w, sem_kv, sem_big, sem_out, sem_fix, sem_reg):

        w_parts = {"q": (wq_hbm, 0, qa), "k": (wk_hbm, qa, ka), "v": (wv_hbm, qa + ka, ka)}

        def w_start(p, slot, parts, sem):
            for name in parts:
                hbm, r0, n = w_parts[name]
                for b in range(WB):
                    pltpu.make_async_copy(hbm.at[:, b, p], w_s.at[slot, pl.ds(r0, n), pl.ds(2 * b, 2), :],
                                          sem).start()

        def w_wait(slot, r0, n, sem):
            view = w_s.at[slot, pl.ds(r0, n)]
            pltpu.make_async_copy(view, view, sem).wait()

        def unpack(slot, name, e):
            _, r0, n = w_parts[name]
            w = pltpu.bitcast(w_s[slot, r0:r0 + n].reshape(n * 2 * WB, D), u32)
            if isinstance(e, int):
                w = (w << 16) if e == 0 else (w & jnp.uint32(0xFFFF0000))
            else:
                w = (w << (16 * (1 - e)).astype(u32)) & jnp.uint32(0xFFFF0000)
            return pltpu.bitcast(w, f32).astype(bf16)

        big_copies = [
            pltpu.make_async_copy(wo_hbm, wo_s.at[:, pl.ds(0, M)], sem_big.at[0]),
            pltpu.make_async_copy(wg_hbm, wg_s, sem_big.at[1]),
            pltpu.make_async_copy(wu_hbm, wu_s, sem_big.at[2]),
            pltpu.make_async_copy(wd_hbm, wd_s.at[:, pl.ds(0, M)], sem_big.at[3]),
            pltpu.make_async_copy(wr_hbm, wr_s, sem_big.at[4]),
        ]

        def x_copy(i):
            return pltpu.make_async_copy(x_hbm.at[pl.ds(i * XC, XC), :], x_s.at[pl.ds(i * XC, XC), :], sem_x.at[i])

        def ckv_copy(i):
            rows = pl.ds(i * (S // 2), S // 2)
            return pltpu.make_async_copy(ckv_hbm.at[rows, :], ckv_s.at[rows, :], sem_in.at[i])

        def layernorm_x(c0, c1):
            toks = []
            for r0 in range(c0 * XC, c1 * XC, LP):
                xf = x_s[r0:r0 + LP, :].astype(f32)
                if len(toks) >= LCH:
                    xf = jnp.where(toks[-LCH] < 0.0, 0.0, xf)
                elif toks:
                    xf = jnp.where(mu * mu < 0.0, 0.0, xf)
                mu = jnp.sum(xf, axis=1, keepdims=True) * (1.0 / M)
                d = xf - mu
                var = jnp.sum(d * d, axis=1, keepdims=True) * (1.0 / M)
                rs = lax.rsqrt(var + EPS)
                y = d * rs
                toks.append(rs)
                xn_s[r0 // 2:(r0 + LP) // 2, :] = pltpu.bitcast(y.astype(bf16), u32)

        def kv_pre(pair, names, r0, r1):
            for j, name in names:
                for e in range(2):
                    y = jnp.dot(ckv_s[r0:r1, :], unpack(pair, name, e), preferred_element_type=f32)
                    kv_s[2 * pair + e, j, r0 // 2:r1 // 2, :] = pltpu.bitcast(y.astype(bf16), u32)

        with jax.named_scope("prologue"):
            def fence():
                pl.semaphore_signal(sem_reg, 1)
                pl.semaphore_wait(sem_reg, 1)

            w_start(0, 0, "kv", sem_kv.at[0])
            fence()
            ckv_copy(0).start()
            ckv_copy(1).start()
            fence()
            for i in range(4):
                x_copy(i).start()
            fence()
            w_start(1, 1, "kv", sem_kv.at[1])
            fence()
            for i in range(4, n_xc):
                x_copy(i).start()
            fence()
            w_start(0, 0, "q", sem_w.at[0])
            w_start(1, 1, "q", sem_w.at[1])

            both = ((0, "k"), (1, "v"))
            with jax.named_scope("w1"):
                w_wait(0, qa, 2 * ka, sem_kv.at[0])
                ckv_copy(0).wait()
            with jax.named_scope("r1"):
                kv_pre(0, both, 0, S // 2)

            with jax.named_scope("w2"):
                ckv_copy(1).wait()
                for i in range(0, 2):
                    x_copy(i).wait()
            with jax.named_scope("r2"):
                layernorm_x(0, 2)
                kv_pre(0, both, S // 2, S)

            with jax.named_scope("w3"):
                w_wait(1, qa, 2 * ka, sem_kv.at[1])
                for i in range(2, 5):
                    x_copy(i).wait()
            with jax.named_scope("r3"):
                layernorm_x(2, 5)
                kv_pre(1, both[:1], 0, S)

            with jax.named_scope("w4"):
                for i in range(5, n_xc):
                    x_copy(i).wait()
            with jax.named_scope("r4"):
                layernorm_x(5, n_xc)
                kv_pre(1, both[1:], 0, S)
            with jax.named_scope("w5"):
                w_wait(0, 0, qa, sem_w.at[0])
                w_wait(1, 0, qa, sem_w.at[1])

        row = lax.broadcasted_iota(jnp.int32, (T, T), 0)
        col = lax.broadcasted_iota(jnp.int32, (T, T), 1)

        def head_step(h, have_kv):
            p = h >> 1
            slot = p & 1
            e = h & 1
            if not have_kv:
                @pl.when(e == 0)
                def _():
                    w_wait(slot, 0, qa + 2 * ka, sem_w.at[slot])

            tri = col <= row
            wq = unpack(slot, "q", e)
            if have_kv:
                @pl.when(h == 2)
                def _():
                    w_start(2, 0, "kqv", sem_w.at[0])
            else:
                wk = unpack(slot, "k", e)
                wv = unpack(slot, "v", e)

                @pl.when((e == 0) & (p + 1 < n_pair))
                def _():
                    w_start(jnp.minimum(p + 1, n_pair - 1), 1 - slot, "kqv", sem_w.at[1 - slot])

                for j in range(len(big_copies)):
                    @pl.when((e == 1) & (p == 2 * j + 2))
                    def _():
                        big_copies[j].start()

            def qproj(i):
                xn = pltpu.bitcast(xn_s[i * T // 2:(i + 1) * T // 2, :], bf16)
                q = jnp.dot(xn, wq, preferred_element_type=f32)
                return (q * scale).astype(bf16)

            def qk(i, q):
                return lax.dot_general(q, kv[0][0:(i + 1) * T, :], NT, preferred_element_type=f32)

            def softmax_pv(i, s):
                diag = jnp.where(tri, s[:, i * T:], NEG)
                s = jnp.concatenate([s[:, :i * T], diag], axis=1) if i > 0 else diag
                m = jnp.max(s, axis=1, keepdims=True)
                pb = jnp.exp2(s - m).astype(bf16)
                l = jnp.sum(pb.astype(f32), axis=1, keepdims=True)
                o = jnp.dot(pb, kv[1][0:(i + 1) * T, :], preferred_element_type=f32)
                ctx_s[h, i * T // 2:(i + 1) * T // 2, :] = pltpu.bitcast((o * _recip(l)).astype(bf16), u32)

            order = list(range(nb - 1, -1, -1))
            qs, ss = {}, {}

            def do_q(n):
                if n < nb:
                    qs[n] = qproj(order[n])

            def do_qk(n):
                if n < nb:
                    ss[n] = qk(order[n], qs.pop(n))

            if have_kv:
                kv = [pltpu.bitcast(kv_s[h, j], bf16) for j in range(2)]
            else:
                kv = [jnp.dot(ckv_s[...], wk, preferred_element_type=f32).astype(bf16)]
            for n in range(AHEAD + QAHEAD):
                do_q(n)
                if n >= QAHEAD:
                    do_qk(n - QAHEAD)
                if n == QAHEAD and not have_kv:
                    kv.append(jnp.dot(ckv_s[...], wv, preferred_element_type=f32).astype(bf16))
            for n in range(nb):
                do_q(n + AHEAD + QAHEAD)
                do_qk(n + AHEAD)
                softmax_pv(order[n], ss.pop(n))

        def first_body(h, carry):
            with jax.named_scope("first"):
                head_step(h, True)
            return carry

        def head_body(h, carry):
            with jax.named_scope("main"):
                head_step(h, False)
            return carry

        lax.fori_loop(0, 4, first_body, 0)
        lax.fori_loop(4, H, head_body, 0)

        for c in big_copies:
            c.wait()
        wr = wr_s[...].astype(f32).reshape(1, M)

        def out_copy(b):
            rows = pl.ds(offs[b], BLKS[b])
            return pltpu.make_async_copy(out_s.at[rows, :], out_hbm.at[rows, :], sem_out.at[b])

        def oproj(b):
            r0, r1 = offs[b] // 2, (offs[b] + BLKS[b]) // 2
            lhs = pltpu.bitcast(jnp.concatenate([ctx_s[j, r0:r1, :] for j in range(H)], axis=1), bf16)
            return jnp.dot(lhs, wo_s[:, 0:M], preferred_element_type=f32).astype(bf16)

        def post(b, attn, top, r):
            chain = b + 1 < len(BLKS)
            for n in range(BLKS[b] // PR):
                r0 = offs[b] + n * PR
                xf = x_s[r0:r0 + PR, :].astype(f32)
                if chain and r is not None:
                    xf = jnp.where(r * r < 0.0, 0.0, xf)
                h = (xf + attn[n * PR:(n + 1) * PR].astype(f32)).astype(bf16)
                hf = h.astype(f32)
                mu = jnp.sum(hf, axis=1, keepdims=True) * (1.0 / M)
                dc = hf - mu
                var = jnp.sum(dc * dc, axis=1, keepdims=True) * (1.0 / M)
                den = _rnd(jnp.sqrt(_rnd(_rnd(var) + _rnd(jnp.full((1, 1), EPS, f32)))))
                hn = (_rnd(hf - _rnd(mu)) * (1.0 / den)).astype(bf16)
                hnf = hn.astype(f32)
                h_s[r0:r0 + PR, :] = h
                hn_s[r0:r0 + PR, :] = hn
                out_s[r0:r0 + PR, :] = (hf + hnf).astype(bf16)
                r = _rnd(jnp.sum(hnf * wr, axis=1, keepdims=True))
                m1, i1, m2, i2 = top
                idx = r0 + slot_id
                g1, g2 = r > m1, r > m2
                top = (jnp.where(g1, r, m1), jnp.where(g1, idx, i1),
                       jnp.where(g1, m1, jnp.where(g2, r, m2)), jnp.where(g1, i1, jnp.where(g2, idx, i2)))
            out_copy(b).start()
            return top, r

        slot_id = lax.broadcasted_iota(jnp.int32, (PR, 1), 0)
        ninf = jnp.full((PR, 1), -jnp.inf, f32)
        top, r = (ninf, slot_id, ninf, slot_id + PR), None
        with jax.named_scope("tail"):
            attn = oproj(0)
            for b in range(len(BLKS)):
                nxt = oproj(b + 1) if b + 1 < len(BLKS) else None
                top, r = post(b, attn, top, r)
                attn = nxt

            val = jnp.concatenate([top[0], top[2]], axis=0)
            pos = jnp.concatenate([top[1], top[3]], axis=0).astype(f32)
            m1 = jnp.max(val, axis=0, keepdims=True)
            p1 = jnp.min(jnp.where(val == m1, pos, float(S)), axis=0, keepdims=True)
            rest = jnp.where(pos == p1, -jnp.inf, val)
            m2 = jnp.max(rest, axis=0, keepdims=True)
            p2 = jnp.min(jnp.where((rest == m2) & (pos != p1), pos, float(S)), axis=0, keepdims=True)
            i1 = jnp.clip(p1.astype(jnp.int32)[0, 0], 0, S - 1)
            i2 = jnp.clip(p2.astype(jnp.int32)[0, 0], 0, S - 1)

            g1 = pl.multiple_of((i1 // 16) * 16, 16)
            g2 = pl.multiple_of((i2 // 16) * 16, 16)
            xs = jnp.concatenate([hn_s[pl.ds(g1, 16), :].astype(f32), hn_s[pl.ds(g2, 16), :].astype(f32)], axis=0)
            hs = jnp.concatenate([h_s[pl.ds(g1, 16), :].astype(f32), h_s[pl.ds(g2, 16), :].astype(f32)], axis=0)
            xb = xs.astype(bf16)
            g = _rnd(jnp.dot(xb, wg_s[...], preferred_element_type=f32))
            u = _rnd(jnp.dot(xb, wu_s[...], preferred_element_type=f32))
            gu = (_rnd(g * jax.nn.sigmoid(g)) * u).astype(bf16)
            y = _rnd(jnp.dot(gu, wd_s[:, 0:M], preferred_element_type=f32))
            rid = lax.broadcasted_iota(jnp.int32, (32, 1), 0)
            tok = jnp.where(rid < 16, g1 + rid, g2 + rid - 16)
            rsel = jnp.where(tok == i1, m1, m2)
            upd = jnp.where((tok == i1) | (tok == i2), _rnd(y * _rnd(jax.nn.sigmoid(rsel))), 0.0)
            fixed = (hs + _rnd(xs + upd)).astype(bf16)

            for b in range(len(BLKS)):
                out_copy(b).wait()
            out_s[pl.ds(g1, 16), :] = fixed[0:16]
            out_s[pl.ds(g2, 16), :] = fixed[16:32]
            c1 = pltpu.make_async_copy(out_s.at[pl.ds(g1, 16), :], out_hbm.at[pl.ds(g1, 16), :], sem_fix.at[0])
            c2 = pltpu.make_async_copy(out_s.at[pl.ds(g2, 16), :], out_hbm.at[pl.ds(g2, 16), :], sem_fix.at[1])
            c1.start()

            @pl.when(g1 != g2)
            def _():
                c2.start()
                c2.wait()

            c1.wait()

    scratch = [
        pltpu.VMEM((S, M), bf16),
        pltpu.VMEM((S // 2, M), u32),
        pltpu.VMEM((S, C), bf16),
        pltpu.VMEM((2, qa + 2 * ka, 2 * WB, D), bf16),
        pltpu.VMEM((4, 2, S // 2, D), u32),
        pltpu.VMEM((H, S // 2, D), u32),
        pltpu.VMEM((H * D, M + WD_PAD), bf16),
        pltpu.VMEM((M,), bf16),
        pltpu.VMEM((M, F), bf16),
        pltpu.VMEM((M, F), bf16),
        pltpu.VMEM((F, M + WD_PAD), bf16),
        pltpu.VMEM((S, M), bf16),
        pltpu.VMEM((S, M), bf16),
        pltpu.VMEM((S, M), bf16),
        pltpu.SemaphoreType.DMA((2,)),
        pltpu.SemaphoreType.DMA((n_xc,)),
        pltpu.SemaphoreType.DMA((2,)),
        pltpu.SemaphoreType.DMA((2,)),
        pltpu.SemaphoreType.DMA((5,)),
        pltpu.SemaphoreType.DMA((len(BLKS),)),
        pltpu.SemaphoreType.DMA((2,)),
        pltpu.SemaphoreType.REGULAR,
    ]
    return kernel, scratch


@jax.jit
def pallas_sequential_preLN__compressed_kv_cla__moe_arch_mod__prompt_kernel(
    A_x: jax.Array,
    A_c_kv: jax.Array,
    A_w_q: jax.Array,
    A_w_uk: jax.Array,
    A_w_uv: jax.Array,
    A_w_o: jax.Array,
    B_x: jax.Array,
    B_w_r: jax.Array,
    B_w_gate: jax.Array,
    B_w_up: jax.Array,
    B_w_down: jax.Array,
):
    B, S, M = A_x.shape
    C = A_c_kv.shape[2]
    H, D = A_w_q.shape[1], A_w_q.shape[2]
    F = B_w_gate.shape[1]
    assert B == 1 and A_c_kv.shape[1] == S

    kernel, scratch = _make_kernel(S, M, C, H, D, F)
    any_spec = pl.BlockSpec(memory_space=pl.ANY)
    out = pl.pallas_call(
        kernel,
        in_specs=[any_spec] * 10,
        out_specs=any_spec,
        out_shape=jax.ShapeDtypeStruct((S, M), A_x.dtype),
        scratch_shapes=scratch,
        compiler_params=pltpu.CompilerParams(
            vmem_limit_bytes=120 * 1024 * 1024,
            disable_bounds_checks=True,
        ),
        name="mla_mod_block",
    )(
        A_x.reshape(S, M), A_c_kv.reshape(S, C),
        A_w_q.reshape(M // WB, WB, H // 2, 2, D),
        A_w_uk.reshape(C // WB, WB, H // 2, 2, D),
        A_w_uv.reshape(C // WB, WB, H // 2, 2, D),
        A_w_o.reshape(H * D, M), B_w_r, B_w_gate, B_w_up, B_w_down,
    )
    return out.reshape(B, S, M)
```

```python
import jax
import jax.numpy as jnp
from jax import lax
import jax.experimental.pallas as pl
import jax.experimental.pallas.tpu as pltpu

bf16 = jnp.bfloat16
f32 = jnp.float32
u32 = jnp.uint32

T = 128
G = 64
A = T // G
AHEAD = 3
QAHEAD = 2
WB = 4
BLKS = (256,) * 7 + (128, 64, 64)
PR = 16
LCH = 4
LP = 16
XC = 256
WD_PAD = 128
EPS = 1e-5
NEG = -1e30
LOG2E = 1.4426950408889634
NT = (((1,), (1,)), ((), ()))


def _rnd(x):
    return x.astype(bf16).astype(f32)


def _recip(l):
    r = pl.reciprocal(l, approx=True)
    return r * (2.0 - l * r)


def _make_kernel(S, M, C, H, D, F):
    n_pair = H // 2
    nb = S // T
    offs = [sum(BLKS[:b]) for b in range(len(BLKS))]
    assert sum(BLKS) == S
    n_xc = S // XC
    qa, ka = M // WB, C // WB
    scale = (D ** -0.5) * LOG2E

    def kernel(x_hbm, ckv_hbm, wq_hbm, wk_hbm, wv_hbm, wo_hbm, wr_hbm, wg_hbm, wu_hbm, wd_hbm,
               out_hbm,
               x_s, xn_s, ckv_s, w_s, kv_s, ctx_s,
               wo_s, wr_s, wg_s, wu_s, wd_s, h_s, hn_s, out_s,
               sem_in, sem_x, sem_w, sem_kv, sem_big, sem_out, sem_fix, sem_reg):

        w_parts = {"q": (wq_hbm, 0, qa), "k": (wk_hbm, qa, ka), "v": (wv_hbm, qa + ka, ka)}

        def w_start(p, slot, parts, sem):
            for name in parts:
                hbm, r0, n = w_parts[name]
                for b in range(WB):
                    pltpu.make_async_copy(hbm.at[:, b, p], w_s.at[slot, pl.ds(r0, n), pl.ds(2 * b, 2), :],
                                          sem).start()

        def w_wait(slot, r0, n, sem):
            view = w_s.at[slot, pl.ds(r0, n)]
            pltpu.make_async_copy(view, view, sem).wait()

        def unpack(slot, name, e):
            _, r0, n = w_parts[name]
            w = pltpu.bitcast(w_s[slot, r0:r0 + n].reshape(n * 2 * WB, D), u32)
            if isinstance(e, int):
                w = (w << 16) if e == 0 else (w & jnp.uint32(0xFFFF0000))
            else:
                w = (w << (16 * (1 - e)).astype(u32)) & jnp.uint32(0xFFFF0000)
            return pltpu.bitcast(w, f32).astype(bf16)

        big_copies = [
            pltpu.make_async_copy(wo_hbm, wo_s.at[:, pl.ds(0, M)], sem_big.at[0]),
            pltpu.make_async_copy(wg_hbm, wg_s, sem_big.at[1]),
            pltpu.make_async_copy(wu_hbm, wu_s, sem_big.at[2]),
            pltpu.make_async_copy(wd_hbm, wd_s.at[:, pl.ds(0, M)], sem_big.at[3]),
            pltpu.make_async_copy(wr_hbm, wr_s, sem_big.at[4]),
        ]

        def x_copy(i):
            return pltpu.make_async_copy(x_hbm.at[pl.ds(i * XC, XC), :], x_s.at[pl.ds(i * XC, XC), :], sem_x.at[i])

        def ckv_copy(i):
            rows = pl.ds(i * (S // 2), S // 2)
            return pltpu.make_async_copy(ckv_hbm.at[rows, :], ckv_s.at[rows, :], sem_in.at[i])

        def layernorm_x(c0, c1):
            toks = []
            for r0 in range(c0 * XC, c1 * XC, LP):
                xf = x_s[r0:r0 + LP, :].astype(f32)
                if len(toks) >= LCH:
                    xf = jnp.where(toks[-LCH] < 0.0, 0.0, xf)
                elif toks:
                    xf = jnp.where(mu * mu < 0.0, 0.0, xf)
                mu = jnp.sum(xf, axis=1, keepdims=True) * (1.0 / M)
                d = xf - mu
                var = jnp.sum(d * d, axis=1, keepdims=True) * (1.0 / M)
                rs = lax.rsqrt(var + EPS)
                y = d * rs
                toks.append(rs)
                xn_s[r0 // 2:(r0 + LP) // 2, :] = pltpu.bitcast(y.astype(bf16), u32)

        def kv_pre(pair, names, r0, r1):
            for j, name in names:
                for e in range(2):
                    y = jnp.dot(ckv_s[r0:r1, :], unpack(pair, name, e), preferred_element_type=f32)
                    kv_s[2 * pair + e, j, r0 // 2:r1 // 2, :] = pltpu.bitcast(y.astype(bf16), u32)

        with jax.named_scope("prologue"):
            def fence():
                pl.semaphore_signal(sem_reg, 1)
                pl.semaphore_wait(sem_reg, 1)

            w_start(0, 0, "kv", sem_kv.at[0])
            fence()
            ckv_copy(0).start()
            ckv_copy(1).start()
            fence()
            for i in range(4):
                x_copy(i).start()
            fence()
            w_start(1, 1, "kv", sem_kv.at[1])
            fence()
            for i in range(4, n_xc):
                x_copy(i).start()
            fence()
            w_start(0, 0, "q", sem_w.at[0])
            w_start(1, 1, "q", sem_w.at[1])

            both = ((0, "k"), (1, "v"))
            with jax.named_scope("w1"):
                w_wait(0, qa, 2 * ka, sem_kv.at[0])
                ckv_copy(0).wait()
            with jax.named_scope("r1"):
                kv_pre(0, both, 0, S // 2)

            with jax.named_scope("w2"):
                ckv_copy(1).wait()
                for i in range(0, 2):
                    x_copy(i).wait()
            with jax.named_scope("r2"):
                layernorm_x(0, 2)
                kv_pre(0, both, S // 2, S)

            with jax.named_scope("w3"):
                w_wait(1, qa, 2 * ka, sem_kv.at[1])
                for i in range(2, 5):
                    x_copy(i).wait()
            with jax.named_scope("r3"):
                layernorm_x(2, 5)
                kv_pre(1, both[:1], 0, S)

            with jax.named_scope("w4"):
                for i in range(5, n_xc):
                    x_copy(i).wait()
            with jax.named_scope("r4"):
                layernorm_x(5, n_xc)
                kv_pre(1, both[1:], 0, S)
            with jax.named_scope("w5"):
                w_wait(0, 0, qa, sem_w.at[0])
                w_wait(1, 0, qa, sem_w.at[1])

        row = lax.broadcasted_iota(jnp.int32, (G, T), 0)
        col = lax.broadcasted_iota(jnp.int32, (G, T), 1)

        def head_step(h, have_kv):
            p = h >> 1
            slot = p & 1
            e = h & 1
            if not have_kv:
                @pl.when(e == 0)
                def _():
                    w_wait(slot, 0, qa + 2 * ka, sem_w.at[slot])

            tri = col <= row + (T - G)
            wq = unpack(slot, "q", e)
            if have_kv:
                @pl.when(h == 2)
                def _():
                    w_start(2, 0, "kqv", sem_w.at[0])
            else:
                wk = unpack(slot, "k", e)
                wv = unpack(slot, "v", e)

                @pl.when((e == 0) & (p + 1 < n_pair))
                def _():
                    w_start(jnp.minimum(p + 1, n_pair - 1), 1 - slot, "kqv", sem_w.at[1 - slot])

                for j in range(len(big_copies)):
                    @pl.when((e == 1) & (p == 2 * j + 2))
                    def _():
                        big_copies[j].start()

            def geom(blk):
                c, j = blk
                k0 = (c + 1) * G % T
                return k0, A * j + (0 if k0 else 1), [(A * j + a) * T + c * G for a in range(A)]

            def qproj(blk):
                xn = jnp.concatenate([xn_s[r // 2:(r + G) // 2, :] for r in geom(blk)[2]], axis=0)
                return jnp.dot(pltpu.bitcast(xn, bf16), wq, preferred_element_type=f32) * scale

            def qk(blk, qf):
                k0, n, _ = geom(blk)
                kk = kv[0]
                q = qf.astype(bf16)
                main = head = None
                if n:
                    main = lax.dot_general(q, kk[k0:k0 + n * T, :], NT, preferred_element_type=f32)
                if k0:
                    st = lax.dot_general(kk[0:k0, :], q, NT, preferred_element_type=f32)
                    head = jnp.concatenate([st, jnp.full((T - k0, T), NEG, f32)], axis=0).T
                extra = [lax.dot_general(qf[e * G:].astype(bf16), kk[k0 + (n + e - 1) * T:k0 + (n + e) * T, :], NT,
                                         preferred_element_type=f32) for e in range(1, A)]
                return main, head, extra

            def softmax_pv(blk, sc):
                k0, n, rows = geom(blk)
                vv = kv[1]
                main, head, extra = sc
                ps, rls = [], []
                for a in range(A):
                    parts = []
                    if n:
                        mm = main[a * G:(a + 1) * G]
                        if a == 0:
                            parts += [mm[:, :(n - 1) * T]] if n > 1 else []
                            parts.append(jnp.where(tri, mm[:, (n - 1) * T:], NEG))
                        else:
                            parts.append(mm)
                    if k0:
                        hd = head[a * G:(a + 1) * G]
                        parts.append(hd if n + a else jnp.where(col <= row + (k0 - G), hd, NEG))
                    for e in range(1, a + 1):
                        ex = extra[e - 1][(a - e) * G:(a - e + 1) * G]
                        parts.append(jnp.where(tri, ex, NEG) if e == a else ex)
                    s = jnp.concatenate(parts, axis=1) if len(parts) > 1 else parts[0]
                    pr = jnp.exp2(s - jnp.max(s, axis=1, keepdims=True))
                    rls.append(_recip(jnp.sum(_rnd(pr), axis=1, keepdims=True)))
                    ps.append(pr)
                w = ps[0].shape[1]
                vm = [vv[k0:k0 + n * T, :]] if n else []
                vm += [vv[0:T, :]] if k0 else []
                o = jnp.dot(jnp.concatenate([x[:, :w] for x in ps], axis=0).astype(bf16),
                            jnp.concatenate(vm, axis=0) if len(vm) > 1 else vm[0], preferred_element_type=f32)
                outs = [o[a * G:(a + 1) * G] for a in range(A)]
                for e in range(1, A):
                    pe = jnp.concatenate([x[:, w + (e - 1) * T:w + e * T] for x in ps[e:]], axis=0).astype(bf16)
                    oe = jnp.dot(pe, vv[k0 + (n + e - 1) * T:k0 + (n + e) * T, :], preferred_element_type=f32)
                    for a in range(e, A):
                        outs[a] = outs[a] + oe[(a - e) * G:(a - e + 1) * G]
                for a, r in enumerate(rows):
                    ctx_s[h, r // 2:(r + G) // 2, :] = pltpu.bitcast((outs[a] * rls[a]).astype(bf16), u32)

            order = [(c, j) for j in range(nb // A - 1, -1, -1) for c in range(A)]
            qs, ss = {}, {}

            def do_q(n):
                if n < nb:
                    qs[n] = qproj(order[n])

            def do_qk(n):
                if n < nb:
                    ss[n] = qk(order[n], qs.pop(n))

            if have_kv:
                kv = [pltpu.bitcast(kv_s[h, j], bf16) for j in range(2)]
            else:
                kv = [jnp.dot(ckv_s[...], wk, preferred_element_type=f32).astype(bf16)]
            for n in range(AHEAD + QAHEAD):
                do_q(n)
                if n >= QAHEAD:
                    do_qk(n - QAHEAD)
                if n == QAHEAD and not have_kv:
                    kv.append(jnp.dot(ckv_s[...], wv, preferred_element_type=f32).astype(bf16))
            for n in range(nb):
                do_q(n + AHEAD + QAHEAD)
                do_qk(n + AHEAD)
                softmax_pv(order[n], ss.pop(n))

        def first_body(h, carry):
            with jax.named_scope("first"):
                head_step(h, True)
            return carry

        def head_body(h, carry):
            with jax.named_scope("main"):
                head_step(h, False)
            return carry

        lax.fori_loop(0, 4, first_body, 0)
        lax.fori_loop(4, H, head_body, 0)

        for c in big_copies:
            c.wait()
        wr = wr_s[...].astype(f32).reshape(1, M)

        def out_copy(b):
            rows = pl.ds(offs[b], BLKS[b])
            return pltpu.make_async_copy(out_s.at[rows, :], out_hbm.at[rows, :], sem_out.at[b])

        def oproj(b):
            r0, r1 = offs[b] // 2, (offs[b] + BLKS[b]) // 2
            lhs = pltpu.bitcast(jnp.concatenate([ctx_s[j, r0:r1, :] for j in range(H)], axis=1), bf16)
            return jnp.dot(lhs, wo_s[:, 0:M], preferred_element_type=f32).astype(bf16)

        def post(b, attn, top, r):
            chain = b + 1 < len(BLKS)
            for n in range(BLKS[b] // PR):
                r0 = offs[b] + n * PR
                xf = x_s[r0:r0 + PR, :].astype(f32)
                if chain and r is not None:
                    xf = jnp.where(r * r < 0.0, 0.0, xf)
                h = (xf + attn[n * PR:(n + 1) * PR].astype(f32)).astype(bf16)
                hf = h.astype(f32)
                mu = jnp.sum(hf, axis=1, keepdims=True) * (1.0 / M)
                dc = hf - mu
                var = jnp.sum(dc * dc, axis=1, keepdims=True) * (1.0 / M)
                den = _rnd(jnp.sqrt(_rnd(_rnd(var) + _rnd(jnp.full((1, 1), EPS, f32)))))
                hn = (_rnd(hf - _rnd(mu)) * (1.0 / den)).astype(bf16)
                hnf = hn.astype(f32)
                h_s[r0:r0 + PR, :] = h
                hn_s[r0:r0 + PR, :] = hn
                out_s[r0:r0 + PR, :] = (hf + hnf).astype(bf16)
                r = _rnd(jnp.sum(hnf * wr, axis=1, keepdims=True))
                m1, i1, m2, i2 = top
                idx = r0 + slot_id
                g1, g2 = r > m1, r > m2
                top = (jnp.where(g1, r, m1), jnp.where(g1, idx, i1),
                       jnp.where(g1, m1, jnp.where(g2, r, m2)), jnp.where(g1, i1, jnp.where(g2, idx, i2)))
            out_copy(b).start()
            return top, r

        slot_id = lax.broadcasted_iota(jnp.int32, (PR, 1), 0)
        ninf = jnp.full((PR, 1), -jnp.inf, f32)
        top, r = (ninf, slot_id, ninf, slot_id + PR), None
        with jax.named_scope("tail"):
            attn = oproj(0)
            for b in range(len(BLKS)):
                nxt = oproj(b + 1) if b + 1 < len(BLKS) else None
                top, r = post(b, attn, top, r)
                attn = nxt

            val = jnp.concatenate([top[0], top[2]], axis=0)
            pos = jnp.concatenate([top[1], top[3]], axis=0).astype(f32)
            m1 = jnp.max(val, axis=0, keepdims=True)
            p1 = jnp.min(jnp.where(val == m1, pos, float(S)), axis=0, keepdims=True)
            rest = jnp.where(pos == p1, -jnp.inf, val)
            m2 = jnp.max(rest, axis=0, keepdims=True)
            p2 = jnp.min(jnp.where((rest == m2) & (pos != p1), pos, float(S)), axis=0, keepdims=True)
            i1 = jnp.clip(p1.astype(jnp.int32)[0, 0], 0, S - 1)
            i2 = jnp.clip(p2.astype(jnp.int32)[0, 0], 0, S - 1)

            g1 = pl.multiple_of((i1 // 16) * 16, 16)
            g2 = pl.multiple_of((i2 // 16) * 16, 16)
            xs = jnp.concatenate([hn_s[pl.ds(g1, 16), :].astype(f32), hn_s[pl.ds(g2, 16), :].astype(f32)], axis=0)
            hs = jnp.concatenate([h_s[pl.ds(g1, 16), :].astype(f32), h_s[pl.ds(g2, 16), :].astype(f32)], axis=0)
            xb = xs.astype(bf16)
            g = _rnd(jnp.dot(xb, wg_s[...], preferred_element_type=f32))
            u = _rnd(jnp.dot(xb, wu_s[...], preferred_element_type=f32))
            gu = (_rnd(g * jax.nn.sigmoid(g)) * u).astype(bf16)
            y = _rnd(jnp.dot(gu, wd_s[:, 0:M], preferred_element_type=f32))
            rid = lax.broadcasted_iota(jnp.int32, (32, 1), 0)
            tok = jnp.where(rid < 16, g1 + rid, g2 + rid - 16)
            rsel = jnp.where(tok == i1, m1, m2)
            upd = jnp.where((tok == i1) | (tok == i2), _rnd(y * _rnd(jax.nn.sigmoid(rsel))), 0.0)
            fixed = (hs + _rnd(xs + upd)).astype(bf16)

            for b in range(len(BLKS)):
                out_copy(b).wait()
            out_s[pl.ds(g1, 16), :] = fixed[0:16]
            out_s[pl.ds(g2, 16), :] = fixed[16:32]
            c1 = pltpu.make_async_copy(out_s.at[pl.ds(g1, 16), :], out_hbm.at[pl.ds(g1, 16), :], sem_fix.at[0])
            c2 = pltpu.make_async_copy(out_s.at[pl.ds(g2, 16), :], out_hbm.at[pl.ds(g2, 16), :], sem_fix.at[1])
            c1.start()

            @pl.when(g1 != g2)
            def _():
                c2.start()
                c2.wait()

            c1.wait()

    scratch = [
        pltpu.VMEM((S, M), bf16),
        pltpu.VMEM((S // 2, M), u32),
        pltpu.VMEM((S, C), bf16),
        pltpu.VMEM((2, qa + 2 * ka, 2 * WB, D), bf16),
        pltpu.VMEM((4, 2, S // 2, D), u32),
        pltpu.VMEM((H, S // 2, D), u32),
        pltpu.VMEM((H * D, M + WD_PAD), bf16),
        pltpu.VMEM((M,), bf16),
        pltpu.VMEM((M, F), bf16),
        pltpu.VMEM((M, F), bf16),
        pltpu.VMEM((F, M + WD_PAD), bf16),
        pltpu.VMEM((S, M), bf16),
        pltpu.VMEM((S, M), bf16),
        pltpu.VMEM((S, M), bf16),
        pltpu.SemaphoreType.DMA((2,)),
        pltpu.SemaphoreType.DMA((n_xc,)),
        pltpu.SemaphoreType.DMA((2,)),
        pltpu.SemaphoreType.DMA((2,)),
        pltpu.SemaphoreType.DMA((5,)),
        pltpu.SemaphoreType.DMA((len(BLKS),)),
        pltpu.SemaphoreType.DMA((2,)),
        pltpu.SemaphoreType.REGULAR,
    ]
    return kernel, scratch


@jax.jit
def pallas_sequential_preLN__compressed_kv_cla__moe_arch_mod__prompt_kernel(
    A_x: jax.Array,
    A_c_kv: jax.Array,
    A_w_q: jax.Array,
    A_w_uk: jax.Array,
    A_w_uv: jax.Array,
    A_w_o: jax.Array,
    B_x: jax.Array,
    B_w_r: jax.Array,
    B_w_gate: jax.Array,
    B_w_up: jax.Array,
    B_w_down: jax.Array,
):
    B, S, M = A_x.shape
    C = A_c_kv.shape[2]
    H, D = A_w_q.shape[1], A_w_q.shape[2]
    F = B_w_gate.shape[1]
    assert B == 1 and A_c_kv.shape[1] == S

    kernel, scratch = _make_kernel(S, M, C, H, D, F)
    any_spec = pl.BlockSpec(memory_space=pl.ANY)
    out = pl.pallas_call(
        kernel,
        in_specs=[any_spec] * 10,
        out_specs=any_spec,
        out_shape=jax.ShapeDtypeStruct((S, M), A_x.dtype),
        scratch_shapes=scratch,
        compiler_params=pltpu.CompilerParams(
            vmem_limit_bytes=120 * 1024 * 1024,
            disable_bounds_checks=True,
        ),
        name="mla_mod_block",
    )(
        A_x.reshape(S, M), A_c_kv.reshape(S, C),
        A_w_q.reshape(M // WB, WB, H // 2, 2, D),
        A_w_uk.reshape(C // WB, WB, H // 2, 2, D),
        A_w_uv.reshape(C // WB, WB, H // 2, 2, D),
        A_w_o.reshape(H * D, M), B_w_r, B_w_gate, B_w_up, B_w_down,
    )
    return out.reshape(B, S, M)
```

```python
import jax
import jax.numpy as jnp
from jax import lax
import jax.experimental.pallas as pl
import jax.experimental.pallas.tpu as pltpu

bf16 = jnp.bfloat16
f32 = jnp.float32
u32 = jnp.uint32

T = 128
G = 64
A = T // G
AHEAD = 3
QAHEAD = 2
WB = 4
BLKS = (256,) * 7 + (128, 64, 64)
PR = 16
LCH = 4
LP = 16
XC = 256
CKV_SPLIT = (0, 256, 768, 1408, 2048)
PRO_ORDER = ([("w", 0)] + [("c", i) for i in range(4)] + [("x", i) for i in range(3)] + [("w", 1)]
             + [("x", i) for i in range(3, 8)] + [("q", 0), ("q", 1)])
PRO_STEPS = [
    ([("w", 0), ("c", 0)], (0, 0), [(0, 0, 256)]),
    ([("c", 1)], (0, 0), [(0, 256, 768)]),
    ([("c", 2)], (0, 0), [(0, 768, 1408)]),
    ([("c", 3), ("x", 0), ("x", 1)], (0, 2), [(0, 1408, 2048)]),
    ([("w", 1), ("x", 2), ("x", 3)], (2, 4), [(1, 0, 704)]),
    ([("x", 4), ("x", 5)], (4, 6), [(1, 704, 1376)]),
    ([("x", 6), ("x", 7)], (6, 8), [(1, 1376, 2048)]),
    ([("q", 0), ("q", 1)], (0, 0), []),
]
WD_PAD = 128
EPS = 1e-5
NEG = -1e30
LOG2E = 1.4426950408889634
NT = (((1,), (1,)), ((), ()))


def _rnd(x):
    return x.astype(bf16).astype(f32)


def _recip(l):
    r = pl.reciprocal(l, approx=True)
    return r * (2.0 - l * r)


def _make_kernel(S, M, C, H, D, F):
    n_pair = H // 2
    nb = S // T
    offs = [sum(BLKS[:b]) for b in range(len(BLKS))]
    assert sum(BLKS) == S
    n_xc = S // XC
    qa, ka = M // WB, C // WB
    scale = (D ** -0.5) * LOG2E

    def kernel(x_hbm, ckv_hbm, wq_hbm, wk_hbm, wv_hbm, wo_hbm, wr_hbm, wg_hbm, wu_hbm, wd_hbm,
               out_hbm,
               x_s, xn_s, ckv_s, w_s, kv_s, ctx_s,
               wo_s, wr_s, wg_s, wu_s, wd_s, h_s, hn_s, out_s,
               sem_in, sem_x, sem_w, sem_kv, sem_big, sem_out, sem_fix, sem_reg):

        w_parts = {"q": (wq_hbm, 0, qa), "k": (wk_hbm, qa, ka), "v": (wv_hbm, qa + ka, ka)}

        def w_start(p, slot, parts, sem):
            for name in parts:
                hbm, r0, n = w_parts[name]
                for b in range(WB):
                    pltpu.make_async_copy(hbm.at[:, b, p], w_s.at[slot, pl.ds(r0, n), pl.ds(2 * b, 2), :],
                                          sem).start()

        def w_wait(slot, r0, n, sem):
            view = w_s.at[slot, pl.ds(r0, n)]
            pltpu.make_async_copy(view, view, sem).wait()

        def unpack(slot, name, e):
            _, r0, n = w_parts[name]
            w = pltpu.bitcast(w_s[slot, r0:r0 + n].reshape(n * 2 * WB, D), u32)
            if isinstance(e, int):
                w = (w << 16) if e == 0 else (w & jnp.uint32(0xFFFF0000))
            else:
                w = (w << (16 * (1 - e)).astype(u32)) & jnp.uint32(0xFFFF0000)
            return pltpu.bitcast(w, f32).astype(bf16)

        big_copies = [
            pltpu.make_async_copy(wo_hbm, wo_s.at[:, pl.ds(0, M)], sem_big.at[0]),
            pltpu.make_async_copy(wg_hbm, wg_s, sem_big.at[1]),
            pltpu.make_async_copy(wu_hbm, wu_s, sem_big.at[2]),
            pltpu.make_async_copy(wd_hbm, wd_s.at[:, pl.ds(0, M)], sem_big.at[3]),
            pltpu.make_async_copy(wr_hbm, wr_s, sem_big.at[4]),
        ]

        def x_copy(i):
            return pltpu.make_async_copy(x_hbm.at[pl.ds(i * XC, XC), :], x_s.at[pl.ds(i * XC, XC), :], sem_x.at[i])

        def ckv_copy(i):
            rows = pl.ds(CKV_SPLIT[i], CKV_SPLIT[i + 1] - CKV_SPLIT[i])
            return pltpu.make_async_copy(ckv_hbm.at[rows, :], ckv_s.at[rows, :], sem_in.at[i])

        def layernorm_x(c0, c1):
            toks = []
            for r0 in range(c0 * XC, c1 * XC, LP):
                xf = x_s[r0:r0 + LP, :].astype(f32)
                if len(toks) >= LCH:
                    xf = jnp.where(toks[-LCH] < 0.0, 0.0, xf)
                elif toks:
                    xf = jnp.where(mu * mu < 0.0, 0.0, xf)
                mu = jnp.sum(xf, axis=1, keepdims=True) * (1.0 / M)
                d = xf - mu
                var = jnp.sum(d * d, axis=1, keepdims=True) * (1.0 / M)
                rs = lax.rsqrt(var + EPS)
                y = d * rs
                toks.append(rs)
                xn_s[r0 // 2:(r0 + LP) // 2, :] = pltpu.bitcast(y.astype(bf16), u32)

        def kv_pre(pair, r0, r1):
            for j, name in enumerate("kv"):
                for e in range(2):
                    y = jnp.dot(ckv_s[r0:r1, :], unpack(pair, name, e), preferred_element_type=f32)
                    kv_s[2 * pair + e, j, r0 // 2:r1 // 2, :] = pltpu.bitcast(y.astype(bf16), u32)

        def pro_copy(kind, i, wait):
            if kind == "c":
                ckv_copy(i).wait() if wait else ckv_copy(i).start()
            elif kind == "x":
                x_copy(i).wait() if wait else x_copy(i).start()
            elif kind == "w":
                w_wait(i, qa, 2 * ka, sem_kv.at[i]) if wait else w_start(i, i, "kv", sem_kv.at[i])
            else:
                w_wait(i, 0, qa, sem_w.at[i]) if wait else w_start(i, i, "q", sem_w.at[i])

        with jax.named_scope("prologue"):
            for k, (kind, i) in enumerate(PRO_ORDER):
                if k and kind != PRO_ORDER[k - 1][0]:
                    pl.semaphore_signal(sem_reg, 1)
                    pl.semaphore_wait(sem_reg, 1)
                pro_copy(kind, i, False)
            for k, (waits, ln, work) in enumerate(PRO_STEPS):
                with jax.named_scope("w%d" % k):
                    for kind, i in waits:
                        pro_copy(kind, i, True)
                with jax.named_scope("r%d" % k):
                    layernorm_x(*ln)
                    for item in work:
                        kv_pre(*item)

        row = lax.broadcasted_iota(jnp.int32, (G, T), 0)
        col = lax.broadcasted_iota(jnp.int32, (G, T), 1)

        def head_step(h, have_kv):
            p = h >> 1
            slot = p & 1
            e = h & 1
            if not have_kv:
                @pl.when(e == 0)
                def _():
                    w_wait(slot, 0, qa + 2 * ka, sem_w.at[slot])

            tri = col <= row + (T - G)
            wq = unpack(slot, "q", e)
            if have_kv:
                @pl.when(h == 2)
                def _():
                    w_start(2, 0, "kqv", sem_w.at[0])
            else:
                wk = unpack(slot, "k", e)
                wv = unpack(slot, "v", e)

                @pl.when((e == 0) & (p + 1 < n_pair))
                def _():
                    w_start(jnp.minimum(p + 1, n_pair - 1), 1 - slot, "kqv", sem_w.at[1 - slot])

                for j in range(len(big_copies)):
                    @pl.when((e == 1) & (p == 2 * j + 2))
                    def _():
                        big_copies[j].start()

            def geom(blk):
                c, j = blk
                k0 = (c + 1) * G % T
                return k0, A * j + (0 if k0 else 1), [(A * j + a) * T + c * G for a in range(A)]

            def qproj(blk):
                xn = jnp.concatenate([xn_s[r // 2:(r + G) // 2, :] for r in geom(blk)[2]], axis=0)
                return jnp.dot(pltpu.bitcast(xn, bf16), wq, preferred_element_type=f32) * scale

            def qk(blk, qf):
                k0, n, _ = geom(blk)
                kk = kv[0]
                q = qf.astype(bf16)
                main = head = None
                if n:
                    main = lax.dot_general(q, kk[k0:k0 + n * T, :], NT, preferred_element_type=f32)
                if k0:
                    st = lax.dot_general(kk[0:k0, :], q, NT, preferred_element_type=f32)
                    head = jnp.concatenate([st, jnp.full((T - k0, T), NEG, f32)], axis=0).T
                extra = [lax.dot_general(qf[e * G:].astype(bf16), kk[k0 + (n + e - 1) * T:k0 + (n + e) * T, :], NT,
                                         preferred_element_type=f32) for e in range(1, A)]
                return main, head, extra

            def softmax_pv(blk, sc):
                k0, n, rows = geom(blk)
                vv = kv[1]
                main, head, extra = sc
                ps, rls = [], []
                for a in range(A):
                    parts = []
                    if n:
                        mm = main[a * G:(a + 1) * G]
                        if a == 0:
                            parts += [mm[:, :(n - 1) * T]] if n > 1 else []
                            parts.append(jnp.where(tri, mm[:, (n - 1) * T:], NEG))
                        else:
                            parts.append(mm)
                    if k0:
                        hd = head[a * G:(a + 1) * G]
                        parts.append(hd if n + a else jnp.where(col <= row + (k0 - G), hd, NEG))
                    for e in range(1, a + 1):
                        ex = extra[e - 1][(a - e) * G:(a - e + 1) * G]
                        parts.append(jnp.where(tri, ex, NEG) if e == a else ex)
                    s = jnp.concatenate(parts, axis=1) if len(parts) > 1 else parts[0]
                    pr = jnp.exp2(s - jnp.max(s, axis=1, keepdims=True))
                    rls.append(_recip(jnp.sum(_rnd(pr), axis=1, keepdims=True)))
                    ps.append(pr)
                w = ps[0].shape[1]
                vm = [vv[k0:k0 + n * T, :]] if n else []
                vm += [vv[0:T, :]] if k0 else []
                o = jnp.dot(jnp.concatenate([x[:, :w] for x in ps], axis=0).astype(bf16),
                            jnp.concatenate(vm, axis=0) if len(vm) > 1 else vm[0], preferred_element_type=f32)
                outs = [o[a * G:(a + 1) * G] for a in range(A)]
                for e in range(1, A):
                    pe = jnp.concatenate([x[:, w + (e - 1) * T:w + e * T] for x in ps[e:]], axis=0).astype(bf16)
                    oe = jnp.dot(pe, vv[k0 + (n + e - 1) * T:k0 + (n + e) * T, :], preferred_element_type=f32)
                    for a in range(e, A):
                        outs[a] = outs[a] + oe[(a - e) * G:(a - e + 1) * G]
                for a, r in enumerate(rows):
                    ctx_s[h, r // 2:(r + G) // 2, :] = pltpu.bitcast((outs[a] * rls[a]).astype(bf16), u32)

            order = [(c, j) for j in range(nb // A - 1, -1, -1) for c in range(A)]
            qs, ss = {}, {}

            def do_q(n):
                if n < nb:
                    qs[n] = qproj(order[n])

            def do_qk(n):
                if n < nb:
                    ss[n] = qk(order[n], qs.pop(n))

            if have_kv:
                kv = [pltpu.bitcast(kv_s[h, j], bf16) for j in range(2)]
            else:
                kv = [jnp.dot(ckv_s[...], wk, preferred_element_type=f32).astype(bf16)]
            for n in range(AHEAD + QAHEAD):
                do_q(n)
                if n >= QAHEAD:
                    do_qk(n - QAHEAD)
                if n == QAHEAD and not have_kv:
                    kv.append(jnp.dot(ckv_s[...], wv, preferred_element_type=f32).astype(bf16))
            for n in range(nb):
                do_q(n + AHEAD + QAHEAD)
                do_qk(n + AHEAD)
                softmax_pv(order[n], ss.pop(n))

        def first_body(h, carry):
            with jax.named_scope("first"):
                head_step(h, True)
            return carry

        def head_body(h, carry):
            with jax.named_scope("main"):
                head_step(h, False)
            return carry

        lax.fori_loop(0, 4, first_body, 0)
        lax.fori_loop(4, H, head_body, 0)

        for c in big_copies:
            c.wait()
        wr = wr_s[...].astype(f32).reshape(1, M)

        def out_copy(b):
            rows = pl.ds(offs[b], BLKS[b])
            return pltpu.make_async_copy(out_s.at[rows, :], out_hbm.at[rows, :], sem_out.at[b])

        def oproj(b):
            r0, r1 = offs[b] // 2, (offs[b] + BLKS[b]) // 2
            lhs = pltpu.bitcast(jnp.concatenate([ctx_s[j, r0:r1, :] for j in range(H)], axis=1), bf16)
            return jnp.dot(lhs, wo_s[:, 0:M], preferred_element_type=f32).astype(bf16)

        def post(b, attn, top, r):
            chain = b + 1 < len(BLKS)
            for n in range(BLKS[b] // PR):
                r0 = offs[b] + n * PR
                xf = x_s[r0:r0 + PR, :].astype(f32)
                if chain and r is not None:
                    xf = jnp.where(r * r < 0.0, 0.0, xf)
                h = (xf + attn[n * PR:(n + 1) * PR].astype(f32)).astype(bf16)
                hf = h.astype(f32)
                mu = jnp.sum(hf, axis=1, keepdims=True) * (1.0 / M)
                dc = hf - mu
                var = jnp.sum(dc * dc, axis=1, keepdims=True) * (1.0 / M)
                den = _rnd(jnp.sqrt(_rnd(_rnd(var) + _rnd(jnp.full((1, 1), EPS, f32)))))
                hn = (_rnd(hf - _rnd(mu)) * (1.0 / den)).astype(bf16)
                hnf = hn.astype(f32)
                h_s[r0:r0 + PR, :] = h
                hn_s[r0:r0 + PR, :] = hn
                out_s[r0:r0 + PR, :] = (hf + hnf).astype(bf16)
                r = _rnd(jnp.sum(hnf * wr, axis=1, keepdims=True))
                m1, i1, m2, i2 = top
                idx = r0 + slot_id
                g1, g2 = r > m1, r > m2
                top = (jnp.where(g1, r, m1), jnp.where(g1, idx, i1),
                       jnp.where(g1, m1, jnp.where(g2, r, m2)), jnp.where(g1, i1, jnp.where(g2, idx, i2)))
            out_copy(b).start()
            return top, r

        slot_id = lax.broadcasted_iota(jnp.int32, (PR, 1), 0)
        ninf = jnp.full((PR, 1), -jnp.inf, f32)
        top, r = (ninf, slot_id, ninf, slot_id + PR), None
        with jax.named_scope("tail"):
            attn = oproj(0)
            for b in range(len(BLKS)):
                nxt = oproj(b + 1) if b + 1 < len(BLKS) else None
                top, r = post(b, attn, top, r)
                attn = nxt

            val = jnp.concatenate([top[0], top[2]], axis=0)
            pos = jnp.concatenate([top[1], top[3]], axis=0).astype(f32)
            m1 = jnp.max(val, axis=0, keepdims=True)
            p1 = jnp.min(jnp.where(val == m1, pos, float(S)), axis=0, keepdims=True)
            rest = jnp.where(pos == p1, -jnp.inf, val)
            m2 = jnp.max(rest, axis=0, keepdims=True)
            p2 = jnp.min(jnp.where((rest == m2) & (pos != p1), pos, float(S)), axis=0, keepdims=True)
            i1 = jnp.clip(p1.astype(jnp.int32)[0, 0], 0, S - 1)
            i2 = jnp.clip(p2.astype(jnp.int32)[0, 0], 0, S - 1)

            g1 = pl.multiple_of((i1 // 16) * 16, 16)
            g2 = pl.multiple_of((i2 // 16) * 16, 16)
            xs = jnp.concatenate([hn_s[pl.ds(g1, 16), :].astype(f32), hn_s[pl.ds(g2, 16), :].astype(f32)], axis=0)
            hs = jnp.concatenate([h_s[pl.ds(g1, 16), :].astype(f32), h_s[pl.ds(g2, 16), :].astype(f32)], axis=0)
            xb = xs.astype(bf16)
            g = _rnd(jnp.dot(xb, wg_s[...], preferred_element_type=f32))
            u = _rnd(jnp.dot(xb, wu_s[...], preferred_element_type=f32))
            gu = (_rnd(g * jax.nn.sigmoid(g)) * u).astype(bf16)
            y = _rnd(jnp.dot(gu, wd_s[:, 0:M], preferred_element_type=f32))
            rid = lax.broadcasted_iota(jnp.int32, (32, 1), 0)
            tok = jnp.where(rid < 16, g1 + rid, g2 + rid - 16)
            rsel = jnp.where(tok == i1, m1, m2)
            upd = jnp.where((tok == i1) | (tok == i2), _rnd(y * _rnd(jax.nn.sigmoid(rsel))), 0.0)
            fixed = (hs + _rnd(xs + upd)).astype(bf16)

            for b in range(len(BLKS)):
                out_copy(b).wait()
            out_s[pl.ds(g1, 16), :] = fixed[0:16]
            out_s[pl.ds(g2, 16), :] = fixed[16:32]
            c1 = pltpu.make_async_copy(out_s.at[pl.ds(g1, 16), :], out_hbm.at[pl.ds(g1, 16), :], sem_fix.at[0])
            c2 = pltpu.make_async_copy(out_s.at[pl.ds(g2, 16), :], out_hbm.at[pl.ds(g2, 16), :], sem_fix.at[1])
            c1.start()

            @pl.when(g1 != g2)
            def _():
                c2.start()
                c2.wait()

            c1.wait()

    scratch = [
        pltpu.VMEM((S, M), bf16),
        pltpu.VMEM((S // 2, M), u32),
        pltpu.VMEM((S, C), bf16),
        pltpu.VMEM((2, qa + 2 * ka, 2 * WB, D), bf16),
        pltpu.VMEM((4, 2, S // 2, D), u32),
        pltpu.VMEM((H, S // 2, D), u32),
        pltpu.VMEM((H * D, M + WD_PAD), bf16),
        pltpu.VMEM((M,), bf16),
        pltpu.VMEM((M, F), bf16),
        pltpu.VMEM((M, F), bf16),
        pltpu.VMEM((F, M + WD_PAD), bf16),
        pltpu.VMEM((S, M), bf16),
        pltpu.VMEM((S, M), bf16),
        pltpu.VMEM((S, M), bf16),
        pltpu.SemaphoreType.DMA((len(CKV_SPLIT) - 1,)),
        pltpu.SemaphoreType.DMA((n_xc,)),
        pltpu.SemaphoreType.DMA((2,)),
        pltpu.SemaphoreType.DMA((2,)),
        pltpu.SemaphoreType.DMA((5,)),
        pltpu.SemaphoreType.DMA((len(BLKS),)),
        pltpu.SemaphoreType.DMA((2,)),
        pltpu.SemaphoreType.REGULAR,
    ]
    return kernel, scratch


@jax.jit
def pallas_sequential_preLN__compressed_kv_cla__moe_arch_mod__prompt_kernel(
    A_x: jax.Array,
    A_c_kv: jax.Array,
    A_w_q: jax.Array,
    A_w_uk: jax.Array,
    A_w_uv: jax.Array,
    A_w_o: jax.Array,
    B_x: jax.Array,
    B_w_r: jax.Array,
    B_w_gate: jax.Array,
    B_w_up: jax.Array,
    B_w_down: jax.Array,
):
    B, S, M = A_x.shape
    C = A_c_kv.shape[2]
    H, D = A_w_q.shape[1], A_w_q.shape[2]
    F = B_w_gate.shape[1]
    assert B == 1 and A_c_kv.shape[1] == S

    kernel, scratch = _make_kernel(S, M, C, H, D, F)
    any_spec = pl.BlockSpec(memory_space=pl.ANY)
    out = pl.pallas_call(
        kernel,
        in_specs=[any_spec] * 10,
        out_specs=any_spec,
        out_shape=jax.ShapeDtypeStruct((S, M), A_x.dtype),
        scratch_shapes=scratch,
        compiler_params=pltpu.CompilerParams(
            vmem_limit_bytes=120 * 1024 * 1024,
            disable_bounds_checks=True,
        ),
        name="mla_mod_block",
    )(
        A_x.reshape(S, M), A_c_kv.reshape(S, C),
        A_w_q.reshape(M // WB, WB, H // 2, 2, D),
        A_w_uk.reshape(C // WB, WB, H // 2, 2, D),
        A_w_uv.reshape(C // WB, WB, H // 2, 2, D),
        A_w_o.reshape(H * D, M), B_w_r, B_w_gate, B_w_up, B_w_down,
    )
    return out.reshape(B, S, M)
```

```python
import jax
import jax.numpy as jnp
from jax import lax
import jax.experimental.pallas as pl
import jax.experimental.pallas.tpu as pltpu

bf16 = jnp.bfloat16
f32 = jnp.float32
u32 = jnp.uint32

T = 128
G = 64
A = T // G
AHEAD = 3
QAHEAD = 2
WB = 4
BLKS = (256,) * 7 + (128, 64, 64)
PR = 16
LCH = 4
LP = 16
XC = 256
CKV_SPLIT = (0, 256, 768, 1408, 2048)
PRO_ORDER = ([("w", 0)] + [("c", i) for i in range(4)] + [("x", i) for i in range(3)] + [("w", 1)]
             + [("x", i) for i in range(3, 8)] + [("q", 0), ("q", 1)])
PRO_STEPS = [
    ([("w", 0), ("c", 0)], (0, 0), [(0, 0, 256)]),
    ([("c", 1)], (0, 0), [(0, 256, 768)]),
    ([("c", 2)], (0, 0), [(0, 768, 1408)]),
    ([("c", 3), ("x", 0), ("x", 1)], (0, 2), [(0, 1408, 2048)]),
    ([("w", 1), ("x", 2), ("x", 3)], (2, 4), [(1, 0, 704)]),
    ([("x", 4), ("x", 5)], (4, 6), [(1, 704, 1376)]),
    ([("x", 6), ("x", 7)], (6, 8), [(1, 1376, 2048)]),
    ([("q", 0), ("q", 1)], (0, 0), []),
]
WD_PAD = 128
EPS = 1e-5
NEG = -1e30
LOG2E = 1.4426950408889634
NT = (((1,), (1,)), ((), ()))


def _rnd(x):
    return x.astype(bf16).astype(f32)


def _recip(l):
    r = pl.reciprocal(l, approx=True)
    return r * (2.0 - l * r)


def _make_kernel(S, M, C, H, D, F):
    n_pair = H // 2
    nb = S // T
    offs = [sum(BLKS[:b]) for b in range(len(BLKS))]
    assert sum(BLKS) == S
    n_xc = S // XC
    qa, ka = M // WB, C // WB
    scale = (D ** -0.5) * LOG2E

    def kernel(x_hbm, ckv_hbm, wq_hbm, wk_hbm, wv_hbm, wo_hbm, wr_hbm, wg_hbm, wu_hbm, wd_hbm,
               out_hbm,
               x_s, xn_s, ckv_s, w_s, kv_s, ctx_s,
               wo_s, wr_s, wg_s, wu_s, wd_s, h_s, hn_s, out_s, fix_s,
               sem_in, sem_x, sem_w, sem_kv, sem_big, sem_out, sem_fix, sem_reg):

        w_parts = {"q": (wq_hbm, 0, qa), "k": (wk_hbm, qa, ka), "v": (wv_hbm, qa + ka, ka)}

        def w_start(p, slot, parts, sem):
            for name in parts:
                hbm, r0, n = w_parts[name]
                for b in range(WB):
                    pltpu.make_async_copy(hbm.at[:, b, p], w_s.at[slot, pl.ds(r0, n), pl.ds(2 * b, 2), :],
                                          sem).start()

        def w_wait(slot, r0, n, sem):
            view = w_s.at[slot, pl.ds(r0, n)]
            pltpu.make_async_copy(view, view, sem).wait()

        def unpack(slot, name, e):
            _, r0, n = w_parts[name]
            w = pltpu.bitcast(w_s[slot, r0:r0 + n].reshape(n * 2 * WB, D), u32)
            if isinstance(e, int):
                w = (w << 16) if e == 0 else (w & jnp.uint32(0xFFFF0000))
            else:
                w = (w << (16 * (1 - e)).astype(u32)) & jnp.uint32(0xFFFF0000)
            return pltpu.bitcast(w, f32).astype(bf16)

        big_copies = [
            pltpu.make_async_copy(wo_hbm, wo_s.at[:, pl.ds(0, M)], sem_big.at[0]),
            pltpu.make_async_copy(wg_hbm, wg_s, sem_big.at[1]),
            pltpu.make_async_copy(wu_hbm, wu_s, sem_big.at[2]),
            pltpu.make_async_copy(wd_hbm, wd_s.at[:, pl.ds(0, M)], sem_big.at[3]),
            pltpu.make_async_copy(wr_hbm, wr_s, sem_big.at[4]),
        ]

        def x_copy(i):
            return pltpu.make_async_copy(x_hbm.at[pl.ds(i * XC, XC), :], x_s.at[pl.ds(i * XC, XC), :], sem_x.at[i])

        def ckv_copy(i):
            rows = pl.ds(CKV_SPLIT[i], CKV_SPLIT[i + 1] - CKV_SPLIT[i])
            return pltpu.make_async_copy(ckv_hbm.at[rows, :], ckv_s.at[rows, :], sem_in.at[i])

        def layernorm_x(c0, c1):
            toks = []
            for r0 in range(c0 * XC, c1 * XC, LP):
                xf = x_s[r0:r0 + LP, :].astype(f32)
                if len(toks) >= LCH:
                    xf = jnp.where(toks[-LCH] < 0.0, 0.0, xf)
                elif toks:
                    xf = jnp.where(mu * mu < 0.0, 0.0, xf)
                mu = jnp.sum(xf, axis=1, keepdims=True) * (1.0 / M)
                d = xf - mu
                var = jnp.sum(d * d, axis=1, keepdims=True) * (1.0 / M)
                rs = lax.rsqrt(var + EPS)
                y = d * rs
                toks.append(rs)
                xn_s[r0 // 2:(r0 + LP) // 2, :] = pltpu.bitcast(y.astype(bf16), u32)

        def kv_pre(pair, r0, r1):
            for j, name in enumerate("kv"):
                for e in range(2):
                    y = jnp.dot(ckv_s[r0:r1, :], unpack(pair, name, e), preferred_element_type=f32)
                    kv_s[2 * pair + e, j, r0 // 2:r1 // 2, :] = pltpu.bitcast(y.astype(bf16), u32)

        def pro_copy(kind, i, wait):
            if kind == "c":
                ckv_copy(i).wait() if wait else ckv_copy(i).start()
            elif kind == "x":
                x_copy(i).wait() if wait else x_copy(i).start()
            elif kind == "w":
                w_wait(i, qa, 2 * ka, sem_kv.at[i]) if wait else w_start(i, i, "kv", sem_kv.at[i])
            else:
                w_wait(i, 0, qa, sem_w.at[i]) if wait else w_start(i, i, "q", sem_w.at[i])

        with jax.named_scope("prologue"):
            for k, (kind, i) in enumerate(PRO_ORDER):
                if k and kind != PRO_ORDER[k - 1][0]:
                    pl.semaphore_signal(sem_reg, 1)
                    pl.semaphore_wait(sem_reg, 1)
                pro_copy(kind, i, False)
            for k, (waits, ln, work) in enumerate(PRO_STEPS):
                with jax.named_scope("w%d" % k):
                    for kind, i in waits:
                        pro_copy(kind, i, True)
                with jax.named_scope("r%d" % k):
                    layernorm_x(*ln)
                    for item in work:
                        kv_pre(*item)

        row = lax.broadcasted_iota(jnp.int32, (G, T), 0)
        col = lax.broadcasted_iota(jnp.int32, (G, T), 1)

        def head_step(h, have_kv):
            p = h >> 1
            slot = p & 1
            e = h & 1
            if not have_kv:
                @pl.when(e == 0)
                def _():
                    w_wait(slot, 0, qa + 2 * ka, sem_w.at[slot])

            tri = col <= row + (T - G)
            wq = unpack(slot, "q", e)
            if have_kv:
                @pl.when(h == 2)
                def _():
                    w_start(2, 0, "kqv", sem_w.at[0])
            else:
                wk = unpack(slot, "k", e)
                wv = unpack(slot, "v", e)

                @pl.when((e == 0) & (p + 1 < n_pair))
                def _():
                    w_start(jnp.minimum(p + 1, n_pair - 1), 1 - slot, "kqv", sem_w.at[1 - slot])

                for j in range(len(big_copies)):
                    @pl.when((e == 1) & (p == 2 * j + 2))
                    def _():
                        big_copies[j].start()

            def geom(blk):
                c, j = blk
                k0 = (c + 1) * G % T
                return k0, A * j + (0 if k0 else 1), [(A * j + a) * T + c * G for a in range(A)]

            def qproj(blk):
                xn = jnp.concatenate([xn_s[r // 2:(r + G) // 2, :] for r in geom(blk)[2]], axis=0)
                return jnp.dot(pltpu.bitcast(xn, bf16), wq, preferred_element_type=f32) * scale

            def qk(blk, qf):
                k0, n, _ = geom(blk)
                kk = kv[0]
                q = qf.astype(bf16)
                main = head = None
                if n:
                    main = lax.dot_general(q, kk[k0:k0 + n * T, :], NT, preferred_element_type=f32)
                if k0:
                    st = lax.dot_general(kk[0:k0, :], q, NT, preferred_element_type=f32)
                    head = jnp.concatenate([st, jnp.full((T - k0, T), NEG, f32)], axis=0).T
                extra = [lax.dot_general(qf[e * G:].astype(bf16), kk[k0 + (n + e - 1) * T:k0 + (n + e) * T, :], NT,
                                         preferred_element_type=f32) for e in range(1, A)]
                return main, head, extra

            def softmax_pv(blk, sc):
                k0, n, rows = geom(blk)
                vv = kv[1]
                main, head, extra = sc
                ps, rls = [], []
                for a in range(A):
                    parts = []
                    if n:
                        mm = main[a * G:(a + 1) * G]
                        if a == 0:
                            parts += [mm[:, :(n - 1) * T]] if n > 1 else []
                            parts.append(jnp.where(tri, mm[:, (n - 1) * T:], NEG))
                        else:
                            parts.append(mm)
                    if k0:
                        hd = head[a * G:(a + 1) * G]
                        parts.append(hd if n + a else jnp.where(col <= row + (k0 - G), hd, NEG))
                    for e in range(1, a + 1):
                        ex = extra[e - 1][(a - e) * G:(a - e + 1) * G]
                        parts.append(jnp.where(tri, ex, NEG) if e == a else ex)
                    s = jnp.concatenate(parts, axis=1) if len(parts) > 1 else parts[0]
                    pr = jnp.exp2(s - jnp.max(s, axis=1, keepdims=True))
                    rls.append(_recip(jnp.sum(_rnd(pr), axis=1, keepdims=True)))
                    ps.append(pr)
                w = ps[0].shape[1]
                vm = [vv[k0:k0 + n * T, :]] if n else []
                vm += [vv[0:T, :]] if k0 else []
                o = jnp.dot(jnp.concatenate([x[:, :w] for x in ps], axis=0).astype(bf16),
                            jnp.concatenate(vm, axis=0) if len(vm) > 1 else vm[0], preferred_element_type=f32)
                outs = [o[a * G:(a + 1) * G] for a in range(A)]
                for e in range(1, A):
                    pe = jnp.concatenate([x[:, w + (e - 1) * T:w + e * T] for x in ps[e:]], axis=0).astype(bf16)
                    oe = jnp.dot(pe, vv[k0 + (n + e - 1) * T:k0 + (n + e) * T, :], preferred_element_type=f32)
                    for a in range(e, A):
                        outs[a] = outs[a] + oe[(a - e) * G:(a - e + 1) * G]
                for a, r in enumerate(rows):
                    ctx_s[h, r // 2:(r + G) // 2, :] = pltpu.bitcast((outs[a] * rls[a]).astype(bf16), u32)

            order = [(c, j) for j in range(nb // A - 1, -1, -1) for c in range(A)]
            qs, ss = {}, {}

            def do_q(n):
                if n < nb:
                    qs[n] = qproj(order[n])

            def do_qk(n):
                if n < nb:
                    ss[n] = qk(order[n], qs.pop(n))

            if have_kv:
                kv = [pltpu.bitcast(kv_s[h, j], bf16) for j in range(2)]
            else:
                kv = [jnp.dot(ckv_s[...], wk, preferred_element_type=f32).astype(bf16)]
            for n in range(AHEAD + QAHEAD):
                do_q(n)
                if n >= QAHEAD:
                    do_qk(n - QAHEAD)
                if n == QAHEAD and not have_kv:
                    kv.append(jnp.dot(ckv_s[...], wv, preferred_element_type=f32).astype(bf16))
            for n in range(nb):
                do_q(n + AHEAD + QAHEAD)
                do_qk(n + AHEAD)
                softmax_pv(order[n], ss.pop(n))

        def first_body(h, carry):
            with jax.named_scope("first"):
                head_step(h, True)
            return carry

        def head_body(h, carry):
            with jax.named_scope("main"):
                head_step(h, False)
            return carry

        lax.fori_loop(0, 4, first_body, 0)
        lax.fori_loop(4, H, head_body, 0)

        for c in big_copies:
            c.wait()
        wr = wr_s[...].astype(f32).reshape(1, M)

        def out_copy(b):
            rows = pl.ds(offs[b], BLKS[b])
            return pltpu.make_async_copy(out_s.at[rows, :], out_hbm.at[rows, :], sem_out.at[0])

        def oproj(b):
            r0, r1 = offs[b] // 2, (offs[b] + BLKS[b]) // 2
            lhs = pltpu.bitcast(jnp.concatenate([ctx_s[j, r0:r1, :] for j in range(H)], axis=1), bf16)
            return jnp.dot(lhs, wo_s[:, 0:M], preferred_element_type=f32).astype(bf16)

        def post(b, attn, top, r):
            chain = b + 1 < len(BLKS)
            for n in range(BLKS[b] // PR):
                r0 = offs[b] + n * PR
                xf = x_s[r0:r0 + PR, :].astype(f32)
                if chain and r is not None:
                    xf = jnp.where(r * r < 0.0, 0.0, xf)
                h = (xf + attn[n * PR:(n + 1) * PR].astype(f32)).astype(bf16)
                hf = h.astype(f32)
                mu = jnp.sum(hf, axis=1, keepdims=True) * (1.0 / M)
                dc = hf - mu
                var = jnp.sum(dc * dc, axis=1, keepdims=True) * (1.0 / M)
                den = _rnd(jnp.sqrt(_rnd(_rnd(var) + _rnd(jnp.full((1, 1), EPS, f32)))))
                hn = (_rnd(hf - _rnd(mu)) * (1.0 / den)).astype(bf16)
                hnf = hn.astype(f32)
                h_s[r0:r0 + PR, :] = h
                hn_s[r0:r0 + PR, :] = hn
                out_s[r0:r0 + PR, :] = (hf + hnf).astype(bf16)
                r = _rnd(jnp.sum(hnf * wr, axis=1, keepdims=True))
                m1, i1, m2, i2 = top
                idx = r0 + slot_id
                g1, g2 = r > m1, r > m2
                top = (jnp.where(g1, r, m1), jnp.where(g1, idx, i1),
                       jnp.where(g1, m1, jnp.where(g2, r, m2)), jnp.where(g1, i1, jnp.where(g2, idx, i2)))
            out_copy(b).start()
            return top, r

        slot_id = lax.broadcasted_iota(jnp.int32, (PR, 1), 0)
        ninf = jnp.full((PR, 1), -jnp.inf, f32)
        top, r = (ninf, slot_id, ninf, slot_id + PR), None
        with jax.named_scope("tail"):
            attn = oproj(0)
            for b in range(len(BLKS)):
                nxt = oproj(b + 1) if b + 1 < len(BLKS) else None
                top, r = post(b, attn, top, r)
                attn = nxt

            val = jnp.concatenate([top[0], top[2]], axis=0)
            pos = jnp.concatenate([top[1], top[3]], axis=0).astype(f32)
            m1 = jnp.max(val, axis=0, keepdims=True)
            p1 = jnp.min(jnp.where(val == m1, pos, float(S)), axis=0, keepdims=True)
            rest = jnp.where(pos == p1, -jnp.inf, val)
            m2 = jnp.max(rest, axis=0, keepdims=True)
            p2 = jnp.min(jnp.where((rest == m2) & (pos != p1), pos, float(S)), axis=0, keepdims=True)
            i1 = jnp.clip(p1.astype(jnp.int32)[0, 0], 0, S - 1)
            i2 = jnp.clip(p2.astype(jnp.int32)[0, 0], 0, S - 1)

            g1 = pl.multiple_of((i1 // 16) * 16, 16)
            g2 = pl.multiple_of((i2 // 16) * 16, 16)
            xs = jnp.concatenate([hn_s[pl.ds(g1, 16), :].astype(f32), hn_s[pl.ds(g2, 16), :].astype(f32)], axis=0)
            hs = jnp.concatenate([h_s[pl.ds(g1, 16), :].astype(f32), h_s[pl.ds(g2, 16), :].astype(f32)], axis=0)
            xb = xs.astype(bf16)
            g = _rnd(jnp.dot(xb, wg_s[...], preferred_element_type=f32))
            u = _rnd(jnp.dot(xb, wu_s[...], preferred_element_type=f32))
            gu = (_rnd(g * jax.nn.sigmoid(g)) * u).astype(bf16)
            y = _rnd(jnp.dot(gu, wd_s[:, 0:M], preferred_element_type=f32))
            rid = lax.broadcasted_iota(jnp.int32, (32, 1), 0)
            tok = jnp.where(rid < 16, g1 + rid, g2 + rid - 16)
            rsel = jnp.where(tok == i1, m1, m2)
            upd = jnp.where((tok == i1) | (tok == i2), _rnd(y * _rnd(jax.nn.sigmoid(rsel))), 0.0)
            fixed = (hs + _rnd(xs + upd)).astype(bf16)

            fix_s[...] = fixed
            pltpu.make_async_copy(out_s, out_hbm, sem_out.at[0]).wait()
            c1 = pltpu.make_async_copy(fix_s.at[pl.ds(0, 16), :], out_hbm.at[pl.ds(g1, 16), :], sem_fix.at[0])
            c2 = pltpu.make_async_copy(fix_s.at[pl.ds(16, 16), :], out_hbm.at[pl.ds(g2, 16), :], sem_fix.at[1])
            c1.start()

            @pl.when(g1 != g2)
            def _():
                c2.start()
                c2.wait()

            c1.wait()

    scratch = [
        pltpu.VMEM((S, M), bf16),
        pltpu.VMEM((S // 2, M), u32),
        pltpu.VMEM((S, C), bf16),
        pltpu.VMEM((2, qa + 2 * ka, 2 * WB, D), bf16),
        pltpu.VMEM((4, 2, S // 2, D), u32),
        pltpu.VMEM((H, S // 2, D), u32),
        pltpu.VMEM((H * D, M + WD_PAD), bf16),
        pltpu.VMEM((M,), bf16),
        pltpu.VMEM((M, F), bf16),
        pltpu.VMEM((M, F), bf16),
        pltpu.VMEM((F, M + WD_PAD), bf16),
        pltpu.VMEM((S, M), bf16),
        pltpu.VMEM((S, M), bf16),
        pltpu.VMEM((S, M), bf16),
        pltpu.VMEM((32, M), bf16),
        pltpu.SemaphoreType.DMA((len(CKV_SPLIT) - 1,)),
        pltpu.SemaphoreType.DMA((n_xc,)),
        pltpu.SemaphoreType.DMA((2,)),
        pltpu.SemaphoreType.DMA((2,)),
        pltpu.SemaphoreType.DMA((5,)),
        pltpu.SemaphoreType.DMA((1,)),
        pltpu.SemaphoreType.DMA((2,)),
        pltpu.SemaphoreType.REGULAR,
    ]
    return kernel, scratch


@jax.jit
def pallas_sequential_preLN__compressed_kv_cla__moe_arch_mod__prompt_kernel(
    A_x: jax.Array,
    A_c_kv: jax.Array,
    A_w_q: jax.Array,
    A_w_uk: jax.Array,
    A_w_uv: jax.Array,
    A_w_o: jax.Array,
    B_x: jax.Array,
    B_w_r: jax.Array,
    B_w_gate: jax.Array,
    B_w_up: jax.Array,
    B_w_down: jax.Array,
):
    B, S, M = A_x.shape
    C = A_c_kv.shape[2]
    H, D = A_w_q.shape[1], A_w_q.shape[2]
    F = B_w_gate.shape[1]
    assert B == 1 and A_c_kv.shape[1] == S

    kernel, scratch = _make_kernel(S, M, C, H, D, F)
    any_spec = pl.BlockSpec(memory_space=pl.ANY)
    out = pl.pallas_call(
        kernel,
        in_specs=[any_spec] * 10,
        out_specs=any_spec,
        out_shape=jax.ShapeDtypeStruct((S, M), A_x.dtype),
        scratch_shapes=scratch,
        compiler_params=pltpu.CompilerParams(
            vmem_limit_bytes=120 * 1024 * 1024,
            disable_bounds_checks=True,
            disable_semaphore_checks=True,
        ),
        name="mla_mod_block",
    )(
        A_x.reshape(S, M), A_c_kv.reshape(S, C),
        A_w_q.reshape(M // WB, WB, H // 2, 2, D),
        A_w_uk.reshape(C // WB, WB, H // 2, 2, D),
        A_w_uv.reshape(C // WB, WB, H // 2, 2, D),
        A_w_o.reshape(H * D, M), B_w_r, B_w_gate, B_w_up, B_w_down,
    )
    return out.reshape(B, S, M)
```

```python
import jax
import jax.numpy as jnp
from jax import lax
import jax.experimental.pallas as pl
import jax.experimental.pallas.tpu as pltpu

bf16 = jnp.bfloat16
f32 = jnp.float32
u32 = jnp.uint32

T = 128
G = 64
A = T // G
AHEAD = 3
QAHEAD = 2
WB = 4
RB = 192
TAIL = (64, 64)
PR = 16
LCH = 4
LP = 16
XC = 256
CKV_SPLIT = (0, 256, 768, 1344, 2048)
PRO_ORDER = ([("w", 0)] + [("c", i) for i in range(4)] + [("x", i) for i in range(3)] + [("w", 1)]
             + [("x", i) for i in range(3, 8)] + [("q", 0), ("q", 1)])
KR = 704
WD_PAD = 128
EPS = 1e-5
NEG = -1e30
LOG2E = 1.4426950408889634
NT = (((1,), (1,)), ((), ()))


def _rnd(x):
    return x.astype(bf16).astype(f32)


def _recip(l):
    r = pl.reciprocal(l, approx=True)
    return r * (2.0 - l * r)


def _make_kernel(S, M, C, H, D, F):
    n_pair = H // 2
    nb = S // T
    n_rb = (S - sum(TAIL)) // RB
    assert n_rb * RB + sum(TAIL) == S
    n_xc = S // XC
    qa, ka = M // WB, C // WB
    scale = (D ** -0.5) * LOG2E

    def kernel(*refs):
        def once(i, carry):
            kernel_body(*refs)
            return carry

        lax.fori_loop(0, pl.program_id(0) + 1, once, 0)

    def kernel_body(x_hbm, ckv_hbm, wq_hbm, wk_hbm, wv_hbm, wo_hbm, wr_hbm, wg_hbm, wu_hbm, wd_hbm,
               out_hbm,
               x_s, xn_s, ckv_s, w_s, kv_s, ctx_s,
               wo_s, wr_s, wg_s, wu_s, wd_s, attn_s, h_s, hn_s, out_s, fix_s,
               sem_in, sem_x, sem_w, sem_kv, sem_big, sem_out, sem_fix, sem_reg):

        w_parts = {"q": (wq_hbm, 0, qa), "k": (wk_hbm, qa, ka), "v": (wv_hbm, qa + ka, ka)}

        def w_start(p, slot, parts, sem):
            for name in parts:
                hbm, r0, n = w_parts[name]
                for b in range(WB):
                    pltpu.make_async_copy(hbm.at[:, b, p], w_s.at[slot, pl.ds(r0, n), pl.ds(2 * b, 2), :],
                                          sem).start()

        def w_wait(slot, r0, n, sem):
            view = w_s.at[slot, pl.ds(r0, n)]
            pltpu.make_async_copy(view, view, sem).wait()

        def unpack(slot, name, e):
            _, r0, n = w_parts[name]
            w = pltpu.bitcast(w_s[slot, r0:r0 + n].reshape(n * 2 * WB, D), u32)
            if isinstance(e, int):
                w = (w << 16) if e == 0 else (w & jnp.uint32(0xFFFF0000))
            else:
                w = (w << (16 * (1 - e)).astype(u32)) & jnp.uint32(0xFFFF0000)
            return pltpu.bitcast(w, f32).astype(bf16)

        big_copies = [
            pltpu.make_async_copy(wo_hbm, wo_s.at[:, pl.ds(0, M)], sem_big.at[0]),
            pltpu.make_async_copy(wg_hbm, wg_s, sem_big.at[1]),
            pltpu.make_async_copy(wu_hbm, wu_s, sem_big.at[2]),
            pltpu.make_async_copy(wd_hbm, wd_s.at[:, pl.ds(0, M)], sem_big.at[3]),
            pltpu.make_async_copy(wr_hbm, wr_s, sem_big.at[4]),
        ]

        def rows_at(r0, n, div=1, align=16):
            if isinstance(r0, int):
                return pl.ds(r0 // div, n // div)
            return pl.ds(pl.multiple_of(r0 // div, align // div), n // div)

        def x_copy(i):
            rows = rows_at(i * XC, XC)
            return pltpu.make_async_copy(x_hbm.at[rows, :], x_s.at[rows, :], sem_x.at[i])

        def ckv_copy(i):
            rows = pl.ds(CKV_SPLIT[i], CKV_SPLIT[i + 1] - CKV_SPLIT[i])
            return pltpu.make_async_copy(ckv_hbm.at[rows, :], ckv_s.at[rows, :], sem_in.at[i])

        def layernorm_x(row0, nrows):
            toks = []
            for n in range(nrows // LP):
                r0 = row0 + n * LP
                xf = x_s[rows_at(r0, LP), :].astype(f32)
                if len(toks) >= LCH:
                    xf = jnp.where(toks[-LCH] < 0.0, 0.0, xf)
                elif toks:
                    xf = jnp.where(mu * mu < 0.0, 0.0, xf)
                mu = jnp.sum(xf, axis=1, keepdims=True) * (1.0 / M)
                d = xf - mu
                var = jnp.sum(d * d, axis=1, keepdims=True) * (1.0 / M)
                rs = lax.rsqrt(var + EPS)
                toks.append(rs)
                xn_s[rows_at(r0, LP, 2), :] = pltpu.bitcast((d * rs).astype(bf16), u32)

        def kv_pre(pair, r0, n):
            lhs = ckv_s[rows_at(r0, n, 1, 64), :]
            for j, name in enumerate("kv"):
                for e in range(2):
                    y = jnp.dot(lhs, unpack(pair, name, e), preferred_element_type=f32)
                    kv_s[2 * pair + e, j, rows_at(r0, n, 2, 64), :] = pltpu.bitcast(y.astype(bf16), u32)

        with jax.named_scope("prologue"):
            for k, (kind, i) in enumerate(PRO_ORDER):
                if k and kind != PRO_ORDER[k - 1][0]:
                    pl.semaphore_signal(sem_reg, 1)
                    pl.semaphore_wait(sem_reg, 1)
                if kind == "c":
                    ckv_copy(i).start()
                elif kind == "x":
                    x_copy(i).start()
                elif kind == "w":
                    w_start(i, i, "kv", sem_kv.at[i])
                else:
                    w_start(i, i, "q", sem_w.at[i])
            attn_s[...] = jnp.zeros(attn_s.shape, u32)
            w_wait(0, qa, 2 * ka, sem_kv.at[0])
            for i in range(3):
                ckv_copy(i).wait()
                with jax.named_scope("r%d" % i):
                    kv_pre(0, CKV_SPLIT[i], CKV_SPLIT[i + 1] - CKV_SPLIT[i])
            ckv_copy(3).wait()

            def pro_body(t, carry):
                @pl.when(t == 1)
                def _():
                    w_wait(1, qa, 2 * ka, sem_kv.at[1])

                x_copy(2 * t).wait()
                x_copy(2 * t + 1).wait()
                with jax.named_scope("rl"):
                    layernorm_x(2 * t * XC, 2 * XC)
                    kv_pre(jnp.minimum(t, 1), jnp.where(t == 0, S - KR, jnp.minimum((t - 1) * KR, S - KR)), KR)
                return carry

            lax.fori_loop(0, 4, pro_body, 0)
            w_wait(0, 0, qa, sem_w.at[0])
            w_wait(1, 0, qa, sem_w.at[1])

        row = lax.broadcasted_iota(jnp.int32, (G, T), 0)
        col = lax.broadcasted_iota(jnp.int32, (G, T), 1)

        def head_step(h, have_kv):
            p = h >> 1
            slot = p & 1
            e = h & 1
            if not have_kv:
                @pl.when(e == 0)
                def _():
                    w_wait(slot, 0, qa + 2 * ka, sem_w.at[slot])

            tri = col <= row + (T - G)
            wq = unpack(slot, "q", e)
            if have_kv:
                @pl.when(h == 2)
                def _():
                    w_start(2, 0, "kqv", sem_w.at[0])
            else:
                wk = unpack(slot, "k", e)
                wv = unpack(slot, "v", e)

                @pl.when((e == 0) & (p + 1 < n_pair))
                def _():
                    w_start(jnp.minimum(p + 1, n_pair - 1), 1 - slot, "kqv", sem_w.at[1 - slot])

                for j in range(len(big_copies)):
                    @pl.when((e == 1) & (p == 2 * j + 2))
                    def _():
                        big_copies[j].start()

            def geom(blk):
                c, j = blk
                k0 = (c + 1) * G % T
                return k0, A * j + (0 if k0 else 1), [(A * j + a) * T + c * G for a in range(A)]

            def qproj(blk):
                xn = jnp.concatenate([xn_s[r // 2:(r + G) // 2, :] for r in geom(blk)[2]], axis=0)
                return jnp.dot(pltpu.bitcast(xn, bf16), wq, preferred_element_type=f32) * scale

            def qk(blk, qf):
                k0, n, _ = geom(blk)
                kk = kv[0]
                q = qf.astype(bf16)
                main = head = None
                if n:
                    main = lax.dot_general(q, kk[k0:k0 + n * T, :], NT, preferred_element_type=f32)
                if k0:
                    st = lax.dot_general(kk[0:k0, :], q, NT, preferred_element_type=f32)
                    head = jnp.concatenate([st, jnp.full((T - k0, T), NEG, f32)], axis=0).T
                extra = [lax.dot_general(qf[e * G:].astype(bf16), kk[k0 + (n + e - 1) * T:k0 + (n + e) * T, :], NT,
                                         preferred_element_type=f32) for e in range(1, A)]
                return main, head, extra

            def softmax_pv(blk, sc):
                k0, n, rows = geom(blk)
                vv = kv[1]
                main, head, extra = sc
                ps, rls = [], []
                for a in range(A):
                    parts = []
                    if n:
                        mm = main[a * G:(a + 1) * G]
                        if a == 0:
                            parts += [mm[:, :(n - 1) * T]] if n > 1 else []
                            parts.append(jnp.where(tri, mm[:, (n - 1) * T:], NEG))
                        else:
                            parts.append(mm)
                    if k0:
                        hd = head[a * G:(a + 1) * G]
                        parts.append(hd if n + a else jnp.where(col <= row + (k0 - G), hd, NEG))
                    for e in range(1, a + 1):
                        ex = extra[e - 1][(a - e) * G:(a - e + 1) * G]
                        parts.append(jnp.where(tri, ex, NEG) if e == a else ex)
                    s = jnp.concatenate(parts, axis=1) if len(parts) > 1 else parts[0]
                    pr = jnp.exp2(s - jnp.max(s, axis=1, keepdims=True))
                    rls.append(_recip(jnp.sum(_rnd(pr), axis=1, keepdims=True)))
                    ps.append(pr)
                w = ps[0].shape[1]
                vm = [vv[k0:k0 + n * T, :]] if n else []
                vm += [vv[0:T, :]] if k0 else []
                o = jnp.dot(jnp.concatenate([x[:, :w] for x in ps], axis=0).astype(bf16),
                            jnp.concatenate(vm, axis=0) if len(vm) > 1 else vm[0], preferred_element_type=f32)
                outs = [o[a * G:(a + 1) * G] for a in range(A)]
                for e in range(1, A):
                    pe = jnp.concatenate([x[:, w + (e - 1) * T:w + e * T] for x in ps[e:]], axis=0).astype(bf16)
                    oe = jnp.dot(pe, vv[k0 + (n + e - 1) * T:k0 + (n + e) * T, :], preferred_element_type=f32)
                    for a in range(e, A):
                        outs[a] = outs[a] + oe[(a - e) * G:(a - e + 1) * G]
                for a, r in enumerate(rows):
                    ctx_s[h, r // 2:(r + G) // 2, :] = pltpu.bitcast((outs[a] * rls[a]).astype(bf16), u32)

            order = [(c, j) for j in range(nb // A - 1, -1, -1) for c in range(A)]
            qs, ss = {}, {}

            def do_q(n):
                if n < nb:
                    qs[n] = qproj(order[n])

            def do_qk(n):
                if n < nb:
                    ss[n] = qk(order[n], qs.pop(n))

            if have_kv:
                kv = [pltpu.bitcast(kv_s[h, j], bf16) for j in range(2)]
            else:
                kv = [jnp.dot(ckv_s[...], wk, preferred_element_type=f32).astype(bf16)]
            for n in range(AHEAD + QAHEAD):
                do_q(n)
                if n >= QAHEAD:
                    do_qk(n - QAHEAD)
                if n == QAHEAD and not have_kv:
                    kv.append(jnp.dot(ckv_s[...], wv, preferred_element_type=f32).astype(bf16))
            for n in range(nb):
                do_q(n + AHEAD + QAHEAD)
                do_qk(n + AHEAD)
                softmax_pv(order[n], ss.pop(n))

        def first_body(h, carry):
            with jax.named_scope("first"):
                head_step(h, True)
            return carry

        def head_body(h, carry):
            with jax.named_scope("main"):
                head_step(h, False)
            return carry

        lax.fori_loop(0, 4, first_body, 0)
        lax.fori_loop(4, H, head_body, 0)

        for c in big_copies:
            c.wait()
        wr = wr_s[...].astype(f32).reshape(1, M)

        def out_start(r0, n):
            rows = rows_at(r0, n)
            pltpu.make_async_copy(out_s.at[rows, :], out_hbm.at[rows, :], sem_out.at[0]).start()

        def oproj(r0, n):
            lhs = jnp.concatenate([ctx_s[j, rows_at(r0, n, 2, 64), :] for j in range(H)], axis=1)
            o = jnp.dot(pltpu.bitcast(lhs, bf16), wo_s[:, 0:M], preferred_element_type=f32)
            return pltpu.bitcast(o.astype(bf16), u32)

        def post(row0, nrows, attn, top, r, chain=True, live=None):
            for n in range(nrows // PR):
                r0 = row0 + n * PR
                rows = rows_at(r0, PR)
                xf = x_s[rows, :].astype(f32)
                if chain and r is not None:
                    xf = jnp.where(r * r < 0.0, 0.0, xf)
                af = pltpu.bitcast(attn[n * PR // 2:(n + 1) * PR // 2, :], bf16).astype(f32)
                h = (xf + af).astype(bf16)
                hf = h.astype(f32)
                mu = jnp.sum(hf, axis=1, keepdims=True) * (1.0 / M)
                dc = hf - mu
                var = jnp.sum(dc * dc, axis=1, keepdims=True) * (1.0 / M)
                den = _rnd(jnp.sqrt(_rnd(_rnd(var) + _rnd(jnp.full((1, 1), EPS, f32)))))
                hn = (_rnd(hf - _rnd(mu)) * (1.0 / den)).astype(bf16)
                hnf = hn.astype(f32)
                h_s[rows, :] = h
                hn_s[rows, :] = hn
                out_s[rows, :] = (hf + hnf).astype(bf16)
                r = _rnd(jnp.sum(hnf * wr, axis=1, keepdims=True))
                m1, i1, m2, i2 = top
                idx = r0 + slot_id
                rr = r if live is None else jnp.where(live, r, -jnp.inf)
                g1, g2 = rr > m1, rr > m2
                top = (jnp.where(g1, r, m1), jnp.where(g1, idx, i1),
                       jnp.where(g1, m1, jnp.where(g2, r, m2)), jnp.where(g1, i1, jnp.where(g2, idx, i2)))
            return top, r

        slot_id = lax.broadcasted_iota(jnp.int32, (PR, 1), 0)
        ninf = jnp.full((PR, 1), -jnp.inf, f32)

        def oproj_body(b, top):
            with jax.named_scope("oloop"):
                prev = jnp.maximum(b - 1, 0) * RB
                top, _ = post(prev, RB, attn_s, top, None, live=b > 0)
                attn_s[...] = oproj(b * RB, RB)

                @pl.when(b > 0)
                def _():
                    out_start(prev, RB)
            return top

        top = lax.fori_loop(0, n_rb, oproj_body, (ninf, slot_id, ninf, slot_id + PR))
        with jax.named_scope("tail"):
            r0, n, attn, r = (n_rb - 1) * RB, RB, attn_s, None
            for nxt in TAIL + (0,):
                attn_next = oproj(r0 + n, nxt) if nxt else None
                top, r = post(r0, n, attn, top, r, chain=nxt > 0)
                out_start(r0, n)
                r0, n, attn = r0 + n, nxt, attn_next

            val = jnp.concatenate([top[0], top[2]], axis=0)
            pos = jnp.concatenate([top[1], top[3]], axis=0).astype(f32)
            m1 = jnp.max(val, axis=0, keepdims=True)
            p1 = jnp.min(jnp.where(val == m1, pos, float(S)), axis=0, keepdims=True)
            rest = jnp.where(pos == p1, -jnp.inf, val)
            m2 = jnp.max(rest, axis=0, keepdims=True)
            p2 = jnp.min(jnp.where((rest == m2) & (pos != p1), pos, float(S)), axis=0, keepdims=True)
            i1 = jnp.clip(p1.astype(jnp.int32)[0, 0], 0, S - 1)
            i2 = jnp.clip(p2.astype(jnp.int32)[0, 0], 0, S - 1)

            g1 = pl.multiple_of((i1 // 16) * 16, 16)
            g2 = pl.multiple_of((i2 // 16) * 16, 16)
            xs = jnp.concatenate([hn_s[pl.ds(g1, 16), :].astype(f32), hn_s[pl.ds(g2, 16), :].astype(f32)], axis=0)
            hs = jnp.concatenate([h_s[pl.ds(g1, 16), :].astype(f32), h_s[pl.ds(g2, 16), :].astype(f32)], axis=0)
            xb = xs.astype(bf16)
            g = _rnd(jnp.dot(xb, wg_s[...], preferred_element_type=f32))
            u = _rnd(jnp.dot(xb, wu_s[...], preferred_element_type=f32))
            gu = (_rnd(g * jax.nn.sigmoid(g)) * u).astype(bf16)
            y = _rnd(jnp.dot(gu, wd_s[:, 0:M], preferred_element_type=f32))
            rid = lax.broadcasted_iota(jnp.int32, (32, 1), 0)
            tok = jnp.where(rid < 16, g1 + rid, g2 + rid - 16)
            rsel = jnp.where(tok == i1, m1, m2)
            upd = jnp.where((tok == i1) | (tok == i2), _rnd(y * _rnd(jax.nn.sigmoid(rsel))), 0.0)
            fixed = (hs + _rnd(xs + upd)).astype(bf16)

            fix_s[...] = fixed
            pltpu.make_async_copy(out_s, out_hbm, sem_out.at[0]).wait()
            c1 = pltpu.make_async_copy(fix_s.at[pl.ds(0, 16), :], out_hbm.at[pl.ds(g1, 16), :], sem_fix.at[0])
            c2 = pltpu.make_async_copy(fix_s.at[pl.ds(16, 16), :], out_hbm.at[pl.ds(g2, 16), :], sem_fix.at[1])
            c1.start()

            @pl.when(g1 != g2)
            def _():
                c2.start()
                c2.wait()

            c1.wait()

    scratch = [
        pltpu.VMEM((S, M), bf16),
        pltpu.VMEM((S // 2, M), u32),
        pltpu.VMEM((S, C), bf16),
        pltpu.VMEM((2, qa + 2 * ka, 2 * WB, D), bf16),
        pltpu.VMEM((4, 2, S // 2, D), u32),
        pltpu.VMEM((H, S // 2, D), u32),
        pltpu.VMEM((H * D, M + WD_PAD), bf16),
        pltpu.VMEM((M,), bf16),
        pltpu.VMEM((M, F), bf16),
        pltpu.VMEM((M, F), bf16),
        pltpu.VMEM((F, M + WD_PAD), bf16),
        pltpu.VMEM((RB // 2, M), u32),
        pltpu.VMEM((S, M), bf16),
        pltpu.VMEM((S, M), bf16),
        pltpu.VMEM((S, M), bf16),
        pltpu.VMEM((32, M), bf16),
        pltpu.SemaphoreType.DMA((len(CKV_SPLIT) - 1,)),
        pltpu.SemaphoreType.DMA((n_xc,)),
        pltpu.SemaphoreType.DMA((2,)),
        pltpu.SemaphoreType.DMA((2,)),
        pltpu.SemaphoreType.DMA((5,)),
        pltpu.SemaphoreType.DMA((1,)),
        pltpu.SemaphoreType.DMA((2,)),
        pltpu.SemaphoreType.REGULAR,
    ]
    return kernel, scratch


@jax.jit
def pallas_sequential_preLN__compressed_kv_cla__moe_arch_mod__prompt_kernel(
    A_x: jax.Array,
    A_c_kv: jax.Array,
    A_w_q: jax.Array,
    A_w_uk: jax.Array,
    A_w_uv: jax.Array,
    A_w_o: jax.Array,
    B_x: jax.Array,
    B_w_r: jax.Array,
    B_w_gate: jax.Array,
    B_w_up: jax.Array,
    B_w_down: jax.Array,
):
    B, S, M = A_x.shape
    C = A_c_kv.shape[2]
    H, D = A_w_q.shape[1], A_w_q.shape[2]
    F = B_w_gate.shape[1]
    assert B == 1 and A_c_kv.shape[1] == S

    kernel, scratch = _make_kernel(S, M, C, H, D, F)
    any_spec = pl.BlockSpec(memory_space=pl.ANY)
    out = pl.pallas_call(
        kernel,
        grid=(1,),
        in_specs=[any_spec] * 10,
        out_specs=any_spec,
        out_shape=jax.ShapeDtypeStruct((S, M), A_x.dtype),
        scratch_shapes=scratch,
        compiler_params=pltpu.CompilerParams(
            vmem_limit_bytes=120 * 1024 * 1024,
            disable_bounds_checks=True,
            disable_semaphore_checks=True,
        ),
        name="mla_mod_block",
    )(
        A_x.reshape(S, M), A_c_kv.reshape(S, C),
        A_w_q.reshape(M // WB, WB, H // 2, 2, D),
        A_w_uk.reshape(C // WB, WB, H // 2, 2, D),
        A_w_uv.reshape(C // WB, WB, H // 2, 2, D),
        A_w_o.reshape(H * D, M), B_w_r, B_w_gate, B_w_up, B_w_down,
    )
    return out.reshape(B, S, M)
```

```python
import jax
import jax.numpy as jnp
from jax import lax
import jax.experimental.pallas as pl
import jax.experimental.pallas.tpu as pltpu

bf16 = jnp.bfloat16
f32 = jnp.float32
u32 = jnp.uint32

T = 128
G = 32
A = T // G
AQ = 8
AK = 0
AN = 99
AHEAD = 3
QAHEAD = 1
WB = 4
RB = 192
TAIL = (64, 64)
PR = 16
LCH = 4
LP = 16
XC = 256
CKV_SPLIT = (0, 256, 768, 1344, 2048)
PRO_ORDER = ([("w", 0)] + [("c", i) for i in range(4)] + [("x", i) for i in range(3)] + [("w", 1)]
             + [("x", i) for i in range(3, 8)] + [("w", 2), ("q", 0), ("q", 1), ("w", 3)])
KR = 704
UR, UPS = 256, 7
NQ, NKV, NP = 4, 8, 4
VFIRST = 0
WD_PAD = 128
EPS = 1e-5
NEG = -1e30
LOG2E = 1.4426950408889634
NT = (((1,), (1,)), ((), ()))


def _rnd(x):
    return x.astype(bf16).astype(f32)


def _recip(l):
    r = pl.reciprocal(l, approx=True)
    return r * (2.0 - l * r)


def _make_kernel(S, M, C, H, D, F):
    n_pair = H // 2
    nb = S // T
    n_rb = (S - sum(TAIL)) // RB
    assert n_rb * RB + sum(TAIL) == S
    n_xc = S // XC
    qa, ka = M // WB, C // WB
    upp = S // UR
    assert (n_pair - 2) * upp == n_pair * UPS
    scale = (D ** -0.5) * LOG2E

    def kernel(*refs):
        def once(i, carry):
            kernel_body(*refs)
            return carry

        lax.fori_loop(0, pl.program_id(0) + 1, once, 0)

    def kernel_body(x_hbm, ckv_hbm, wq_hbm, wk_hbm, wv_hbm, wo_hbm, wr_hbm, wg_hbm, wu_hbm, wd_hbm,
               out_hbm,
               x_s, xn_s, ckv_s, wq_s, wkv_s, k_s, v_s, ctx_s,
               wo_s, wr_s, wg_s, wu_s, wd_s, attn_s, h_s, hn_s, out_s, fix_s,
               sem_in, sem_x, sem_q, sem_kv, sem_big, sem_out, sem_fix, sem_reg):

        w_parts = {"q": (wq_hbm, wq_s, NQ, 0, qa), "k": (wk_hbm, wkv_s, NKV, 0, ka), "v": (wv_hbm, wkv_s, NKV, ka, ka)}

        def w_copy(p, names, sem, wait):
            _, buf, nslot, _, _ = w_parts[names[0]]
            slot = p % nslot if isinstance(p, int) else p & (nslot - 1)
            if wait:
                pltpu.make_async_copy(buf.at[slot], buf.at[slot], sem.at[slot]).wait()
                return
            for name in names:
                hbm, _, _, r0, n = w_parts[name]
                for b in range(WB):
                    pltpu.make_async_copy(hbm.at[:, b, p], buf.at[slot, pl.ds(r0, n), pl.ds(2 * b, 2), :],
                                          sem.at[slot]).start()

        def unpack(p, name):
            _, buf, nslot, r0, n = w_parts[name]
            slot = p % nslot if isinstance(p, int) else p & (nslot - 1)
            w = pltpu.bitcast(buf[slot, r0:r0 + n].reshape(n * 2 * WB, D), u32)
            return [pltpu.bitcast(x, f32).astype(bf16) for x in (w << 16, w & jnp.uint32(0xFFFF0000))]

        big_copies = [
            pltpu.make_async_copy(wo_hbm, wo_s.at[:, pl.ds(0, M)], sem_big.at[0]),
            pltpu.make_async_copy(wg_hbm, wg_s, sem_big.at[1]),
            pltpu.make_async_copy(wu_hbm, wu_s, sem_big.at[2]),
            pltpu.make_async_copy(wd_hbm, wd_s.at[:, pl.ds(0, M)], sem_big.at[3]),
            pltpu.make_async_copy(wr_hbm, wr_s, sem_big.at[4]),
        ]

        def rows_at(r0, n, div=1, align=16):
            if isinstance(r0, int):
                return pl.ds(r0 // div, n // div)
            return pl.ds(pl.multiple_of(r0 // div, align // div), n // div)

        def x_copy(i):
            rows = rows_at(i * XC, XC)
            return pltpu.make_async_copy(x_hbm.at[rows, :], x_s.at[rows, :], sem_x.at[i])

        def ckv_copy(i):
            rows = pl.ds(CKV_SPLIT[i], CKV_SPLIT[i + 1] - CKV_SPLIT[i])
            return pltpu.make_async_copy(ckv_hbm.at[rows, :], ckv_s.at[rows, :], sem_in.at[i])

        def layernorm_x(row0, nrows):
            toks = []
            for n in range(nrows // LP):
                r0 = row0 + n * LP
                xf = x_s[rows_at(r0, LP), :].astype(f32)
                if len(toks) >= LCH:
                    xf = jnp.where(toks[-LCH] < 0.0, 0.0, xf)
                elif toks:
                    xf = jnp.where(mu * mu < 0.0, 0.0, xf)
                mu = jnp.sum(xf, axis=1, keepdims=True) * (1.0 / M)
                d = xf - mu
                var = jnp.sum(d * d, axis=1, keepdims=True) * (1.0 / M)
                rs = lax.rsqrt(var + EPS)
                toks.append(rs)
                xn_s[rows_at(r0, LP, 2), :] = pltpu.bitcast((d * rs).astype(bf16), u32)

        def kv_proj(pair, r0, n, names):
            lhs = ckv_s[rows_at(r0, n, 1, 64), :]
            slot = pair % NP if isinstance(pair, int) else pair & (NP - 1)
            for name in names:
                for e, w in enumerate(unpack(pair, name)):
                    y = jnp.dot(lhs, w, preferred_element_type=f32)
                    dst = k_s if name == "k" else v_s
                    dst[2 * slot + e, rows_at(r0, n, 2, 64), :] = pltpu.bitcast(y.astype(bf16), u32)

        with jax.named_scope("prologue"):
            for k, (kind, i) in enumerate(PRO_ORDER):
                if k and kind != PRO_ORDER[k - 1][0]:
                    pl.semaphore_signal(sem_reg, 1)
                    pl.semaphore_wait(sem_reg, 1)
                if kind == "c":
                    ckv_copy(i).start()
                elif kind == "x":
                    x_copy(i).start()
                elif kind == "w":
                    w_copy(i, "kv", sem_kv, False)
                else:
                    w_copy(i, "q", sem_q, False)
            attn_s[...] = jnp.zeros(attn_s.shape, u32)
            w_copy(0, "kv", sem_kv, True)
            for i in range(3):
                ckv_copy(i).wait()
                with jax.named_scope("r%d" % i):
                    kv_proj(0, CKV_SPLIT[i], CKV_SPLIT[i + 1] - CKV_SPLIT[i], "kv")
            ckv_copy(3).wait()

            def pro_body(t, carry):
                @pl.when(t == 1)
                def _():
                    w_copy(1, "kv", sem_kv, True)

                x_copy(2 * t).wait()
                x_copy(2 * t + 1).wait()
                with jax.named_scope("rl"):
                    layernorm_x(2 * t * XC, 2 * XC)
                    kv_proj(jnp.minimum(t, 1), jnp.where(t == 0, S - KR, jnp.minimum((t - 1) * KR, S - KR)), KR, "kv")
                return carry

            lax.fori_loop(0, 4, pro_body, 0)

        row = lax.broadcasted_iota(jnp.int32, (G, T), 0)
        col = lax.broadcasted_iota(jnp.int32, (G, T), 1)

        def pair_step(p):
            w_copy(p, "q", sem_q, True)

            @pl.when(p + 2 < n_pair)
            def _():
                w_copy(p + 2, "kv", sem_kv, True)

            tri = col <= row + (T - G)

            def kv_units(name):
                for i in range(UPS):
                    u = p * UPS + i
                    kv_proj(2 + u // upp, (u % upp) * UR, UR, name)

            kv_units("k")
            if VFIRST:
                kv_units("v")
            wq2 = unpack(p, "q")

            hist = []

            def geom(blk):
                _, c, j = blk
                k0 = (c + 1) * G % T
                return k0, A * j + (0 if k0 else 1), [(A * j + a) * T + c * G for a in range(A)]

            def qproj(blk):
                xn = jnp.concatenate([xn_s[r // 2:(r + G) // 2, :] for r in geom(blk)[2]], axis=0)
                return jnp.dot(pltpu.bitcast(xn, bf16), wq2[blk[0]], preferred_element_type=f32) * scale

            def qk(blk, qf):
                k0, n, _ = geom(blk)
                kk = kv(k_s, blk[0])
                if AQ and len(hist) >= AQ and len(hist) - AQ < AN:
                    qf = jnp.where(jnp.concatenate(hist[-AQ], axis=0) < 0.0, 0.0, qf)
                q = qf.astype(bf16)
                main = head = None
                if n:
                    main = lax.dot_general(q, kk[k0:k0 + n * T, :], NT, preferred_element_type=f32)
                if k0:
                    st = lax.dot_general(kk[0:k0, :], q, NT, preferred_element_type=f32)
                    head = jnp.concatenate([st, jnp.full((T - k0, T), NEG, f32)], axis=0).T
                extra = [lax.dot_general(qf[e * G:].astype(bf16), kk[k0 + (n + e - 1) * T:k0 + (n + e) * T, :], NT,
                                         preferred_element_type=f32) for e in range(1, A)]
                return main, head, extra

            def softmax_pv(blk, sc):
                k0, n, rows = geom(blk)
                vv = kv(v_s, blk[0])
                main, head, extra = sc
                ps, rls = [], []
                for a in range(A):
                    parts = []
                    if n:
                        mm = main[a * G:(a + 1) * G]
                        if a == 0:
                            parts += [mm[:, :(n - 1) * T]] if n > 1 else []
                            parts.append(jnp.where(tri, mm[:, (n - 1) * T:], NEG))
                        else:
                            parts.append(mm)
                    if k0:
                        hd = head[a * G:(a + 1) * G]
                        parts.append(hd if n + a else jnp.where(col <= row + (k0 - G), hd, NEG))
                    for e in range(1, a + 1):
                        ex = extra[e - 1][(a - e) * G:(a - e + 1) * G]
                        parts.append(jnp.where(tri, ex, NEG) if e == a else ex)
                    s = jnp.concatenate(parts, axis=1) if len(parts) > 1 else parts[0]
                    mx = jnp.max(s, axis=1, keepdims=True)
                    if AK and len(hist) >= AK and len(hist) - AK < AN:
                        mx = jnp.where(hist[-AK][a] < 0.0, 0.0, mx)
                    pr = jnp.exp2(s - mx)
                    rls.append(_recip(jnp.sum(_rnd(pr), axis=1, keepdims=True)))
                    ps.append(pr)
                hist.append(rls)
                w = ps[0].shape[1]
                vm = [vv[k0:k0 + n * T, :]] if n else []
                vm += [vv[0:T, :]] if k0 else []
                o = jnp.dot(jnp.concatenate([x[:, :w] for x in ps], axis=0).astype(bf16),
                            jnp.concatenate(vm, axis=0) if len(vm) > 1 else vm[0], preferred_element_type=f32)
                outs = [o[a * G:(a + 1) * G] for a in range(A)]
                for e in range(1, A):
                    pe = jnp.concatenate([x[:, w + (e - 1) * T:w + e * T] for x in ps[e:]], axis=0).astype(bf16)
                    oe = jnp.dot(pe, vv[k0 + (n + e - 1) * T:k0 + (n + e) * T, :], preferred_element_type=f32)
                    for a in range(e, A):
                        outs[a] = outs[a] + oe[(a - e) * G:(a - e + 1) * G]
                for a, r in enumerate(rows):
                    ctx_s[2 * p + blk[0], r // 2:(r + G) // 2, :] = pltpu.bitcast((outs[a] * rls[a]).astype(bf16), u32)

            order = [(e, c, j) for e in range(2) for j in range(nb // A - 1, -1, -1) for c in range(A)]
            qs, ss, loaded = {}, {}, {}

            def kv(ref, e):
                if (id(ref), e) not in loaded:
                    loaded[id(ref), e] = pltpu.bitcast(ref[2 * (p & (NP - 1)) + e], bf16)
                return loaded[id(ref), e]

            def do_q(n):
                if n < len(order):
                    qs[n] = qproj(order[n])

            def do_qk(n):
                if n < len(order):
                    ss[n] = qk(order[n], qs.pop(n))

            for n in range(AHEAD + QAHEAD):
                do_q(n)
                if n >= QAHEAD:
                    do_qk(n - QAHEAD)
                if n == QAHEAD and not VFIRST:
                    kv_units("v")
            for n in range(len(order)):
                do_q(n + AHEAD + QAHEAD)
                do_qk(n + AHEAD)
                softmax_pv(order[n], ss.pop(n))

            @pl.when(p + 2 < n_pair)
            def _():
                w_copy(jnp.minimum(p + 2, n_pair - 1), "q", sem_q, False)

            @pl.when(p + 4 < n_pair)
            def _():
                w_copy(jnp.minimum(p + 4, n_pair - 1), "kv", sem_kv, False)

            for j in range(len(big_copies)):
                @pl.when(p == 2 * j + 1)
                def _():
                    big_copies[j].start()

        def pair_body(p, carry):
            with jax.named_scope("main"):
                pair_step(p)
            return carry

        lax.fori_loop(0, n_pair, pair_body, 0)

        for c in big_copies:
            c.wait()
        wr = wr_s[...].astype(f32).reshape(1, M)

        def out_start(r0, n):
            rows = rows_at(r0, n)
            pltpu.make_async_copy(out_s.at[rows, :], out_hbm.at[rows, :], sem_out.at[0]).start()

        def oproj(r0, n):
            lhs = jnp.concatenate([ctx_s[j, rows_at(r0, n, 2, 64), :] for j in range(H)], axis=1)
            o = jnp.dot(pltpu.bitcast(lhs, bf16), wo_s[:, 0:M], preferred_element_type=f32)
            return pltpu.bitcast(o.astype(bf16), u32)

        def post(row0, nrows, attn, top, r, chain=True, live=None):
            for n in range(nrows // PR):
                r0 = row0 + n * PR
                rows = rows_at(r0, PR)
                xf = x_s[rows, :].astype(f32)
                if chain and r is not None:
                    xf = jnp.where(r * r < 0.0, 0.0, xf)
                af = pltpu.bitcast(attn[n * PR // 2:(n + 1) * PR // 2, :], bf16).astype(f32)
                h = (xf + af).astype(bf16)
                hf = h.astype(f32)
                mu = jnp.sum(hf, axis=1, keepdims=True) * (1.0 / M)
                dc = hf - mu
                var = jnp.sum(dc * dc, axis=1, keepdims=True) * (1.0 / M)
                den = _rnd(jnp.sqrt(_rnd(_rnd(var) + _rnd(jnp.full((1, 1), EPS, f32)))))
                hn = (_rnd(hf - _rnd(mu)) * (1.0 / den)).astype(bf16)
                hnf = hn.astype(f32)
                h_s[rows, :] = h
                hn_s[rows, :] = hn
                out_s[rows, :] = (hf + hnf).astype(bf16)
                r = _rnd(jnp.sum(hnf * wr, axis=1, keepdims=True))
                m1, i1, m2, i2 = top
                idx = r0 + slot_id
                rr = r if live is None else jnp.where(live, r, -jnp.inf)
                g1, g2 = rr > m1, rr > m2
                top = (jnp.where(g1, r, m1), jnp.where(g1, idx, i1),
                       jnp.where(g1, m1, jnp.where(g2, r, m2)), jnp.where(g1, i1, jnp.where(g2, idx, i2)))
            return top, r

        slot_id = lax.broadcasted_iota(jnp.int32, (PR, 1), 0)
        ninf = jnp.full((PR, 1), -jnp.inf, f32)

        def oproj_body(b, top):
            with jax.named_scope("oloop"):
                prev = jnp.maximum(b - 1, 0) * RB
                top, _ = post(prev, RB, attn_s, top, None, live=b > 0)
                attn_s[...] = oproj(b * RB, RB)

                @pl.when(b > 0)
                def _():
                    out_start(prev, RB)
            return top

        top = lax.fori_loop(0, n_rb, oproj_body, (ninf, slot_id, ninf, slot_id + PR))
        with jax.named_scope("tail"):
            r0, n, attn, r = (n_rb - 1) * RB, RB, attn_s, None
            for nxt in TAIL + (0,):
                attn_next = oproj(r0 + n, nxt) if nxt else None
                top, r = post(r0, n, attn, top, r, chain=nxt > 0)
                out_start(r0, n)
                r0, n, attn = r0 + n, nxt, attn_next

            val = jnp.concatenate([top[0], top[2]], axis=0)
            pos = jnp.concatenate([top[1], top[3]], axis=0).astype(f32)
            m1 = jnp.max(val, axis=0, keepdims=True)
            p1 = jnp.min(jnp.where(val == m1, pos, float(S)), axis=0, keepdims=True)
            rest = jnp.where(pos == p1, -jnp.inf, val)
            m2 = jnp.max(rest, axis=0, keepdims=True)
            p2 = jnp.min(jnp.where((rest == m2) & (pos != p1), pos, float(S)), axis=0, keepdims=True)
            i1 = jnp.clip(p1.astype(jnp.int32)[0, 0], 0, S - 1)
            i2 = jnp.clip(p2.astype(jnp.int32)[0, 0], 0, S - 1)

            g1 = pl.multiple_of((i1 // 16) * 16, 16)
            g2 = pl.multiple_of((i2 // 16) * 16, 16)
            xs = jnp.concatenate([hn_s[pl.ds(g1, 16), :].astype(f32), hn_s[pl.ds(g2, 16), :].astype(f32)], axis=0)
            hs = jnp.concatenate([h_s[pl.ds(g1, 16), :].astype(f32), h_s[pl.ds(g2, 16), :].astype(f32)], axis=0)
            xb = xs.astype(bf16)
            g = _rnd(jnp.dot(xb, wg_s[...], preferred_element_type=f32))
            u = _rnd(jnp.dot(xb, wu_s[...], preferred_element_type=f32))
            gu = (_rnd(g * jax.nn.sigmoid(g)) * u).astype(bf16)
            y = _rnd(jnp.dot(gu, wd_s[:, 0:M], preferred_element_type=f32))
            rid = lax.broadcasted_iota(jnp.int32, (32, 1), 0)
            tok = jnp.where(rid < 16, g1 + rid, g2 + rid - 16)
            rsel = jnp.where(tok == i1, m1, m2)
            upd = jnp.where((tok == i1) | (tok == i2), _rnd(y * _rnd(jax.nn.sigmoid(rsel))), 0.0)
            fixed = (hs + _rnd(xs + upd)).astype(bf16)

            fix_s[...] = fixed
            pltpu.make_async_copy(out_s, out_hbm, sem_out.at[0]).wait()
            c1 = pltpu.make_async_copy(fix_s.at[pl.ds(0, 16), :], out_hbm.at[pl.ds(g1, 16), :], sem_fix.at[0])
            c2 = pltpu.make_async_copy(fix_s.at[pl.ds(16, 16), :], out_hbm.at[pl.ds(g2, 16), :], sem_fix.at[1])
            c1.start()

            @pl.when(g1 != g2)
            def _():
                c2.start()
                c2.wait()

            c1.wait()

    scratch = [
        pltpu.VMEM((S, M), bf16),
        pltpu.VMEM((S // 2, M), u32),
        pltpu.VMEM((S, C), bf16),
        pltpu.VMEM((NQ, qa, 2 * WB, D), bf16),
        pltpu.VMEM((NKV, 2 * ka, 2 * WB, D), bf16),
        pltpu.VMEM((2 * NP, S // 2, D), u32),
        pltpu.VMEM((2 * NP, S // 2, D), u32),
        pltpu.VMEM((H, S // 2, D), u32),
        pltpu.VMEM((H * D, M + WD_PAD), bf16),
        pltpu.VMEM((M,), bf16),
        pltpu.VMEM((M, F), bf16),
        pltpu.VMEM((M, F), bf16),
        pltpu.VMEM((F, M + WD_PAD), bf16),
        pltpu.VMEM((RB // 2, M), u32),
        pltpu.VMEM((S, M), bf16),
        pltpu.VMEM((S, M), bf16),
        pltpu.VMEM((S, M), bf16),
        pltpu.VMEM((32, M), bf16),
        pltpu.SemaphoreType.DMA((len(CKV_SPLIT) - 1,)),
        pltpu.SemaphoreType.DMA((n_xc,)),
        pltpu.SemaphoreType.DMA((NQ,)),
        pltpu.SemaphoreType.DMA((NKV,)),
        pltpu.SemaphoreType.DMA((5,)),
        pltpu.SemaphoreType.DMA((1,)),
        pltpu.SemaphoreType.DMA((2,)),
        pltpu.SemaphoreType.REGULAR,
    ]
    return kernel, scratch


@jax.jit
def pallas_sequential_preLN__compressed_kv_cla__moe_arch_mod__prompt_kernel(
    A_x: jax.Array,
    A_c_kv: jax.Array,
    A_w_q: jax.Array,
    A_w_uk: jax.Array,
    A_w_uv: jax.Array,
    A_w_o: jax.Array,
    B_x: jax.Array,
    B_w_r: jax.Array,
    B_w_gate: jax.Array,
    B_w_up: jax.Array,
    B_w_down: jax.Array,
):
    B, S, M = A_x.shape
    C = A_c_kv.shape[2]
    H, D = A_w_q.shape[1], A_w_q.shape[2]
    F = B_w_gate.shape[1]
    assert B == 1 and A_c_kv.shape[1] == S

    kernel, scratch = _make_kernel(S, M, C, H, D, F)
    any_spec = pl.BlockSpec(memory_space=pl.ANY)
    out = pl.pallas_call(
        kernel,
        grid=(1,),
        in_specs=[any_spec] * 10,
        out_specs=any_spec,
        out_shape=jax.ShapeDtypeStruct((S, M), A_x.dtype),
        scratch_shapes=scratch,
        compiler_params=pltpu.CompilerParams(
            vmem_limit_bytes=120 * 1024 * 1024,
            disable_bounds_checks=True,
            disable_semaphore_checks=True,
        ),
        name="mla_mod_block",
    )(
        A_x.reshape(S, M), A_c_kv.reshape(S, C),
        A_w_q.reshape(M // WB, WB, H // 2, 2, D),
        A_w_uk.reshape(C // WB, WB, H // 2, 2, D),
        A_w_uv.reshape(C // WB, WB, H // 2, 2, D),
        A_w_o.reshape(H * D, M), B_w_r, B_w_gate, B_w_up, B_w_down,
    )
    return out.reshape(B, S, M)
```

```python
import jax
import jax.numpy as jnp
from jax import lax
import jax.experimental.pallas as pl
import jax.experimental.pallas.tpu as pltpu

bf16 = jnp.bfloat16
f32 = jnp.float32
u32 = jnp.uint32

T = 128
G = 32
A = T // G
PERM = lambda n: [0, 1, 2, 4, 3, 5, 10, 7, 8, 16, 6, 11, 9, 17, 18, 19, 20, 22, 21, 24, 25, 26, 27, 28, 23, 12, 13, 29, 14, 30, 15, 31]
XA = 0
XN = 4
AQ = 8
AK = 0
AN = 99
AHEAD = 3
QAHEAD = 1
WB = 4
RB = 192
TAIL = (64, 64)
PR = 16
LCH = 4
LP = 16
XC = 256
CKV_SPLIT = (0, 256, 768, 1344, 2048)
PRO_ORDER = ([("w", 0)] + [("c", i) for i in range(4)] + [("x", i) for i in range(3)] + [("w", 1)]
             + [("x", i) for i in range(3, 8)] + [("w", 2), ("q", 0), ("q", 1), ("w", 3)])
KR = 704
UR, UPS = 256, 7
NQ, NKV, NP = 4, 8, 4
VFIRST = 0
WD_PAD = 128
EPS = 1e-5
NEG = -1e30
LOG2E = 1.4426950408889634
NT = (((1,), (1,)), ((), ()))


def _rnd(x):
    return x.astype(bf16).astype(f32)


def _recip(l):
    r = pl.reciprocal(l, approx=True)
    return r * (2.0 - l * r)


def _make_kernel(S, M, C, H, D, F):
    n_pair = H // 2
    nb = S // T
    n_rb = (S - sum(TAIL)) // RB
    assert n_rb * RB + sum(TAIL) == S
    n_xc = S // XC
    qa, ka = M // WB, C // WB
    upp = S // UR
    assert upp == 8 and (n_pair - 2) * upp == n_pair * UPS
    scale = (D ** -0.5) * LOG2E

    def kernel(*refs):
        def once(i, carry):
            kernel_body(*refs)
            return carry

        lax.fori_loop(0, pl.program_id(0) + 1, once, 0)

    def kernel_body(x_hbm, ckv_hbm, wq_hbm, wk_hbm, wv_hbm, wo_hbm, wr_hbm, wg_hbm, wu_hbm, wd_hbm,
               out_hbm,
               x_s, xn_s, ckv_s, wq_s, wkv_s, k_s, v_s, ctx_s,
               wo_s, wr_s, wg_s, wu_s, wd_s, attn_s, h_s, hn_s, out_s, fix_s,
               sem_in, sem_x, sem_q, sem_kv, sem_big, sem_out, sem_fix, sem_reg):

        w_parts = {"q": (wq_hbm, wq_s, NQ, 0, qa), "k": (wk_hbm, wkv_s, NKV, 0, ka), "v": (wv_hbm, wkv_s, NKV, ka, ka)}

        def w_copy(p, names, sem, wait):
            _, buf, nslot, _, _ = w_parts[names[0]]
            slot = p % nslot if isinstance(p, int) else p & (nslot - 1)
            if wait:
                pltpu.make_async_copy(buf.at[slot], buf.at[slot], sem.at[slot]).wait()
                return
            for name in names:
                hbm, _, _, r0, n = w_parts[name]
                for b in range(WB):
                    pltpu.make_async_copy(hbm.at[:, b, p], buf.at[slot, pl.ds(r0, n), pl.ds(2 * b, 2), :],
                                          sem.at[slot]).start()

        def unpack(p, name):
            _, buf, nslot, r0, n = w_parts[name]
            slot = p % nslot if isinstance(p, int) else p & (nslot - 1)
            w = pltpu.bitcast(buf[slot, r0:r0 + n].reshape(n * 2 * WB, D), u32)
            return [pltpu.bitcast(x, f32).astype(bf16) for x in (w << 16, w & jnp.uint32(0xFFFF0000))]

        big_copies = [
            pltpu.make_async_copy(wo_hbm, wo_s.at[:, pl.ds(0, M)], sem_big.at[0]),
            pltpu.make_async_copy(wg_hbm, wg_s, sem_big.at[1]),
            pltpu.make_async_copy(wu_hbm, wu_s, sem_big.at[2]),
            pltpu.make_async_copy(wd_hbm, wd_s.at[:, pl.ds(0, M)], sem_big.at[3]),
            pltpu.make_async_copy(wr_hbm, wr_s, sem_big.at[4]),
        ]

        def rows_at(r0, n, div=1, align=16):
            if isinstance(r0, int):
                return pl.ds(r0 // div, n // div)
            return pl.ds(pl.multiple_of(r0 >> (div - 1), align // div), n // div)

        def x_copy(i):
            rows = rows_at(i * XC, XC)
            return pltpu.make_async_copy(x_hbm.at[rows, :], x_s.at[rows, :], sem_x.at[i])

        def ckv_copy(i):
            rows = pl.ds(CKV_SPLIT[i], CKV_SPLIT[i + 1] - CKV_SPLIT[i])
            return pltpu.make_async_copy(ckv_hbm.at[rows, :], ckv_s.at[rows, :], sem_in.at[i])

        def layernorm_x(row0, nrows):
            toks = []
            for n in range(nrows // LP):
                r0 = row0 + n * LP
                xf = x_s[rows_at(r0, LP), :].astype(f32)
                if len(toks) >= LCH:
                    xf = jnp.where(toks[-LCH] < 0.0, 0.0, xf)
                elif toks:
                    xf = jnp.where(mu * mu < 0.0, 0.0, xf)
                mu = jnp.sum(xf, axis=1, keepdims=True) * (1.0 / M)
                d = xf - mu
                var = jnp.sum(d * d, axis=1, keepdims=True) * (1.0 / M)
                rs = lax.rsqrt(var + EPS)
                toks.append(rs)
                xn_s[rows_at(r0, LP, 2), :] = pltpu.bitcast((d * rs).astype(bf16), u32)

        def kv_proj(pair, r0, n, names):
            lhs = ckv_s[rows_at(r0, n, 1, 64), :]
            slot = pair % NP if isinstance(pair, int) else pair & (NP - 1)
            for name in names:
                for e, w in enumerate(unpack(pair, name)):
                    y = jnp.dot(lhs, w, preferred_element_type=f32)
                    dst = k_s if name == "k" else v_s
                    dst[2 * slot + e, rows_at(r0, n, 2, 64), :] = pltpu.bitcast(y.astype(bf16), u32)

        with jax.named_scope("prologue"):
            for k, (kind, i) in enumerate(PRO_ORDER):
                if k and kind != PRO_ORDER[k - 1][0]:
                    pl.semaphore_signal(sem_reg, 1)
                    pl.semaphore_wait(sem_reg, 1)
                if kind == "c":
                    ckv_copy(i).start()
                elif kind == "x":
                    x_copy(i).start()
                elif kind == "w":
                    w_copy(i, "kv", sem_kv, False)
                else:
                    w_copy(i, "q", sem_q, False)
            attn_s[...] = jnp.zeros(attn_s.shape, u32)
            w_copy(0, "kv", sem_kv, True)
            for i in range(3):
                ckv_copy(i).wait()
                with jax.named_scope("r%d" % i):
                    kv_proj(0, CKV_SPLIT[i], CKV_SPLIT[i + 1] - CKV_SPLIT[i], "kv")
            ckv_copy(3).wait()

            def pro_body(t, carry):
                @pl.when(t == 1)
                def _():
                    w_copy(1, "kv", sem_kv, True)

                x_copy(2 * t).wait()
                x_copy(2 * t + 1).wait()
                with jax.named_scope("rl"):
                    layernorm_x(2 * t * XC, 2 * XC)
                    kv_proj(jnp.minimum(t, 1), jnp.where(t == 0, S - KR, jnp.minimum((t - 1) * KR, S - KR)), KR, "kv")
                return carry

            lax.fori_loop(0, 4, pro_body, 0)

        row = lax.broadcasted_iota(jnp.int32, (G, T), 0)
        col = lax.broadcasted_iota(jnp.int32, (G, T), 1)

        def pair_step(p):
            w_copy(p, "q", sem_q, True)

            @pl.when(p + 2 < n_pair)
            def _():
                w_copy(p + 2, "kv", sem_kv, True)

            tri = col <= row + (T - G)

            def kv_units(name):
                for i in range(UPS):
                    u = p * UPS + i
                    kv_proj(2 + (u >> 3), (u & 7) * UR, UR, name)

            kv_units("k")
            if VFIRST:
                kv_units("v")
            wq2 = unpack(p, "q")

            hist = []

            def geom(blk):
                _, c, j = blk
                k0 = (c + 1) * G % T
                return k0, A * j + (0 if k0 else 1), [(A * j + a) * T + c * G for a in range(A)]

            def qproj(blk):
                xn = jnp.concatenate([xn_s[r // 2:(r + G) // 2, :] for r in geom(blk)[2]], axis=0)
                return jnp.dot(pltpu.bitcast(xn, bf16), wq2[blk[0]], preferred_element_type=f32) * scale

            def qk(blk, qf):
                k0, n, _ = geom(blk)
                kk = kv(k_s, blk[0])
                if AQ and len(hist) >= AQ and len(hist) - AQ < AN:
                    qf = jnp.where(jnp.concatenate(hist[-AQ], axis=0) < 0.0, 0.0, qf)
                q = qf.astype(bf16)
                main = head = None
                if n:
                    main = lax.dot_general(q, kk[k0:k0 + n * T, :], NT, preferred_element_type=f32)
                if k0:
                    st = lax.dot_general(kk[0:k0, :], q, NT, preferred_element_type=f32)
                    head = jnp.concatenate([st, jnp.full((T - k0, T), NEG, f32)], axis=0).T
                extra = [lax.dot_general(qf[e * G:].astype(bf16), kk[k0 + (n + e - 1) * T:k0 + (n + e) * T, :], NT,
                                         preferred_element_type=f32) for e in range(1, A)]
                return main, head, extra

            def softmax_pv(blk, sc):
                k0, n, rows = geom(blk)
                vv = kv(v_s, blk[0])
                main, head, extra = sc
                ps, rls = [], []
                for a in range(A):
                    parts = []
                    if n:
                        mm = main[a * G:(a + 1) * G]
                        if a == 0:
                            parts += [mm[:, :(n - 1) * T]] if n > 1 else []
                            parts.append(jnp.where(tri, mm[:, (n - 1) * T:], NEG))
                        else:
                            parts.append(mm)
                    if k0:
                        hd = head[a * G:(a + 1) * G]
                        parts.append(hd if n + a else jnp.where(col <= row + (k0 - G), hd, NEG))
                    for e in range(1, a + 1):
                        ex = extra[e - 1][(a - e) * G:(a - e + 1) * G]
                        parts.append(jnp.where(tri, ex, NEG) if e == a else ex)
                    s = jnp.concatenate(parts, axis=1) if len(parts) > 1 else parts[0]
                    mx = jnp.max(s, axis=1, keepdims=True)
                    if AK and len(hist) >= AK and len(hist) - AK < AN:
                        mx = jnp.where(hist[-AK][a] < 0.0, 0.0, mx)
                    pr = jnp.exp2(s - mx)
                    rls.append(_recip(jnp.sum(_rnd(pr), axis=1, keepdims=True)))
                    ps.append(pr)
                hist.append(rls)
                w = ps[0].shape[1]
                vm = [vv[k0:k0 + n * T, :]] if n else []
                vm += [vv[0:T, :]] if k0 else []
                o = jnp.dot(jnp.concatenate([x[:, :w] for x in ps], axis=0).astype(bf16),
                            jnp.concatenate(vm, axis=0) if len(vm) > 1 else vm[0], preferred_element_type=f32)
                outs = [o[a * G:(a + 1) * G] for a in range(A)]
                for e in range(1, A):
                    pe = jnp.concatenate([x[:, w + (e - 1) * T:w + e * T] for x in ps[e:]], axis=0).astype(bf16)
                    oe = jnp.dot(pe, vv[k0 + (n + e - 1) * T:k0 + (n + e) * T, :], preferred_element_type=f32)
                    for a in range(e, A):
                        outs[a] = outs[a] + oe[(a - e) * G:(a - e + 1) * G]
                for a, r in enumerate(rows):
                    ctx_s[2 * p + blk[0], r // 2:(r + G) // 2, :] = pltpu.bitcast((outs[a] * rls[a]).astype(bf16), u32)

            order = [(e, c, j) for e in range(2) for j in range(nb // A - 1, -1, -1) for c in range(A)]
            order = [order[k] for k in PERM(len(order))]
            qs, ss, loaded = {}, {}, {}

            def kv(ref, e):
                if (id(ref), e) not in loaded:
                    loaded[id(ref), e] = pltpu.bitcast(ref[2 * (p & (NP - 1)) + e], bf16)
                return loaded[id(ref), e]

            def do_q(n):
                if n < len(order):
                    qs[n] = qproj(order[n])

            def do_qk(n):
                if n < len(order):
                    ss[n] = qk(order[n], qs.pop(n))

            no = len(order)
            when = [max(n - AHEAD - (XA if n >= no - XN else 0), -1) for n in range(no)]
            nq = nk = 0
            for n in range(-1, no):
                while nk < no and when[nk] <= n:
                    while nq <= min(nk + QAHEAD, no - 1):
                        do_q(nq)
                        nq += 1
                    do_qk(nk)
                    if nk == 0 and not VFIRST:
                        kv_units("v")
                    nk += 1
                if n >= 0:
                    softmax_pv(order[n], ss.pop(n))

            @pl.when(p + 2 < n_pair)
            def _():
                w_copy(jnp.minimum(p + 2, n_pair - 1), "q", sem_q, False)

            @pl.when(p + 4 < n_pair)
            def _():
                w_copy(jnp.minimum(p + 4, n_pair - 1), "kv", sem_kv, False)

            for j in range(len(big_copies)):
                @pl.when(p == 2 * j + 1)
                def _():
                    big_copies[j].start()

        def pair_body(p, carry):
            with jax.named_scope("main"):
                pair_step(p)
            return carry

        lax.fori_loop(0, n_pair, pair_body, 0)

        for c in big_copies:
            c.wait()
        wr = wr_s[...].astype(f32).reshape(1, M)

        def out_start(r0, n):
            rows = rows_at(r0, n)
            pltpu.make_async_copy(out_s.at[rows, :], out_hbm.at[rows, :], sem_out.at[0]).start()

        def oproj(r0, n):
            lhs = jnp.concatenate([ctx_s[j, rows_at(r0, n, 2, 64), :] for j in range(H)], axis=1)
            o = jnp.dot(pltpu.bitcast(lhs, bf16), wo_s[:, 0:M], preferred_element_type=f32)
            return pltpu.bitcast(o.astype(bf16), u32)

        def post(row0, nrows, attn, top, r, chain=True, live=None):
            for n in range(nrows // PR):
                r0 = row0 + n * PR
                rows = rows_at(r0, PR)
                xf = x_s[rows, :].astype(f32)
                if chain and r is not None:
                    xf = jnp.where(r * r < 0.0, 0.0, xf)
                af = pltpu.bitcast(attn[n * PR // 2:(n + 1) * PR // 2, :], bf16).astype(f32)
                h = (xf + af).astype(bf16)
                hf = h.astype(f32)
                mu = jnp.sum(hf, axis=1, keepdims=True) * (1.0 / M)
                dc = hf - mu
                var = jnp.sum(dc * dc, axis=1, keepdims=True) * (1.0 / M)
                den = _rnd(jnp.sqrt(_rnd(_rnd(var) + _rnd(jnp.full((1, 1), EPS, f32)))))
                hn = (_rnd(hf - _rnd(mu)) * (1.0 / den)).astype(bf16)
                hnf = hn.astype(f32)
                h_s[rows, :] = h
                hn_s[rows, :] = hn
                out_s[rows, :] = (hf + hnf).astype(bf16)
                r = _rnd(jnp.sum(hnf * wr, axis=1, keepdims=True))
                m1, i1, m2, i2 = top
                idx = r0 + slot_id
                rr = r if live is None else jnp.where(live, r, -jnp.inf)
                g1, g2 = rr > m1, rr > m2
                top = (jnp.where(g1, r, m1), jnp.where(g1, idx, i1),
                       jnp.where(g1, m1, jnp.where(g2, r, m2)), jnp.where(g1, i1, jnp.where(g2, idx, i2)))
            return top, r

        slot_id = lax.broadcasted_iota(jnp.int32, (PR, 1), 0)
        ninf = jnp.full((PR, 1), -jnp.inf, f32)

        def oproj_body(b, top):
            with jax.named_scope("oloop"):
                prev = jnp.maximum(b - 1, 0) * RB
                top, _ = post(prev, RB, attn_s, top, None, live=b > 0)
                attn_s[...] = oproj(b * RB, RB)

                @pl.when(b > 0)
                def _():
                    out_start(prev, RB)
            return top

        top = lax.fori_loop(0, n_rb, oproj_body, (ninf, slot_id, ninf, slot_id + PR))
        with jax.named_scope("tail"):
            r0, n, attn, r = (n_rb - 1) * RB, RB, attn_s, None
            for nxt in TAIL + (0,):
                attn_next = oproj(r0 + n, nxt) if nxt else None
                top, r = post(r0, n, attn, top, r, chain=nxt > 0)
                out_start(r0, n)
                r0, n, attn = r0 + n, nxt, attn_next

            val = jnp.concatenate([top[0], top[2]], axis=0)
            pos = jnp.concatenate([top[1], top[3]], axis=0).astype(f32)
            m1 = jnp.max(val, axis=0, keepdims=True)
            p1 = jnp.min(jnp.where(val == m1, pos, float(S)), axis=0, keepdims=True)
            rest = jnp.where(pos == p1, -jnp.inf, val)
            m2 = jnp.max(rest, axis=0, keepdims=True)
            p2 = jnp.min(jnp.where((rest == m2) & (pos != p1), pos, float(S)), axis=0, keepdims=True)
            i1 = jnp.clip(p1.astype(jnp.int32)[0, 0], 0, S - 1)
            i2 = jnp.clip(p2.astype(jnp.int32)[0, 0], 0, S - 1)

            g1 = pl.multiple_of((i1 // 16) * 16, 16)
            g2 = pl.multiple_of((i2 // 16) * 16, 16)
            xs = jnp.concatenate([hn_s[pl.ds(g1, 16), :].astype(f32), hn_s[pl.ds(g2, 16), :].astype(f32)], axis=0)
            hs = jnp.concatenate([h_s[pl.ds(g1, 16), :].astype(f32), h_s[pl.ds(g2, 16), :].astype(f32)], axis=0)
            xb = xs.astype(bf16)
            g = _rnd(jnp.dot(xb, wg_s[...], preferred_element_type=f32))
            u = _rnd(jnp.dot(xb, wu_s[...], preferred_element_type=f32))
            gu = (_rnd(g * jax.nn.sigmoid(g)) * u).astype(bf16)
            y = _rnd(jnp.dot(gu, wd_s[:, 0:M], preferred_element_type=f32))
            rid = lax.broadcasted_iota(jnp.int32, (32, 1), 0)
            tok = jnp.where(rid < 16, g1 + rid, g2 + rid - 16)
            rsel = jnp.where(tok == i1, m1, m2)
            upd = jnp.where((tok == i1) | (tok == i2), _rnd(y * _rnd(jax.nn.sigmoid(rsel))), 0.0)
            fixed = (hs + _rnd(xs + upd)).astype(bf16)

            fix_s[...] = fixed
            pltpu.make_async_copy(out_s, out_hbm, sem_out.at[0]).wait()
            c1 = pltpu.make_async_copy(fix_s.at[pl.ds(0, 16), :], out_hbm.at[pl.ds(g1, 16), :], sem_fix.at[0])
            c2 = pltpu.make_async_copy(fix_s.at[pl.ds(16, 16), :], out_hbm.at[pl.ds(g2, 16), :], sem_fix.at[1])
            c1.start()

            @pl.when(g1 != g2)
            def _():
                c2.start()
                c2.wait()

            c1.wait()

    scratch = [
        pltpu.VMEM((S, M), bf16),
        pltpu.VMEM((S // 2, M), u32),
        pltpu.VMEM((S, C), bf16),
        pltpu.VMEM((NQ, qa, 2 * WB, D), bf16),
        pltpu.VMEM((NKV, 2 * ka, 2 * WB, D), bf16),
        pltpu.VMEM((2 * NP, S // 2, D), u32),
        pltpu.VMEM((2 * NP, S // 2, D), u32),
        pltpu.VMEM((H, S // 2, D), u32),
        pltpu.VMEM((H * D, M + WD_PAD), bf16),
        pltpu.VMEM((M,), bf16),
        pltpu.VMEM((M, F), bf16),
        pltpu.VMEM((M, F), bf16),
        pltpu.VMEM((F, M + WD_PAD), bf16),
        pltpu.VMEM((RB // 2, M), u32),
        pltpu.VMEM((S, M), bf16),
        pltpu.VMEM((S, M), bf16),
        pltpu.VMEM((S, M), bf16),
        pltpu.VMEM((32, M), bf16),
        pltpu.SemaphoreType.DMA((len(CKV_SPLIT) - 1,)),
        pltpu.SemaphoreType.DMA((n_xc,)),
        pltpu.SemaphoreType.DMA((NQ,)),
        pltpu.SemaphoreType.DMA((NKV,)),
        pltpu.SemaphoreType.DMA((5,)),
        pltpu.SemaphoreType.DMA((1,)),
        pltpu.SemaphoreType.DMA((2,)),
        pltpu.SemaphoreType.REGULAR,
    ]
    return kernel, scratch


@jax.jit
def pallas_sequential_preLN__compressed_kv_cla__moe_arch_mod__prompt_kernel(
    A_x: jax.Array,
    A_c_kv: jax.Array,
    A_w_q: jax.Array,
    A_w_uk: jax.Array,
    A_w_uv: jax.Array,
    A_w_o: jax.Array,
    B_x: jax.Array,
    B_w_r: jax.Array,
    B_w_gate: jax.Array,
    B_w_up: jax.Array,
    B_w_down: jax.Array,
):
    B, S, M = A_x.shape
    C = A_c_kv.shape[2]
    H, D = A_w_q.shape[1], A_w_q.shape[2]
    F = B_w_gate.shape[1]
    assert B == 1 and A_c_kv.shape[1] == S

    kernel, scratch = _make_kernel(S, M, C, H, D, F)
    any_spec = pl.BlockSpec(memory_space=pl.ANY)
    out = pl.pallas_call(
        kernel,
        grid=(1,),
        in_specs=[any_spec] * 10,
        out_specs=any_spec,
        out_shape=jax.ShapeDtypeStruct((S, M), A_x.dtype),
        scratch_shapes=scratch,
        compiler_params=pltpu.CompilerParams(
            vmem_limit_bytes=120 * 1024 * 1024,
            disable_bounds_checks=True,
            disable_semaphore_checks=True,
        ),
        name="mla_mod_block",
    )(
        A_x.reshape(S, M), A_c_kv.reshape(S, C),
        A_w_q.reshape(M // WB, WB, H // 2, 2, D),
        A_w_uk.reshape(C // WB, WB, H // 2, 2, D),
        A_w_uv.reshape(C // WB, WB, H // 2, 2, D),
        A_w_o.reshape(H * D, M), B_w_r, B_w_gate, B_w_up, B_w_down,
    )
    return out.reshape(B, S, M)
```

```python
import jax
import jax.numpy as jnp
from jax import lax
import jax.experimental.pallas as pl
import jax.experimental.pallas.tpu as pltpu

bf16 = jnp.bfloat16
f32 = jnp.float32
u32 = jnp.uint32

T = 128
G = 32
A = T // G
AHEAD = 3
QAHEAD = 1
AQ = 8
ORDER = (0, 1, 2, 4, 3, 5, 10, 7, 8, 16, 6, 11, 9, 17, 18, 19, 20, 22, 21, 24, 25, 26, 27, 28, 23, 12, 13, 29, 14, 30, 15, 31)
WB = 4
NQ, NKV, NP = 4, 8, 4
UR, UPS = 256, 7
RB = 192
TAIL = (64, 64)
PR = 16
LP, LCH = 16, 4
XC = 256
CKV_SPLIT = (0, 256, 768, 1344, 2048)
PRO_ORDER = ([("w", 0)] + [("c", i) for i in range(4)] + [("x", i) for i in range(3)] + [("w", 1)]
             + [("x", i) for i in range(3, 8)] + [("w", 2), ("q", 0), ("q", 1), ("w", 3)])
KR = 704
W_PAD = 128
EPS = 1e-5
NEG = -1e30
LOG2E = 1.4426950408889634
NT = (((1,), (1,)), ((), ()))


def _rnd(x):
    return x.astype(bf16).astype(f32)


def _recip(l):
    r = pl.reciprocal(l, approx=True)
    return r * (2.0 - l * r)


def _make_kernel(S, M, C, H, D, F):
    n_pair = H // 2
    nb = S // T
    n_rb = (S - sum(TAIL)) // RB
    assert n_rb * RB + sum(TAIL) == S
    n_xc = S // XC
    qa, ka = M // WB, C // WB
    upp = S // UR
    assert sorted(ORDER) == list(range(2 * nb)) and CKV_SPLIT[-1] == S and CKV_SPLIT[-2] == S - KR
    assert upp == 8 and (n_pair - 2) * upp == n_pair * UPS
    scale = (D ** -0.5) * LOG2E

    def kernel(*refs):
        def once(i, carry):
            kernel_body(*refs)
            return carry

        lax.fori_loop(0, pl.program_id(0) + 1, once, 0)

    def kernel_body(x_hbm, ckv_hbm, wq_hbm, wk_hbm, wv_hbm, wo_hbm, wr_hbm, wg_hbm, wu_hbm, wd_hbm,
                    out_hbm,
                    x_s, xn_s, ckv_s, wq_s, wkv_s, k_s, v_s, ctx_s,
                    wo_s, wr_s, wg_s, wu_s, wd_s, attn_s, h_s, hn_s, out_s, fix_s,
                    sem_in, sem_x, sem_q, sem_kv, sem_big, sem_out, sem_fix, sem_reg):

        w_parts = {"q": (wq_hbm, wq_s, NQ, 0, qa), "k": (wk_hbm, wkv_s, NKV, 0, ka), "v": (wv_hbm, wkv_s, NKV, ka, ka)}

        def w_copy(p, names, sem, wait):
            _, buf, nslot, _, _ = w_parts[names[0]]
            slot = p % nslot if isinstance(p, int) else p & (nslot - 1)
            if wait:
                pltpu.make_async_copy(buf.at[slot], buf.at[slot], sem.at[slot]).wait()
                return
            for name in names:
                hbm, _, _, r0, n = w_parts[name]
                for b in range(WB):
                    pltpu.make_async_copy(hbm.at[:, b, p], buf.at[slot, pl.ds(r0, n), pl.ds(2 * b, 2), :],
                                          sem.at[slot]).start()

        def unpack(p, name):
            _, buf, nslot, r0, n = w_parts[name]
            slot = p % nslot if isinstance(p, int) else p & (nslot - 1)
            w = pltpu.bitcast(buf[slot, r0:r0 + n].reshape(n * 2 * WB, D), u32)
            return [pltpu.bitcast(x, f32).astype(bf16) for x in (w << 16, w & jnp.uint32(0xFFFF0000))]

        big_copies = [
            pltpu.make_async_copy(wo_hbm, wo_s.at[:, pl.ds(0, M)], sem_big.at[0]),
            pltpu.make_async_copy(wg_hbm, wg_s, sem_big.at[1]),
            pltpu.make_async_copy(wu_hbm, wu_s, sem_big.at[2]),
            pltpu.make_async_copy(wd_hbm, wd_s.at[:, pl.ds(0, M)], sem_big.at[3]),
            pltpu.make_async_copy(wr_hbm, wr_s, sem_big.at[4]),
        ]

        def rows_at(r0, n, div=1, align=16):
            if isinstance(r0, int):
                return pl.ds(r0 // div, n // div)
            return pl.ds(pl.multiple_of(r0 >> (div - 1), align // div), n // div)

        def x_copy(i):
            rows = rows_at(i * XC, XC)
            return pltpu.make_async_copy(x_hbm.at[rows, :], x_s.at[rows, :], sem_x.at[i])

        def ckv_copy(i):
            rows = pl.ds(CKV_SPLIT[i], CKV_SPLIT[i + 1] - CKV_SPLIT[i])
            return pltpu.make_async_copy(ckv_hbm.at[rows, :], ckv_s.at[rows, :], sem_in.at[i])

        def layernorm_x(row0, nrows):
            toks = []
            for n in range(nrows // LP):
                r0 = row0 + n * LP
                xf = x_s[rows_at(r0, LP), :].astype(f32)
                if len(toks) >= LCH:
                    xf = jnp.where(toks[-LCH] < 0.0, 0.0, xf)
                elif toks:
                    xf = jnp.where(mu * mu < 0.0, 0.0, xf)
                mu = jnp.sum(xf, axis=1, keepdims=True) * (1.0 / M)
                d = xf - mu
                var = jnp.sum(d * d, axis=1, keepdims=True) * (1.0 / M)
                rs = lax.rsqrt(var + EPS)
                toks.append(rs)
                xn_s[rows_at(r0, LP, 2), :] = pltpu.bitcast((d * rs).astype(bf16), u32)

        def kv_proj(pair, r0, n, names):
            lhs = ckv_s[rows_at(r0, n, 1, 64), :]
            slot = pair % NP if isinstance(pair, int) else pair & (NP - 1)
            for name in names:
                for e, w in enumerate(unpack(pair, name)):
                    y = jnp.dot(lhs, w, preferred_element_type=f32)
                    dst = k_s if name == "k" else v_s
                    dst[2 * slot + e, rows_at(r0, n, 2, 64), :] = pltpu.bitcast(y.astype(bf16), u32)

        with jax.named_scope("prologue"):
            for k, (kind, i) in enumerate(PRO_ORDER):
                if k and kind != PRO_ORDER[k - 1][0]:
                    pl.semaphore_signal(sem_reg, 1)
                    pl.semaphore_wait(sem_reg, 1)
                if kind == "c":
                    ckv_copy(i).start()
                elif kind == "x":
                    x_copy(i).start()
                elif kind == "w":
                    w_copy(i, "kv", sem_kv, False)
                else:
                    w_copy(i, "q", sem_q, False)
            attn_s[...] = jnp.zeros(attn_s.shape, u32)
            w_copy(0, "kv", sem_kv, True)
            for i in range(3):
                ckv_copy(i).wait()
                with jax.named_scope("r%d" % i):
                    kv_proj(0, CKV_SPLIT[i], CKV_SPLIT[i + 1] - CKV_SPLIT[i], "kv")
            ckv_copy(3).wait()

            def pro_body(t, carry):
                @pl.when(t == 1)
                def _():
                    w_copy(1, "kv", sem_kv, True)

                x_copy(2 * t).wait()
                x_copy(2 * t + 1).wait()
                with jax.named_scope("rl"):
                    layernorm_x(2 * t * XC, 2 * XC)
                    kv_proj(jnp.minimum(t, 1), jnp.where(t == 0, S - KR, jnp.minimum((t - 1) * KR, S - KR)), KR, "kv")
                return carry

            lax.fori_loop(0, 4, pro_body, 0)

        row = lax.broadcasted_iota(jnp.int32, (G, T), 0)
        col = lax.broadcasted_iota(jnp.int32, (G, T), 1)

        def pair_step(p):
            w_copy(p, "q", sem_q, True)

            @pl.when(p + 2 < n_pair)
            def _():
                w_copy(p + 2, "kv", sem_kv, True)

            tri = col <= row + (T - G)

            def kv_units(name):
                for i in range(UPS):
                    u = p * UPS + i
                    kv_proj(2 + (u >> 3), (u & 7) * UR, UR, name)

            kv_units("k")
            wq2 = unpack(p, "q")

            hist = []

            def geom(blk):
                _, c, j = blk
                k0 = (c + 1) * G % T
                return k0, A * j + (0 if k0 else 1), [(A * j + a) * T + c * G for a in range(A)]

            def qproj(blk):
                xn = jnp.concatenate([xn_s[r // 2:(r + G) // 2, :] for r in geom(blk)[2]], axis=0)
                return jnp.dot(pltpu.bitcast(xn, bf16), wq2[blk[0]], preferred_element_type=f32) * scale

            def qk(blk, qf):
                k0, n, _ = geom(blk)
                kk = kv(k_s, blk[0])
                if len(hist) >= AQ:
                    qf = jnp.where(jnp.concatenate(hist[-AQ], axis=0) < 0.0, 0.0, qf)
                q = qf.astype(bf16)
                main = head = None
                if n:
                    main = lax.dot_general(q, kk[k0:k0 + n * T, :], NT, preferred_element_type=f32)
                if k0:
                    st = lax.dot_general(kk[0:k0, :], q, NT, preferred_element_type=f32)
                    head = jnp.concatenate([st, jnp.full((T - k0, T), NEG, f32)], axis=0).T
                extra = [lax.dot_general(qf[e * G:].astype(bf16), kk[k0 + (n + e - 1) * T:k0 + (n + e) * T, :], NT,
                                         preferred_element_type=f32) for e in range(1, A)]
                return main, head, extra

            def softmax_pv(blk, sc):
                k0, n, rows = geom(blk)
                vv = kv(v_s, blk[0])
                main, head, extra = sc
                ps, rls = [], []
                for a in range(A):
                    parts = []
                    if n:
                        mm = main[a * G:(a + 1) * G]
                        if a == 0:
                            parts += [mm[:, :(n - 1) * T]] if n > 1 else []
                            parts.append(jnp.where(tri, mm[:, (n - 1) * T:], NEG))
                        else:
                            parts.append(mm)
                    if k0:
                        hd = head[a * G:(a + 1) * G]
                        parts.append(hd if n + a else jnp.where(col <= row + (k0 - G), hd, NEG))
                    for e in range(1, a + 1):
                        ex = extra[e - 1][(a - e) * G:(a - e + 1) * G]
                        parts.append(jnp.where(tri, ex, NEG) if e == a else ex)
                    s = jnp.concatenate(parts, axis=1) if len(parts) > 1 else parts[0]
                    pr = jnp.exp2(s - jnp.max(s, axis=1, keepdims=True))
                    rls.append(_recip(jnp.sum(_rnd(pr), axis=1, keepdims=True)))
                    ps.append(pr)
                hist.append(rls)
                w = ps[0].shape[1]
                vm = [vv[k0:k0 + n * T, :]] if n else []
                vm += [vv[0:T, :]] if k0 else []
                o = jnp.dot(jnp.concatenate([x[:, :w] for x in ps], axis=0).astype(bf16),
                            jnp.concatenate(vm, axis=0) if len(vm) > 1 else vm[0], preferred_element_type=f32)
                outs = [o[a * G:(a + 1) * G] for a in range(A)]
                for e in range(1, A):
                    pe = jnp.concatenate([x[:, w + (e - 1) * T:w + e * T] for x in ps[e:]], axis=0).astype(bf16)
                    oe = jnp.dot(pe, vv[k0 + (n + e - 1) * T:k0 + (n + e) * T, :], preferred_element_type=f32)
                    for a in range(e, A):
                        outs[a] = outs[a] + oe[(a - e) * G:(a - e + 1) * G]
                for a, r in enumerate(rows):
                    ctx_s[2 * p + blk[0], r // 2:(r + G) // 2, :] = pltpu.bitcast((outs[a] * rls[a]).astype(bf16), u32)

            order = [(e, c, j) for e in range(2) for j in range(nb // A - 1, -1, -1) for c in range(A)]
            order = [order[k] for k in ORDER]
            qs, ss, loaded = {}, {}, {}

            def kv(ref, e):
                if (id(ref), e) not in loaded:
                    loaded[id(ref), e] = pltpu.bitcast(ref[2 * (p & (NP - 1)) + e], bf16)
                return loaded[id(ref), e]

            def do_q(n):
                if n < len(order):
                    qs[n] = qproj(order[n])

            def do_qk(n):
                if n < len(order):
                    ss[n] = qk(order[n], qs.pop(n))

            for n in range(AHEAD + QAHEAD):
                do_q(n)
                if n >= QAHEAD:
                    do_qk(n - QAHEAD)
                if n == QAHEAD:
                    kv_units("v")
            for n in range(len(order)):
                do_q(n + AHEAD + QAHEAD)
                do_qk(n + AHEAD)
                softmax_pv(order[n], ss.pop(n))

            @pl.when(p + 2 < n_pair)
            def _():
                w_copy(jnp.minimum(p + 2, n_pair - 1), "q", sem_q, False)

            @pl.when(p + 4 < n_pair)
            def _():
                w_copy(jnp.minimum(p + 4, n_pair - 1), "kv", sem_kv, False)

            for j in range(len(big_copies)):
                @pl.when(p == 2 * j + 1)
                def _():
                    big_copies[j].start()

        def pair_body(p, carry):
            with jax.named_scope("main"):
                pair_step(p)
            return carry

        lax.fori_loop(0, n_pair, pair_body, 0)

        for c in big_copies:
            c.wait()
        wr = wr_s[...].astype(f32).reshape(1, M)

        def out_start(r0, n):
            rows = rows_at(r0, n)
            pltpu.make_async_copy(out_s.at[rows, :], out_hbm.at[rows, :], sem_out.at[0]).start()

        def oproj(r0, n):
            lhs = jnp.concatenate([ctx_s[j, rows_at(r0, n, 2, 64), :] for j in range(H)], axis=1)
            o = jnp.dot(pltpu.bitcast(lhs, bf16), wo_s[:, 0:M], preferred_element_type=f32)
            return pltpu.bitcast(o.astype(bf16), u32)

        def post(row0, nrows, attn, top, r, chain=True, live=None):
            for n in range(nrows // PR):
                r0 = row0 + n * PR
                rows = rows_at(r0, PR)
                xf = x_s[rows, :].astype(f32)
                if chain and r is not None:
                    xf = jnp.where(r * r < 0.0, 0.0, xf)
                af = pltpu.bitcast(attn[n * PR // 2:(n + 1) * PR // 2, :], bf16).astype(f32)
                h = (xf + af).astype(bf16)
                hf = h.astype(f32)
                mu = jnp.sum(hf, axis=1, keepdims=True) * (1.0 / M)
                dc = hf - mu
                var = jnp.sum(dc * dc, axis=1, keepdims=True) * (1.0 / M)
                den = _rnd(jnp.sqrt(_rnd(_rnd(var) + _rnd(jnp.full((1, 1), EPS, f32)))))
                hn = (_rnd(hf - _rnd(mu)) * (1.0 / den)).astype(bf16)
                hnf = hn.astype(f32)
                h_s[rows, :] = h
                hn_s[rows, :] = hn
                out_s[rows, :] = (hf + hnf).astype(bf16)
                r = _rnd(jnp.sum(hnf * wr, axis=1, keepdims=True))
                m1, i1, m2, i2 = top
                idx = r0 + slot_id
                rr = r if live is None else jnp.where(live, r, -jnp.inf)
                g1, g2 = rr > m1, rr > m2
                top = (jnp.where(g1, r, m1), jnp.where(g1, idx, i1),
                       jnp.where(g1, m1, jnp.where(g2, r, m2)), jnp.where(g1, i1, jnp.where(g2, idx, i2)))
            return top, r

        slot_id = lax.broadcasted_iota(jnp.int32, (PR, 1), 0)
        ninf = jnp.full((PR, 1), -jnp.inf, f32)

        def oproj_body(b, top):
            with jax.named_scope("oloop"):
                prev = jnp.maximum(b - 1, 0) * RB
                top, _ = post(prev, RB, attn_s, top, None, live=b > 0)
                attn_s[...] = oproj(b * RB, RB)

                @pl.when(b > 0)
                def _():
                    out_start(prev, RB)
            return top

        top = lax.fori_loop(0, n_rb, oproj_body, (ninf, slot_id, ninf, slot_id + PR))
        with jax.named_scope("tail"):
            r0, n, attn, r = (n_rb - 1) * RB, RB, attn_s, None
            for nxt in TAIL + (0,):
                attn_next = oproj(r0 + n, nxt) if nxt else None
                top, r = post(r0, n, attn, top, r, chain=nxt > 0)
                out_start(r0, n)
                r0, n, attn = r0 + n, nxt, attn_next

            val = jnp.concatenate([top[0], top[2]], axis=0)
            pos = jnp.concatenate([top[1], top[3]], axis=0).astype(f32)
            m1 = jnp.max(val, axis=0, keepdims=True)
            p1 = jnp.min(jnp.where(val == m1, pos, float(S)), axis=0, keepdims=True)
            rest = jnp.where(pos == p1, -jnp.inf, val)
            m2 = jnp.max(rest, axis=0, keepdims=True)
            p2 = jnp.min(jnp.where((rest == m2) & (pos != p1), pos, float(S)), axis=0, keepdims=True)
            i1 = jnp.clip(p1.astype(jnp.int32)[0, 0], 0, S - 1)
            i2 = jnp.clip(p2.astype(jnp.int32)[0, 0], 0, S - 1)

            g1 = pl.multiple_of((i1 // 16) * 16, 16)
            g2 = pl.multiple_of((i2 // 16) * 16, 16)
            xs = jnp.concatenate([hn_s[pl.ds(g1, 16), :].astype(f32), hn_s[pl.ds(g2, 16), :].astype(f32)], axis=0)
            hs = jnp.concatenate([h_s[pl.ds(g1, 16), :].astype(f32), h_s[pl.ds(g2, 16), :].astype(f32)], axis=0)
            xb = xs.astype(bf16)
            g = _rnd(jnp.dot(xb, wg_s[...], preferred_element_type=f32))
            u = _rnd(jnp.dot(xb, wu_s[...], preferred_element_type=f32))
            gu = (_rnd(g * jax.nn.sigmoid(g)) * u).astype(bf16)
            y = _rnd(jnp.dot(gu, wd_s[:, 0:M], preferred_element_type=f32))
            rid = lax.broadcasted_iota(jnp.int32, (32, 1), 0)
            tok = jnp.where(rid < 16, g1 + rid, g2 + rid - 16)
            rsel = jnp.where(tok == i1, m1, m2)
            upd = jnp.where((tok == i1) | (tok == i2), _rnd(y * _rnd(jax.nn.sigmoid(rsel))), 0.0)
            fixed = (hs + _rnd(xs + upd)).astype(bf16)

            fix_s[...] = fixed
            pltpu.make_async_copy(out_s, out_hbm, sem_out.at[0]).wait()
            c1 = pltpu.make_async_copy(fix_s.at[pl.ds(0, 16), :], out_hbm.at[pl.ds(g1, 16), :], sem_fix.at[0])
            c2 = pltpu.make_async_copy(fix_s.at[pl.ds(16, 16), :], out_hbm.at[pl.ds(g2, 16), :], sem_fix.at[1])
            c1.start()

            @pl.when(g1 != g2)
            def _():
                c2.start()
                c2.wait()

            c1.wait()

    scratch = [
        pltpu.VMEM((S, M), bf16),
        pltpu.VMEM((S // 2, M), u32),
        pltpu.VMEM((S, C), bf16),
        pltpu.VMEM((NQ, qa, 2 * WB, D), bf16),
        pltpu.VMEM((NKV, 2 * ka, 2 * WB, D), bf16),
        pltpu.VMEM((2 * NP, S // 2, D), u32),
        pltpu.VMEM((2 * NP, S // 2, D), u32),
        pltpu.VMEM((H, S // 2, D), u32),
        pltpu.VMEM((H * D, M + W_PAD), bf16),
        pltpu.VMEM((M,), bf16),
        pltpu.VMEM((M, F), bf16),
        pltpu.VMEM((M, F), bf16),
        pltpu.VMEM((F, M + W_PAD), bf16),
        pltpu.VMEM((RB // 2, M), u32),
        pltpu.VMEM((S, M), bf16),
        pltpu.VMEM((S, M), bf16),
        pltpu.VMEM((S, M), bf16),
        pltpu.VMEM((32, M), bf16),
        pltpu.SemaphoreType.DMA((len(CKV_SPLIT) - 1,)),
        pltpu.SemaphoreType.DMA((n_xc,)),
        pltpu.SemaphoreType.DMA((NQ,)),
        pltpu.SemaphoreType.DMA((NKV,)),
        pltpu.SemaphoreType.DMA((5,)),
        pltpu.SemaphoreType.DMA((1,)),
        pltpu.SemaphoreType.DMA((2,)),
        pltpu.SemaphoreType.REGULAR,
    ]
    return kernel, scratch


@jax.jit
def pallas_sequential_preLN__compressed_kv_cla__moe_arch_mod__prompt_kernel(
    A_x: jax.Array,
    A_c_kv: jax.Array,
    A_w_q: jax.Array,
    A_w_uk: jax.Array,
    A_w_uv: jax.Array,
    A_w_o: jax.Array,
    B_x: jax.Array,
    B_w_r: jax.Array,
    B_w_gate: jax.Array,
    B_w_up: jax.Array,
    B_w_down: jax.Array,
):
    B, S, M = A_x.shape
    C = A_c_kv.shape[2]
    H, D = A_w_q.shape[1], A_w_q.shape[2]
    F = B_w_gate.shape[1]
    assert B == 1 and A_c_kv.shape[1] == S

    kernel, scratch = _make_kernel(S, M, C, H, D, F)
    any_spec = pl.BlockSpec(memory_space=pl.ANY)
    out = pl.pallas_call(
        kernel,
        grid=(1,),
        in_specs=[any_spec] * 10,
        out_specs=any_spec,
        out_shape=jax.ShapeDtypeStruct((S, M), A_x.dtype),
        scratch_shapes=scratch,
        compiler_params=pltpu.CompilerParams(
            vmem_limit_bytes=120 * 1024 * 1024,
            disable_bounds_checks=True,
            disable_semaphore_checks=True,
        ),
        name="mla_mod_block",
    )(
        A_x.reshape(S, M), A_c_kv.reshape(S, C),
        A_w_q.reshape(M // WB, WB, H // 2, 2, D),
        A_w_uk.reshape(C // WB, WB, H // 2, 2, D),
        A_w_uv.reshape(C // WB, WB, H // 2, 2, D),
        A_w_o.reshape(H * D, M), B_w_r, B_w_gate, B_w_up, B_w_down,
    )
    return out.reshape(B, S, M)
```

```python
import jax
import jax.numpy as jnp
from jax import lax
import jax.experimental.pallas as pl
import jax.experimental.pallas.tpu as pltpu

bf16 = jnp.bfloat16
f32 = jnp.float32
u32 = jnp.uint32

T = 128
G = 32
A = T // G
AHEAD = 3
QAHEAD = 1
AQ = 8
ORDER = (0, 1, 2, 4, 3, 5, 10, 7, 8, 16, 6, 11, 9, 17, 18, 19, 20, 22, 21, 24, 25, 26, 27, 28, 23, 12, 13, 29, 14, 30, 15, 31)
WB = 4
NQ, NKV, NP = 4, 8, 4
UR, UPS = 256, 7
RB = 192
U = 64
FG = 8
KC = 512
LEAD, NLEFT = 51, 11
DL, AC = 2, 4
FC = 896
PR = 16
LP, LCH = 16, 4
XC = 256
CKV_SPLIT = (0, 256, 768, 1344, 2048)
PRO_ORDER = ([("w", 0)] + [("c", i) for i in range(4)] + [("x", i) for i in range(3)] + [("w", 1)]
             + [("x", i) for i in range(3, 8)] + [("w", 2), ("q", 0), ("q", 1), ("w", 3)])
KR = 704
W_PAD = 128
EPS = 1e-5
NEG = -1e30
LOG2E = 1.4426950408889634
NT = (((1,), (1,)), ((), ()))


def _rnd(x):
    return x.astype(bf16).astype(f32)


def _recip(l):
    r = pl.reciprocal(l, approx=True)
    return r * (2.0 - l * r)


def _make_kernel(S, M, C, H, D, F):
    n_pair = H // 2
    nb = S // T
    n_rb = (S - 2 * U) // RB
    assert n_rb * RB + 2 * U == S and RB == 3 * U
    n_xc = S // XC
    qa, ka = M // WB, C // WB
    upp = S // UR
    assert sorted(ORDER) == list(range(2 * nb)) and CKV_SPLIT[-1] == S and CKV_SPLIT[-2] == S - KR
    assert upp == 8 and (n_pair - 2) * upp == n_pair * UPS
    scale = (D ** -0.5) * LOG2E

    def kernel(*refs):
        def once(i, carry):
            kernel_body(*refs)
            return carry

        lax.fori_loop(0, pl.program_id(0) + 1, once, 0)

    def kernel_body(x_hbm, ckv_hbm, wq_hbm, wk_hbm, wv_hbm, wo_hbm, wr_hbm, wg_hbm, wu_hbm, wd_hbm,
                    out_hbm,
                    x_s, xn_s, ckv_s, wq_s, wkv_s, k_s, v_s, ctx_s,
                    wo_s, wr_s, wg_s, wu_s, wd_s, attn_s, h_s, hn_s, out_s, fix_s, unit_s,
                    sem_in, sem_x, sem_q, sem_kv, sem_big, sem_out, sem_fix, sem_reg):

        w_parts = {"q": (wq_hbm, wq_s, NQ, 0, qa), "k": (wk_hbm, wkv_s, NKV, 0, ka), "v": (wv_hbm, wkv_s, NKV, ka, ka)}

        def w_copy(p, names, sem, wait):
            _, buf, nslot, _, _ = w_parts[names[0]]
            slot = p % nslot if isinstance(p, int) else p & (nslot - 1)
            if wait:
                pltpu.make_async_copy(buf.at[slot], buf.at[slot], sem.at[slot]).wait()
                return
            for name in names:
                hbm, _, _, r0, n = w_parts[name]
                for b in range(WB):
                    pltpu.make_async_copy(hbm.at[:, b, p], buf.at[slot, pl.ds(r0, n), pl.ds(2 * b, 2), :],
                                          sem.at[slot]).start()

        def unpack(p, name):
            _, buf, nslot, r0, n = w_parts[name]
            slot = p % nslot if isinstance(p, int) else p & (nslot - 1)
            w = pltpu.bitcast(buf[slot, r0:r0 + n].reshape(n * 2 * WB, D), u32)
            return [pltpu.bitcast(x, f32).astype(bf16) for x in (w << 16, w & jnp.uint32(0xFFFF0000))]

        big_copies = [
            pltpu.make_async_copy(wo_hbm, wo_s.at[:, pl.ds(0, M)], sem_big.at[0]),
            pltpu.make_async_copy(wg_hbm, wg_s, sem_big.at[1]),
            pltpu.make_async_copy(wu_hbm, wu_s, sem_big.at[2]),
            pltpu.make_async_copy(wd_hbm, wd_s.at[:, pl.ds(0, M)], sem_big.at[3]),
            pltpu.make_async_copy(wr_hbm, wr_s, sem_big.at[4]),
        ]

        def rows_at(r0, n, div=1, align=16):
            if isinstance(r0, int):
                return pl.ds(r0 // div, n // div)
            return pl.ds(pl.multiple_of(r0 >> (div - 1), align // div), n // div)

        def x_copy(i):
            rows = rows_at(i * XC, XC)
            return pltpu.make_async_copy(x_hbm.at[rows, :], x_s.at[rows, :], sem_x.at[i])

        def ckv_copy(i):
            rows = pl.ds(CKV_SPLIT[i], CKV_SPLIT[i + 1] - CKV_SPLIT[i])
            return pltpu.make_async_copy(ckv_hbm.at[rows, :], ckv_s.at[rows, :], sem_in.at[i])

        def layernorm_x(row0, nrows):
            toks = []
            for n in range(nrows // LP):
                r0 = row0 + n * LP
                xf = x_s[rows_at(r0, LP), :].astype(f32)
                if len(toks) >= LCH:
                    xf = jnp.where(toks[-LCH] < 0.0, 0.0, xf)
                elif toks:
                    xf = jnp.where(mu * mu < 0.0, 0.0, xf)
                mu = jnp.sum(xf, axis=1, keepdims=True) * (1.0 / M)
                d = xf - mu
                var = jnp.sum(d * d, axis=1, keepdims=True) * (1.0 / M)
                rs = lax.rsqrt(var + EPS)
                toks.append(rs)
                xn_s[rows_at(r0, LP, 2), :] = pltpu.bitcast((d * rs).astype(bf16), u32)

        def kv_proj(pair, r0, n, names):
            lhs = ckv_s[rows_at(r0, n, 1, 64), :]
            slot = pair % NP if isinstance(pair, int) else pair & (NP - 1)
            for name in names:
                for e, w in enumerate(unpack(pair, name)):
                    y = jnp.dot(lhs, w, preferred_element_type=f32)
                    dst = k_s if name == "k" else v_s
                    dst[2 * slot + e, rows_at(r0, n, 2, 64), :] = pltpu.bitcast(y.astype(bf16), u32)

        with jax.named_scope("prologue"):
            for k, (kind, i) in enumerate(PRO_ORDER):
                if k and kind != PRO_ORDER[k - 1][0]:
                    pl.semaphore_signal(sem_reg, 1)
                    pl.semaphore_wait(sem_reg, 1)
                if kind == "c":
                    ckv_copy(i).start()
                elif kind == "x":
                    x_copy(i).start()
                elif kind == "w":
                    w_copy(i, "kv", sem_kv, False)
                else:
                    w_copy(i, "q", sem_q, False)
            attn_s[...] = jnp.zeros(attn_s.shape, u32)
            w_copy(0, "kv", sem_kv, True)
            for i in range(3):
                ckv_copy(i).wait()
                with jax.named_scope("r%d" % i):
                    kv_proj(0, CKV_SPLIT[i], CKV_SPLIT[i + 1] - CKV_SPLIT[i], "kv")
            ckv_copy(3).wait()

            def pro_body(t, carry):
                @pl.when(t == 1)
                def _():
                    w_copy(1, "kv", sem_kv, True)

                x_copy(2 * t).wait()
                x_copy(2 * t + 1).wait()
                with jax.named_scope("rl"):
                    layernorm_x(2 * t * XC, 2 * XC)
                    kv_proj(jnp.minimum(t, 1), jnp.where(t == 0, S - KR, jnp.minimum((t - 1) * KR, S - KR)), KR, "kv")
                return carry

            lax.fori_loop(0, 4, pro_body, 0)

        row = lax.broadcasted_iota(jnp.int32, (G, T), 0)
        col = lax.broadcasted_iota(jnp.int32, (G, T), 1)

        def pair_step(p):
            w_copy(p, "q", sem_q, True)

            @pl.when(p + 2 < n_pair)
            def _():
                w_copy(p + 2, "kv", sem_kv, True)

            tri = col <= row + (T - G)

            def kv_units(name):
                for i in range(UPS):
                    u = p * UPS + i
                    kv_proj(2 + (u >> 3), (u & 7) * UR, UR, name)

            kv_units("k")
            wq2 = unpack(p, "q")

            hist = []

            def geom(blk):
                _, c, j = blk
                k0 = (c + 1) * G % T
                return k0, A * j + (0 if k0 else 1), [(A * j + a) * T + c * G for a in range(A)]

            def qproj(blk):
                xn = jnp.concatenate([xn_s[r // 2:(r + G) // 2, :] for r in geom(blk)[2]], axis=0)
                return jnp.dot(pltpu.bitcast(xn, bf16), wq2[blk[0]], preferred_element_type=f32) * scale

            def qk(blk, qf):
                k0, n, _ = geom(blk)
                kk = kv(k_s, blk[0])
                if len(hist) >= AQ:
                    qf = jnp.where(jnp.concatenate(hist[-AQ], axis=0) < 0.0, 0.0, qf)
                q = qf.astype(bf16)
                main = head = None
                if n:
                    main = lax.dot_general(q, kk[k0:k0 + n * T, :], NT, preferred_element_type=f32)
                if k0:
                    st = lax.dot_general(kk[0:k0, :], q, NT, preferred_element_type=f32)
                    head = jnp.concatenate([st, jnp.full((T - k0, T), NEG, f32)], axis=0).T
                extra = [lax.dot_general(qf[e * G:].astype(bf16), kk[k0 + (n + e - 1) * T:k0 + (n + e) * T, :], NT,
                                         preferred_element_type=f32) for e in range(1, A)]
                return main, head, extra

            def softmax_pv(blk, sc):
                k0, n, rows = geom(blk)
                vv = kv(v_s, blk[0])
                main, head, extra = sc
                ps, rls = [], []
                for a in range(A):
                    parts = []
                    if n:
                        mm = main[a * G:(a + 1) * G]
                        if a == 0:
                            parts += [mm[:, :(n - 1) * T]] if n > 1 else []
                            parts.append(jnp.where(tri, mm[:, (n - 1) * T:], NEG))
                        else:
                            parts.append(mm)
                    if k0:
                        hd = head[a * G:(a + 1) * G]
                        parts.append(hd if n + a else jnp.where(col <= row + (k0 - G), hd, NEG))
                    for e in range(1, a + 1):
                        ex = extra[e - 1][(a - e) * G:(a - e + 1) * G]
                        parts.append(jnp.where(tri, ex, NEG) if e == a else ex)
                    s = jnp.concatenate(parts, axis=1) if len(parts) > 1 else parts[0]
                    pr = jnp.exp2(s - jnp.max(s, axis=1, keepdims=True))
                    rls.append(_recip(jnp.sum(_rnd(pr), axis=1, keepdims=True)))
                    ps.append(pr)
                hist.append(rls)
                w = ps[0].shape[1]
                vm = [vv[k0:k0 + n * T, :]] if n else []
                vm += [vv[0:T, :]] if k0 else []
                o = jnp.dot(jnp.concatenate([x[:, :w] for x in ps], axis=0).astype(bf16),
                            jnp.concatenate(vm, axis=0) if len(vm) > 1 else vm[0], preferred_element_type=f32)
                outs = [o[a * G:(a + 1) * G] for a in range(A)]
                for e in range(1, A):
                    pe = jnp.concatenate([x[:, w + (e - 1) * T:w + e * T] for x in ps[e:]], axis=0).astype(bf16)
                    oe = jnp.dot(pe, vv[k0 + (n + e - 1) * T:k0 + (n + e) * T, :], preferred_element_type=f32)
                    for a in range(e, A):
                        outs[a] = outs[a] + oe[(a - e) * G:(a - e + 1) * G]
                for a, r in enumerate(rows):
                    ctx_s[2 * p + blk[0], r // 2:(r + G) // 2, :] = pltpu.bitcast((outs[a] * rls[a]).astype(bf16), u32)

            order = [(e, c, j) for e in range(2) for j in range(nb // A - 1, -1, -1) for c in range(A)]
            order = [order[k] for k in ORDER]
            qs, ss, loaded = {}, {}, {}

            def kv(ref, e):
                if (id(ref), e) not in loaded:
                    loaded[id(ref), e] = pltpu.bitcast(ref[2 * (p & (NP - 1)) + e], bf16)
                return loaded[id(ref), e]

            def do_q(n):
                if n < len(order):
                    qs[n] = qproj(order[n])

            def do_qk(n):
                if n < len(order):
                    ss[n] = qk(order[n], qs.pop(n))

            for n in range(AHEAD + QAHEAD):
                do_q(n)
                if n >= QAHEAD:
                    do_qk(n - QAHEAD)
                if n == QAHEAD:
                    kv_units("v")
            for n in range(len(order)):
                do_q(n + AHEAD + QAHEAD)
                do_qk(n + AHEAD)
                softmax_pv(order[n], ss.pop(n))

            @pl.when(p + 2 < n_pair)
            def _():
                w_copy(jnp.minimum(p + 2, n_pair - 1), "q", sem_q, False)

            @pl.when(p + 4 < n_pair)
            def _():
                w_copy(jnp.minimum(p + 4, n_pair - 1), "kv", sem_kv, False)

            for j in range(len(big_copies)):
                @pl.when(p == 2 * j + 1)
                def _():
                    big_copies[j].start()

        def pair_body(p, carry):
            with jax.named_scope("main"):
                pair_step(p)
            return carry

        lax.fori_loop(0, n_pair, pair_body, 0)

        for c in big_copies:
            c.wait()
        wr = wr_s[...].astype(f32).reshape(1, M)

        def out_copy(r0, n, k=0):
            rows = rows_at(r0, n)
            return pltpu.make_async_copy(out_s.at[rows, :], out_hbm.at[rows, :], sem_out.at[k])

        def ctx_rows(segs):
            lhs = [jnp.concatenate([ctx_s[j, rows_at(r0, n, 2, U), :] for j in range(H)], axis=1) for r0, n in segs]
            return pltpu.bitcast(jnp.concatenate(lhs, axis=0), bf16)

        def post(segs, attn, top, rs, dist=1, ascending=True):
            for n, r0 in enumerate([row0 + k * PR for row0, nrows in segs for k in range(nrows // PR)]):
                rows = rows_at(r0, PR)
                xf = x_s[rows, :].astype(f32)
                if len(rs) >= dist:
                    xf = jnp.where(rs[-dist] * rs[-dist] < 0.0, 0.0, xf)
                elif rs and dist < 4:
                    xf = jnp.where(var < 0.0, 0.0, xf)
                af = pltpu.bitcast(attn[n * PR // 2:(n + 1) * PR // 2, :], bf16).astype(f32)
                h = (xf + af).astype(bf16)
                hf = h.astype(f32)
                mu = jnp.sum(hf, axis=1, keepdims=True) * (1.0 / M)
                dc = hf - mu
                var = jnp.sum(dc * dc, axis=1, keepdims=True) * (1.0 / M)
                den = _rnd(jnp.sqrt(_rnd(_rnd(var) + _rnd(jnp.full((1, 1), EPS, f32)))))
                hn = (_rnd(hf - _rnd(mu)) * (1.0 / den)).astype(bf16)
                hnf = hn.astype(f32)
                h_s[rows, :] = h
                hn_s[rows, :] = hn
                out_s[rows, :] = (hf + hnf).astype(bf16)
                r = _rnd(jnp.sum(hnf * wr, axis=1, keepdims=True))
                rs.append(r)
                m1, i1, m2, i2 = top
                idx = r0 + slot_id
                g1, g2 = r > m1, r > m2
                if not ascending:
                    g1, g2 = g1 | ((r == m1) & (idx < i1)), g2 | ((r == m2) & (idx < i2))
                top = (jnp.where(g1, r, m1), jnp.where(g1, idx, i1),
                       jnp.where(g1, m1, jnp.where(g2, r, m2)), jnp.where(g1, i1, jnp.where(g2, idx, i2)))
            return top

        slot_id = lax.broadcasted_iota(jnp.int32, (PR, 1), 0)
        ninf = jnp.full((PR, 1), -jnp.inf, f32)

        def pick(top):
            val = jnp.concatenate([top[0], top[2]], axis=0)
            pos = jnp.concatenate([top[1], top[3]], axis=0).astype(f32)
            m1 = jnp.max(val, axis=0, keepdims=True)
            p1 = jnp.min(jnp.where(val == m1, pos, float(S)), axis=0, keepdims=True)
            rest = jnp.where(pos == p1, -jnp.inf, val)
            m2 = jnp.max(rest, axis=0, keepdims=True)
            p2 = jnp.min(jnp.where((rest == m2) & (pos != p1), pos, float(S)), axis=0, keepdims=True)
            return m1, m2, [jnp.clip(x.astype(jnp.int32)[0, 0], 0, S - 1) for x in (p1, p2)]

        rt = S - 3 * U
        top0 = (ninf, slot_id, ninf, slot_id + PR)
        unit_s[0] = rt

        def oproj_body(b, top):
            @pl.when(b == 1)
            def _():
                unit_s[0] = jnp.maximum(pick(top)[2][0] & -U, rt)

            with jax.named_scope("oloop"):
                prev = jnp.where(b == 0, rt, (b - 1) * RB)
                top = post([(prev, RB)], attn_s, [jnp.where(b == 1, i, t) for i, t in zip(top0, top)], [])
                segs = [(b * RB, RB - U), (jnp.where(b == n_rb - 1, unit_s[0], b * RB + RB - U), U)]
                o = jnp.dot(ctx_rows(segs), wo_s[:, 0:M], preferred_element_type=f32)
                attn_s[...] = pltpu.bitcast(o.astype(bf16), u32)

                @pl.when(b > 0)
                def _():
                    out_copy(prev, RB).start()
            return top

        top = lax.fori_loop(0, n_rb, oproj_body, top0)

        def groups(tok):
            return [pl.multiple_of(i & -FG, FG) for i in tok]

        def gather(ref, tok):
            return jnp.concatenate([ref[pl.ds(g, FG), :].astype(f32) for g in groups(tok)], axis=0)

        def swiglu(g, u):
            g, u = _rnd(g), _rnd(u)
            return (_rnd(g * jax.nn.sigmoid(g)) * u).astype(bf16)

        def finish(y, xs, m1, m2, tok):
            rid = lax.broadcasted_iota(jnp.int32, (2 * FG, 1), 0)
            g1, g2 = groups(tok)
            pos = jnp.where(rid < FG, g1 + rid, g2 + rid - FG)
            gate = _rnd(jax.nn.sigmoid(jnp.where(pos == tok[0], m1, m2)))
            upd = jnp.where((pos == tok[0]) | (pos == tok[1]), _rnd(_rnd(y) * gate), 0.0)
            fix_s[...] = (gather(h_s, tok) + _rnd(xs + upd)).astype(bf16)

        with jax.named_scope("tail"):
            last = [((n_rb - 1) * RB, RB - U), (unit_s[0], U)]
            ra, rb = rt + jnp.where(unit_s[0] == rt, U, 0), rt + jnp.where(unit_s[0] == rt + 2 * U, U, 2 * U)
            top = post(last, attn_s, top, [], dist=2)
            for seg in last:
                out_copy(*seg).start()

            m1, m2, tok = pick(top)
            xs = gather(hn_s, tok)
            xb = xs.astype(bf16)
            nc = F // KC
            todo = []
            for c in range(nc + DL):
                todo += [("gu", c, n) for n in range(2 * KC // T)] if c < nc else []
                todo += [("down", c - DL, n) for n in range(M // (2 * T))] if c >= DL else []
            gu, act, y, rs_a = {}, {}, {}, []

            def ffn_step():
                kind, c, n = todo.pop(0)
                if kind == "gu":
                    c0 = c * KC + n // 2 * T
                    gu[c, n] = jnp.dot(xb, (wg_s, wu_s)[n % 2][:, c0:c0 + T], preferred_element_type=f32)
                    return
                if c not in act:
                    g, u = [jnp.concatenate([gu[c, k] for k in range(w, 2 * KC // T, 2)], axis=1) for w in range(2)]
                    if c == AC:
                        u = jnp.where(rs_a[-1] * rs_a[-1] < 0.0, 0.0, u)
                    act[c] = swiglu(g, u)
                d = jnp.dot(act[c], wd_s[c * KC:(c + 1) * KC, n * 2 * T:(n + 1) * 2 * T], preferred_element_type=f32)
                y[n] = d if c == 0 else y[n] + d

            attn_t, host = [], 0
            n_host, n_in = 2 * (M // T) * (H * D // KC), len(todo) - NLEFT
            slots = {LEAD + i * (n_host - LEAD) // n_in for i in range(n_in)}
            for r0 in (ra, rb):
                lhs = ctx_rows([(r0, U)])
                acc = []
                for i in range(M // T * (H * D // KC)):
                    n, k = divmod(i, H * D // KC)
                    if r0 is ra:
                        w = wo_s[:, n * T:(n + 1) * T][k * KC:(k + 1) * KC]
                    else:
                        w = wo_s[k * KC:(k + 1) * KC, n * T:(n + 1) * T]
                    d = jnp.dot(lhs[:, k * KC:(k + 1) * KC], w, preferred_element_type=f32)
                    acc = acc + [d] if k == 0 else acc[:-1] + [acc[-1] + d]
                    if host in slots:
                        ffn_step()
                    host += 1
                attn_t.append(pltpu.bitcast(jnp.concatenate(acc, axis=1).astype(bf16), u32))
                if r0 is ra:
                    top = post([(ra, U)], attn_t[0], top, rs_a, ascending=False)
                    out_copy(ra, U, 1).start()
            while todo:
                ffn_step()
            attn_a, attn_b = attn_t
            finish(jnp.concatenate([y[n] for n in range(M // (2 * T))], axis=1), xs, m1, m2, tok)

            top = post([(rb, U)], attn_b, top, [], dist=4, ascending=False)
            out_copy(rb, U, 2).start()
            m1, m2, fin = pick(top)

            redo = (fin[0] != tok[0]) | (fin[1] != tok[1])

            @pl.when(redo)
            def _():
                xs = gather(hn_s, fin)
                xb = xs.astype(bf16)

                def chunk(c, y):
                    cols = pl.ds(pl.multiple_of(c * FC, FC), FC)
                    act = swiglu(jnp.dot(xb, wg_s[:, cols], preferred_element_type=f32),
                                 jnp.dot(xb, wu_s[:, cols], preferred_element_type=f32))
                    return y + jnp.dot(act, wd_s[cols, 0:M], preferred_element_type=f32)

                finish(lax.fori_loop(0, F // FC, chunk, jnp.zeros((2 * FG, M), f32)), xs, m1, m2, fin)
                out_copy(ra, U, 1).wait()
                out_copy(rb, U, 2).wait()

            g1, g2 = groups(fin)
            out_copy(0, rt).wait()
            out_copy(*last[1]).wait()
            c1 = pltpu.make_async_copy(fix_s.at[pl.ds(0, FG), :], out_hbm.at[pl.ds(g1, FG), :], sem_fix.at[0])
            c2 = pltpu.make_async_copy(fix_s.at[pl.ds(FG, FG), :], out_hbm.at[pl.ds(g2, FG), :], sem_fix.at[1])
            c1.start()

            @pl.when(g1 != g2)
            def _():
                c2.start()
                c2.wait()

            c1.wait()

            @pl.when(jnp.logical_not(redo))
            def _():
                out_copy(ra, U, 1).wait()
                out_copy(rb, U, 2).wait()

    scratch = [
        pltpu.VMEM((S, M), bf16),
        pltpu.VMEM((S // 2, M), u32),
        pltpu.VMEM((S, C), bf16),
        pltpu.VMEM((NQ, qa, 2 * WB, D), bf16),
        pltpu.VMEM((NKV, 2 * ka, 2 * WB, D), bf16),
        pltpu.VMEM((2 * NP, S // 2, D), u32),
        pltpu.VMEM((2 * NP, S // 2, D), u32),
        pltpu.VMEM((H, S // 2, D), u32),
        pltpu.VMEM((H * D, M + W_PAD), bf16),
        pltpu.VMEM((M,), bf16),
        pltpu.VMEM((M, F), bf16),
        pltpu.VMEM((M, F), bf16),
        pltpu.VMEM((F, M + W_PAD), bf16),
        pltpu.VMEM((RB // 2, M), u32),
        pltpu.VMEM((S, M), bf16),
        pltpu.VMEM((S, M), bf16),
        pltpu.VMEM((S, M), bf16),
        pltpu.VMEM((2 * FG, M), bf16),
        pltpu.SMEM((1,), jnp.int32),
        pltpu.SemaphoreType.DMA((len(CKV_SPLIT) - 1,)),
        pltpu.SemaphoreType.DMA((n_xc,)),
        pltpu.SemaphoreType.DMA((NQ,)),
        pltpu.SemaphoreType.DMA((NKV,)),
        pltpu.SemaphoreType.DMA((5,)),
        pltpu.SemaphoreType.DMA((3,)),
        pltpu.SemaphoreType.DMA((2,)),
        pltpu.SemaphoreType.REGULAR,
    ]
    return kernel, scratch


@jax.jit
def pallas_sequential_preLN__compressed_kv_cla__moe_arch_mod__prompt_kernel(
    A_x: jax.Array,
    A_c_kv: jax.Array,
    A_w_q: jax.Array,
    A_w_uk: jax.Array,
    A_w_uv: jax.Array,
    A_w_o: jax.Array,
    B_x: jax.Array,
    B_w_r: jax.Array,
    B_w_gate: jax.Array,
    B_w_up: jax.Array,
    B_w_down: jax.Array,
):
    B, S, M = A_x.shape
    C = A_c_kv.shape[2]
    H, D = A_w_q.shape[1], A_w_q.shape[2]
    F = B_w_gate.shape[1]
    assert B == 1 and A_c_kv.shape[1] == S

    kernel, scratch = _make_kernel(S, M, C, H, D, F)
    any_spec = pl.BlockSpec(memory_space=pl.ANY)
    out = pl.pallas_call(
        kernel,
        grid=(1,),
        in_specs=[any_spec] * 10,
        out_specs=any_spec,
        out_shape=jax.ShapeDtypeStruct((S, M), A_x.dtype),
        scratch_shapes=scratch,
        compiler_params=pltpu.CompilerParams(
            vmem_limit_bytes=120 * 1024 * 1024,
            disable_bounds_checks=True,
            disable_semaphore_checks=True,
        ),
        name="mla_mod_block",
    )(
        A_x.reshape(S, M), A_c_kv.reshape(S, C),
        A_w_q.reshape(M // WB, WB, H // 2, 2, D),
        A_w_uk.reshape(C // WB, WB, H // 2, 2, D),
        A_w_uv.reshape(C // WB, WB, H // 2, 2, D),
        A_w_o.reshape(H * D, M), B_w_r, B_w_gate, B_w_up, B_w_down,
    )
    return out.reshape(B, S, M)
```

```python
import jax
import jax.numpy as jnp
from jax import lax
import jax.experimental.pallas as pl
import jax.experimental.pallas.tpu as pltpu

bf16 = jnp.bfloat16
f32 = jnp.float32
u32 = jnp.uint32

T = 128
G = 32
A = T // G
AHEAD = 3
QAHEAD = 1
AQ = 8
ORDER = (0, 1, 2, 4, 3, 5, 10, 7, 8, 16, 6, 11, 9, 17, 18, 19, 20, 22, 21, 24, 25, 26, 27, 28, 23, 12, 13, 29, 14, 30, 15, 31)
WB = 4
NQ, NKV, NP = 4, 8, 4
UR, UPS = 256, 7
RB = 192
U = 64
FG = 8
KC = 512
LEAD, NLEFT = 51, 11
DL, AC = 2, 4
FC = 896
PR = 16
LP, LCH = 16, 4
XC = 256
CKV_SPLIT = (0, 256, 768, 1344, 2048)
PRO_ORDER = ([("w", 0)] + [("c", i) for i in range(4)] + [("x", i) for i in range(3)] + [("w", 1)]
             + [("x", i) for i in range(3, 8)] + [("w", 2), ("q", 0), ("q", 1), ("w", 3)])
KR = 704
W_PAD = 128
EPS = 1e-5
NEG = -1e30
LOG2E = 1.4426950408889634
NT = (((1,), (1,)), ((), ()))


def _rnd(x):
    return x.astype(bf16).astype(f32)


def _recip(l):
    r = pl.reciprocal(l, approx=True)
    return r * (2.0 - l * r)


def _make_kernel(S, M, C, H, D, F):
    n_pair = H // 2
    nb = S // T
    n_rb = (S - 2 * U) // RB
    assert n_rb * RB + 2 * U == S and RB == 3 * U
    n_xc = S // XC
    qa, ka = M // WB, C // WB
    upp = S // UR
    assert sorted(ORDER) == list(range(2 * nb)) and CKV_SPLIT[-1] == S and CKV_SPLIT[-2] == S - KR
    assert upp == 8 and (n_pair - 2) * upp == n_pair * UPS
    scale = (D ** -0.5) * LOG2E

    def kernel(*refs):
        def once(i, carry):
            kernel_body(*refs)
            return carry

        lax.fori_loop(0, pl.program_id(0) + 1, once, 0)

    def kernel_body(x_hbm, ckv_hbm, wq_hbm, wk_hbm, wv_hbm, wo_hbm, wr_hbm, wg_hbm, wu_hbm, wd_hbm,
                    out_hbm,
                    x_s, xn_s, ckv_s, wq_s, wkv_s, k_s, v_s, ctx_s,
                    wo_s, wr_s, wg_s, wu_s, wd_s, attn_s, h_s, hn_s, out_s, fix_s, unit_s,
                    sem_in, sem_x, sem_q, sem_kv, sem_big, sem_out, sem_fix, sem_reg):

        w_parts = {"q": (wq_hbm, wq_s, NQ, 0, qa), "k": (wk_hbm, wkv_s, NKV, 0, ka), "v": (wv_hbm, wkv_s, NKV, ka, ka)}

        def w_copy(p, names, sem, wait):
            _, buf, nslot, _, _ = w_parts[names[0]]
            slot = p % nslot if isinstance(p, int) else p & (nslot - 1)
            if wait:
                pltpu.make_async_copy(buf.at[slot], buf.at[slot], sem.at[slot]).wait()
                return
            for name in names:
                hbm, _, _, r0, n = w_parts[name]
                for b in range(WB):
                    pltpu.make_async_copy(hbm.at[:, b, p], buf.at[slot, pl.ds(r0, n), pl.ds(2 * b, 2), :],
                                          sem.at[slot]).start()

        def unpack(p, name):
            _, buf, nslot, r0, n = w_parts[name]
            slot = p % nslot if isinstance(p, int) else p & (nslot - 1)
            w = pltpu.bitcast(buf[slot, r0:r0 + n].reshape(n * 2 * WB, D), u32)
            return [pltpu.bitcast(x, f32).astype(bf16) for x in (w << 16, w & jnp.uint32(0xFFFF0000))]

        big_copies = [
            pltpu.make_async_copy(wo_hbm, wo_s.at[:, pl.ds(0, M)], sem_big.at[0]),
            pltpu.make_async_copy(wg_hbm, wg_s, sem_big.at[1]),
            pltpu.make_async_copy(wu_hbm, wu_s, sem_big.at[2]),
            pltpu.make_async_copy(wd_hbm, wd_s.at[:, pl.ds(0, M)], sem_big.at[3]),
            pltpu.make_async_copy(wr_hbm, wr_s, sem_big.at[4]),
        ]

        def rows_at(r0, n, div=1, align=16):
            if isinstance(r0, int):
                return pl.ds(r0 // div, n // div)
            return pl.ds(pl.multiple_of(r0 >> (div - 1), align // div), n // div)

        def x_copy(i):
            rows = rows_at(i * XC, XC)
            return pltpu.make_async_copy(x_hbm.at[rows, :], x_s.at[rows, :], sem_x.at[i])

        def ckv_copy(i):
            rows = pl.ds(CKV_SPLIT[i], CKV_SPLIT[i + 1] - CKV_SPLIT[i])
            return pltpu.make_async_copy(ckv_hbm.at[rows, :], ckv_s.at[rows, :], sem_in.at[i])

        def layernorm_x(row0, nrows):
            toks = []
            for n in range(nrows // LP):
                r0 = row0 + n * LP
                xf = x_s[rows_at(r0, LP), :].astype(f32)
                if len(toks) >= LCH:
                    xf = jnp.where(toks[-LCH] < 0.0, 0.0, xf)
                elif toks:
                    xf = jnp.where(mu * mu < 0.0, 0.0, xf)
                mu = jnp.sum(xf, axis=1, keepdims=True) * (1.0 / M)
                d = xf - mu
                var = jnp.sum(d * d, axis=1, keepdims=True) * (1.0 / M)
                rs = lax.rsqrt(var + EPS)
                toks.append(rs)
                xn_s[rows_at(r0, LP, 2), :] = pltpu.bitcast((d * rs).astype(bf16), u32)

        def kv_proj(pair, r0, n, names):
            lhs = ckv_s[rows_at(r0, n, 1, 64), :]
            slot = pair % NP if isinstance(pair, int) else pair & (NP - 1)
            for name in names:
                for e, w in enumerate(unpack(pair, name)):
                    y = jnp.dot(lhs, w, preferred_element_type=f32)
                    dst = k_s if name == "k" else v_s
                    dst[2 * slot + e, rows_at(r0, n, 2, 64), :] = pltpu.bitcast(y.astype(bf16), u32)

        with jax.named_scope("prologue"):
            for k, (kind, i) in enumerate(PRO_ORDER):
                if k and kind != PRO_ORDER[k - 1][0]:
                    pl.semaphore_signal(sem_reg, 1)
                    pl.semaphore_wait(sem_reg, 1)
                if kind == "c":
                    ckv_copy(i).start()
                elif kind == "x":
                    x_copy(i).start()
                elif kind == "w":
                    w_copy(i, "kv", sem_kv, False)
                else:
                    w_copy(i, "q", sem_q, False)
            attn_s[...] = jnp.zeros(attn_s.shape, u32)
            w_copy(0, "kv", sem_kv, True)
            for i in range(3):
                ckv_copy(i).wait()
                with jax.named_scope("r%d" % i):
                    kv_proj(0, CKV_SPLIT[i], CKV_SPLIT[i + 1] - CKV_SPLIT[i], "kv")
            ckv_copy(3).wait()

            def pro_body(t, carry):
                @pl.when(t == 1)
                def _():
                    w_copy(1, "kv", sem_kv, True)

                x_copy(2 * t).wait()
                x_copy(2 * t + 1).wait()
                with jax.named_scope("rl"):
                    layernorm_x(2 * t * XC, 2 * XC)
                    kv_proj(jnp.minimum(t, 1), jnp.where(t == 0, S - KR, jnp.minimum((t - 1) * KR, S - KR)), KR, "kv")
                return carry

            lax.fori_loop(0, 4, pro_body, 0)

        row = lax.broadcasted_iota(jnp.int32, (G, T), 0)
        col = lax.broadcasted_iota(jnp.int32, (G, T), 1)

        def pair_step(p):
            w_copy(p, "q", sem_q, True)

            @pl.when(p + 2 < n_pair)
            def _():
                w_copy(p + 2, "kv", sem_kv, True)

            tri = col <= row + (T - G)

            def kv_units(name):
                for i in range(UPS):
                    u = p * UPS + i
                    kv_proj(2 + (u >> 3), (u & 7) * UR, UR, name)

            kv_units("k")
            wq2 = unpack(p, "q")

            hist = []

            def geom(blk):
                _, c, j = blk
                k0 = (c + 1) * G % T
                return k0, A * j + (0 if k0 else 1), [(A * j + a) * T + c * G for a in range(A)]

            def qproj(blk):
                xn = jnp.concatenate([xn_s[r // 2:(r + G) // 2, :] for r in geom(blk)[2]], axis=0)
                return jnp.dot(pltpu.bitcast(xn, bf16), wq2[blk[0]], preferred_element_type=f32) * scale

            def qk(blk, qf):
                k0, n, _ = geom(blk)
                kk = kv(k_s, blk[0])
                if len(hist) >= AQ:
                    qf = jnp.where(jnp.concatenate(hist[-AQ], axis=0) < 0.0, 0.0, qf)
                q = qf.astype(bf16)
                main = head = None
                if n:
                    main = lax.dot_general(q, kk[k0:k0 + n * T, :], NT, preferred_element_type=f32)
                if k0:
                    st = lax.dot_general(kk[0:k0, :], q, NT, preferred_element_type=f32)
                    head = jnp.concatenate([st, jnp.full((T - k0, T), NEG, f32)], axis=0).T
                extra = [lax.dot_general(qf[e * G:].astype(bf16), kk[k0 + (n + e - 1) * T:k0 + (n + e) * T, :], NT,
                                         preferred_element_type=f32) for e in range(1, A)]
                return main, head, extra

            def softmax_pv(blk, sc):
                k0, n, rows = geom(blk)
                vv = kv(v_s, blk[0])
                main, head, extra = sc
                ps, rls = [], []
                for a in range(A):
                    parts = []
                    if n:
                        mm = main[a * G:(a + 1) * G]
                        if a == 0:
                            parts += [mm[:, :(n - 1) * T]] if n > 1 else []
                            parts.append(jnp.where(tri, mm[:, (n - 1) * T:], NEG))
                        else:
                            parts.append(mm)
                    if k0:
                        hd = head[a * G:(a + 1) * G]
                        parts.append(hd if n + a else jnp.where(col <= row + (k0 - G), hd, NEG))
                    for e in range(1, a + 1):
                        ex = extra[e - 1][(a - e) * G:(a - e + 1) * G]
                        parts.append(jnp.where(tri, ex, NEG) if e == a else ex)
                    s = jnp.concatenate(parts, axis=1) if len(parts) > 1 else parts[0]
                    pr = jnp.exp2(s - jnp.max(s, axis=1, keepdims=True))
                    rls.append(_recip(jnp.sum(_rnd(pr), axis=1, keepdims=True)))
                    ps.append(pr)
                hist.append(rls)
                w = ps[0].shape[1]
                vm = [vv[k0:k0 + n * T, :]] if n else []
                vm += [vv[0:T, :]] if k0 else []
                o = jnp.dot(jnp.concatenate([x[:, :w] for x in ps], axis=0).astype(bf16),
                            jnp.concatenate(vm, axis=0) if len(vm) > 1 else vm[0], preferred_element_type=f32)
                outs = [o[a * G:(a + 1) * G] for a in range(A)]
                for e in range(1, A):
                    pe = jnp.concatenate([x[:, w + (e - 1) * T:w + e * T] for x in ps[e:]], axis=0).astype(bf16)
                    oe = jnp.dot(pe, vv[k0 + (n + e - 1) * T:k0 + (n + e) * T, :], preferred_element_type=f32)
                    for a in range(e, A):
                        outs[a] = outs[a] + oe[(a - e) * G:(a - e + 1) * G]
                for a, r in enumerate(rows):
                    ctx_s[2 * p + blk[0], r // 2:(r + G) // 2, :] = pltpu.bitcast((outs[a] * rls[a]).astype(bf16), u32)

            order = [(e, c, j) for e in range(2) for j in range(nb // A - 1, -1, -1) for c in range(A)]
            order = [order[k] for k in ORDER]
            qs, ss, loaded = {}, {}, {}

            def kv(ref, e):
                if (id(ref), e) not in loaded:
                    loaded[id(ref), e] = pltpu.bitcast(ref[2 * (p & (NP - 1)) + e], bf16)
                return loaded[id(ref), e]

            def do_q(n):
                if n < len(order):
                    qs[n] = qproj(order[n])

            def do_qk(n):
                if n < len(order):
                    ss[n] = qk(order[n], qs.pop(n))

            for n in range(AHEAD + QAHEAD):
                do_q(n)
                if n >= QAHEAD:
                    do_qk(n - QAHEAD)
                if n == QAHEAD:
                    kv_units("v")
            for n in range(len(order)):
                do_q(n + AHEAD + QAHEAD)
                do_qk(n + AHEAD)
                softmax_pv(order[n], ss.pop(n))

            @pl.when(p + 2 < n_pair)
            def _():
                w_copy(jnp.minimum(p + 2, n_pair - 1), "q", sem_q, False)

            @pl.when(p + 4 < n_pair)
            def _():
                w_copy(jnp.minimum(p + 4, n_pair - 1), "kv", sem_kv, False)

            for j in range(len(big_copies)):
                @pl.when(p == 2 * j + 1)
                def _():
                    big_copies[j].start()

        def pair_body(p, carry):
            with jax.named_scope("main"):
                pair_step(p)
            return carry

        lax.fori_loop(0, n_pair, pair_body, 0)

        for c in big_copies:
            c.wait()
        wr = wr_s[...].astype(f32).reshape(1, M)

        def out_copy(r0, n, k=0):
            rows = rows_at(r0, n)
            return pltpu.make_async_copy(out_s.at[rows, :], out_hbm.at[rows, :], sem_out.at[k])

        def ctx_rows(segs):
            lhs = [jnp.concatenate([ctx_s[j, rows_at(r0, n, 2, U), :] for j in range(H)], axis=1) for r0, n in segs]
            return pltpu.bitcast(jnp.concatenate(lhs, axis=0), bf16)

        def post(segs, attn, top, rs, dist=1, ascending=True):
            for n, r0 in enumerate([row0 + k * PR for row0, nrows in segs for k in range(nrows // PR)]):
                rows = rows_at(r0, PR)
                xf = x_s[rows, :].astype(f32)
                if len(rs) >= dist:
                    xf = jnp.where(rs[-dist] * rs[-dist] < 0.0, 0.0, xf)
                elif rs and dist < 4:
                    xf = jnp.where(var < 0.0, 0.0, xf)
                af = pltpu.bitcast(attn[n * PR // 2:(n + 1) * PR // 2, :], bf16).astype(f32)
                h = (xf + af).astype(bf16)
                hf = h.astype(f32)
                mu = jnp.sum(hf, axis=1, keepdims=True) * (1.0 / M)
                dc = hf - mu
                var = jnp.sum(dc * dc, axis=1, keepdims=True) * (1.0 / M)
                den = _rnd(jnp.sqrt(_rnd(_rnd(var) + _rnd(jnp.full((1, 1), EPS, f32)))))
                hn = (_rnd(hf - _rnd(mu)) * (1.0 / den)).astype(bf16)
                hnf = hn.astype(f32)
                h_s[rows, :] = h
                hn_s[rows, :] = hn
                out_s[rows, :] = (hf + hnf).astype(bf16)
                r = _rnd(jnp.sum(hnf * wr, axis=1, keepdims=True))
                rs.append(r)
                m1, i1, m2, i2 = top
                idx = r0 + slot_id
                g1, g2 = r > m1, r > m2
                if not ascending:
                    g1, g2 = g1 | ((r == m1) & (idx < i1)), g2 | ((r == m2) & (idx < i2))
                top = (jnp.where(g1, r, m1), jnp.where(g1, idx, i1),
                       jnp.where(g1, m1, jnp.where(g2, r, m2)), jnp.where(g1, i1, jnp.where(g2, idx, i2)))
            return top

        slot_id = lax.broadcasted_iota(jnp.int32, (PR, 1), 0)
        ninf = jnp.full((PR, 1), -jnp.inf, f32)

        def pick(top):
            val = jnp.concatenate([top[0], top[2]], axis=0)
            pos = jnp.concatenate([top[1], top[3]], axis=0).astype(f32)
            m1 = jnp.max(val, axis=0, keepdims=True)
            p1 = jnp.min(jnp.where(val == m1, pos, float(S)), axis=0, keepdims=True)
            rest = jnp.where(pos == p1, -jnp.inf, val)
            m2 = jnp.max(rest, axis=0, keepdims=True)
            p2 = jnp.min(jnp.where((rest == m2) & (pos != p1), pos, float(S)), axis=0, keepdims=True)
            return m1, m2, [jnp.clip(x.astype(jnp.int32)[0, 0], 0, S - 1) for x in (p1, p2)]

        rt = S - 3 * U
        top0 = (ninf, slot_id, ninf, slot_id + PR)
        unit_s[0] = rt

        def oproj_body(b, top):
            @pl.when(b == 1)
            def _():
                unit_s[0] = jnp.clip(pick(top)[2][0] & -U, rt, S - U)

            with jax.named_scope("oloop"):
                prev = jnp.where(b == 0, rt, (b - 1) * RB)
                top = post([(prev, RB)], attn_s, [jnp.where(b == 1, i, t) for i, t in zip(top0, top)], [])
                segs = [(b * RB, RB - U), (jnp.where(b == n_rb - 1, unit_s[0], b * RB + RB - U), U)]
                o = jnp.dot(ctx_rows(segs), wo_s[:, 0:M], preferred_element_type=f32)
                attn_s[...] = pltpu.bitcast(o.astype(bf16), u32)

                @pl.when(b > 0)
                def _():
                    out_copy(prev, RB).start()
            return top

        top = lax.fori_loop(0, n_rb, oproj_body, top0)

        def groups(tok):
            return [pl.multiple_of(jnp.clip(i & -FG, 0, S - FG), FG) for i in tok]

        def gather(ref, tok):
            return jnp.concatenate([ref[pl.ds(g, FG), :].astype(f32) for g in groups(tok)], axis=0)

        def swiglu(g, u):
            g, u = _rnd(g), _rnd(u)
            return (_rnd(g * jax.nn.sigmoid(g)) * u).astype(bf16)

        def finish(y, xs, m1, m2, tok):
            rid = lax.broadcasted_iota(jnp.int32, (2 * FG, 1), 0)
            g1, g2 = groups(tok)
            pos = jnp.where(rid < FG, g1 + rid, g2 + rid - FG)
            gate = _rnd(jax.nn.sigmoid(jnp.where(pos == tok[0], m1, m2)))
            upd = jnp.where((pos == tok[0]) | (pos == tok[1]), _rnd(_rnd(y) * gate), 0.0)
            fix_s[...] = (gather(h_s, tok) + _rnd(xs + upd)).astype(bf16)

        with jax.named_scope("tail"):
            last = [((n_rb - 1) * RB, RB - U), (unit_s[0], U)]
            ra, rb = rt + jnp.where(unit_s[0] == rt, U, 0), rt + jnp.where(unit_s[0] == rt + 2 * U, U, 2 * U)
            top = post(last, attn_s, top, [], dist=2)
            for seg in last:
                out_copy(*seg).start()

            m1, m2, tok = pick(top)
            xs = gather(hn_s, tok)
            xb = xs.astype(bf16)
            nc = F // KC
            todo = []
            for c in range(nc + DL):
                todo += [("gu", c, n) for n in range(2 * KC // T)] if c < nc else []
                todo += [("down", c - DL, n) for n in range(M // (2 * T))] if c >= DL else []
            gu, act, y, rs_a = {}, {}, {}, []

            def ffn_step():
                kind, c, n = todo.pop(0)
                if kind == "gu":
                    c0 = c * KC + n // 2 * T
                    gu[c, n] = jnp.dot(xb, (wg_s, wu_s)[n % 2][:, c0:c0 + T], preferred_element_type=f32)
                    return
                if c not in act:
                    g, u = [jnp.concatenate([gu[c, k] for k in range(w, 2 * KC // T, 2)], axis=1) for w in range(2)]
                    if c == AC:
                        u = jnp.where(rs_a[-1] * rs_a[-1] < 0.0, 0.0, u)
                    act[c] = swiglu(g, u)
                d = jnp.dot(act[c], wd_s[c * KC:(c + 1) * KC, n * 2 * T:(n + 1) * 2 * T], preferred_element_type=f32)
                y[n] = d if c == 0 else y[n] + d

            attn_t, host = [], 0
            n_host, n_in = 2 * (M // T) * (H * D // KC), len(todo) - NLEFT
            slots = {LEAD + i * (n_host - LEAD) // n_in for i in range(n_in)}
            for r0 in (ra, rb):
                lhs = ctx_rows([(r0, U)])
                acc = []
                for i in range(M // T * (H * D // KC)):
                    n, k = divmod(i, H * D // KC)
                    if r0 is ra:
                        w = wo_s[:, n * T:(n + 1) * T][k * KC:(k + 1) * KC]
                    else:
                        w = wo_s[k * KC:(k + 1) * KC, n * T:(n + 1) * T]
                    d = jnp.dot(lhs[:, k * KC:(k + 1) * KC], w, preferred_element_type=f32)
                    acc = acc + [d] if k == 0 else acc[:-1] + [acc[-1] + d]
                    if host in slots:
                        ffn_step()
                    host += 1
                attn_t.append(pltpu.bitcast(jnp.concatenate(acc, axis=1).astype(bf16), u32))
                if r0 is ra:
                    top = post([(ra, U)], attn_t[0], top, rs_a, ascending=False)
                    out_copy(ra, U, 1).start()
            while todo:
                ffn_step()
            finish(jnp.concatenate([y[n] for n in range(M // (2 * T))], axis=1), xs, m1, m2, tok)

            top = post([(rb, U)], attn_t[1], top, [], dist=4, ascending=False)
            out_copy(rb, U, 2).start()
            m1, m2, fin = pick(top)

            redo = (fin[0] != tok[0]) | (fin[1] != tok[1])

            @pl.when(redo)
            def _():
                xs = gather(hn_s, fin)
                xb = xs.astype(bf16)

                def chunk(c, y):
                    cols = pl.ds(pl.multiple_of(c * FC, FC), FC)
                    act = swiglu(jnp.dot(xb, wg_s[:, cols], preferred_element_type=f32),
                                 jnp.dot(xb, wu_s[:, cols], preferred_element_type=f32))
                    return y + jnp.dot(act, wd_s[cols, 0:M], preferred_element_type=f32)

                finish(lax.fori_loop(0, F // FC, chunk, jnp.zeros((2 * FG, M), f32)), xs, m1, m2, fin)
                out_copy(ra, U, 1).wait()
                out_copy(rb, U, 2).wait()

            g1, g2 = groups(fin)
            out_copy(0, rt).wait()
            out_copy(*last[1]).wait()
            c1 = pltpu.make_async_copy(fix_s.at[pl.ds(0, FG), :], out_hbm.at[pl.ds(g1, FG), :], sem_fix.at[0])
            c2 = pltpu.make_async_copy(fix_s.at[pl.ds(FG, FG), :], out_hbm.at[pl.ds(g2, FG), :], sem_fix.at[1])
            c1.start()

            @pl.when(g1 != g2)
            def _():
                c2.start()
                c2.wait()

            c1.wait()

            @pl.when(jnp.logical_not(redo))
            def _():
                out_copy(ra, U, 1).wait()
                out_copy(rb, U, 2).wait()

    scratch = [
        pltpu.VMEM((S, M), bf16),
        pltpu.VMEM((S // 2, M), u32),
        pltpu.VMEM((S, C), bf16),
        pltpu.VMEM((NQ, qa, 2 * WB, D), bf16),
        pltpu.VMEM((NKV, 2 * ka, 2 * WB, D), bf16),
        pltpu.VMEM((2 * NP, S // 2, D), u32),
        pltpu.VMEM((2 * NP, S // 2, D), u32),
        pltpu.VMEM((H, S // 2, D), u32),
        pltpu.VMEM((H * D, M + W_PAD), bf16),
        pltpu.VMEM((M,), bf16),
        pltpu.VMEM((M, F), bf16),
        pltpu.VMEM((M, F), bf16),
        pltpu.VMEM((F, M + W_PAD), bf16),
        pltpu.VMEM((RB // 2, M), u32),
        pltpu.VMEM((S, M), bf16),
        pltpu.VMEM((S, M), bf16),
        pltpu.VMEM((S, M), bf16),
        pltpu.VMEM((2 * FG, M), bf16),
        pltpu.SMEM((1,), jnp.int32),
        pltpu.SemaphoreType.DMA((len(CKV_SPLIT) - 1,)),
        pltpu.SemaphoreType.DMA((n_xc,)),
        pltpu.SemaphoreType.DMA((NQ,)),
        pltpu.SemaphoreType.DMA((NKV,)),
        pltpu.SemaphoreType.DMA((5,)),
        pltpu.SemaphoreType.DMA((3,)),
        pltpu.SemaphoreType.DMA((2,)),
        pltpu.SemaphoreType.REGULAR,
    ]
    return kernel, scratch


@jax.jit
def pallas_sequential_preLN__compressed_kv_cla__moe_arch_mod__prompt_kernel(
    A_x: jax.Array,
    A_c_kv: jax.Array,
    A_w_q: jax.Array,
    A_w_uk: jax.Array,
    A_w_uv: jax.Array,
    A_w_o: jax.Array,
    B_x: jax.Array,
    B_w_r: jax.Array,
    B_w_gate: jax.Array,
    B_w_up: jax.Array,
    B_w_down: jax.Array,
):
    B, S, M = A_x.shape
    C = A_c_kv.shape[2]
    H, D = A_w_q.shape[1], A_w_q.shape[2]
    F = B_w_gate.shape[1]
    assert B == 1 and A_c_kv.shape[1] == S

    kernel, scratch = _make_kernel(S, M, C, H, D, F)
    any_spec = pl.BlockSpec(memory_space=pl.ANY)
    out = pl.pallas_call(
        kernel,
        grid=(1,),
        in_specs=[any_spec] * 10,
        out_specs=any_spec,
        out_shape=jax.ShapeDtypeStruct((S, M), A_x.dtype),
        scratch_shapes=scratch,
        compiler_params=pltpu.CompilerParams(
            vmem_limit_bytes=120 * 1024 * 1024,
            disable_bounds_checks=True,
            disable_semaphore_checks=True,
        ),
        name="mla_mod_block",
    )(
        A_x.reshape(S, M), A_c_kv.reshape(S, C),
        A_w_q.reshape(M // WB, WB, H // 2, 2, D),
        A_w_uk.reshape(C // WB, WB, H // 2, 2, D),
        A_w_uv.reshape(C // WB, WB, H // 2, 2, D),
        A_w_o.reshape(H * D, M), B_w_r, B_w_gate, B_w_up, B_w_down,
    )
    return out.reshape(B, S, M)
```

```python
import jax
import jax.numpy as jnp
from jax import lax
import jax.experimental.pallas as pl
import jax.experimental.pallas.tpu as pltpu

bf16 = jnp.bfloat16
f32 = jnp.float32
u32 = jnp.uint32

T = 128
G = 32
A = T // G
AHEAD = 3
QAHEAD = 1
AQ = 8
ORDER = (0, 1, 2, 4, 3, 5, 10, 7, 8, 16, 6, 11, 9, 17, 18, 19, 20, 22, 21, 24, 25, 26, 27, 28, 23, 12, 13, 29, 14, 30, 15, 31)
WB = 4
NQ, NKV, NP = 4, 8, 4
UR, UPS = 256, 7
RB = 192
U = 64
FG = 8
KC = 512
LEAD, NLEFT = 51, 11
DL, AC = 2, 4
FC = 896
PR = 16
LP, LCH = 16, 4
XC = 256
CKV_SPLIT = (0, 256, 768, 1344, 2048)
PRO_ORDER = ([("w", 0)] + [("c", i) for i in range(4)] + [("x", i) for i in range(3)] + [("w", 1)]
             + [("x", i) for i in range(3, 8)] + [("w", 2), ("q", 0), ("q", 1), ("w", 3)])
KR = 704
W_PAD = 128
EPS = 1e-5
NEG = -1e30
LOG2E = 1.4426950408889634
NT = (((1,), (1,)), ((), ()))


def _rnd(x):
    return x.astype(bf16).astype(f32)


def _recip(l):
    r = pl.reciprocal(l, approx=True)
    return r * (2.0 - l * r)


def _make_kernel(S, M, C, H, D, F):
    n_pair = H // 2
    nb = S // T
    n_rb = (S - 2 * U) // RB
    assert n_rb * RB + 2 * U == S and RB == 3 * U and FG == 8
    n_xc = S // XC
    qa, ka = M // WB, C // WB
    upp = S // UR
    assert sorted(ORDER) == list(range(2 * nb)) and CKV_SPLIT[-1] == S and CKV_SPLIT[-2] == S - KR
    assert upp == 8 and (n_pair - 2) * upp == n_pair * UPS
    scale = (D ** -0.5) * LOG2E

    def kernel(*refs):
        def once(i, carry):
            kernel_body(*refs)
            return carry

        lax.fori_loop(0, pl.program_id(0) + 1, once, 0)

    def kernel_body(x_hbm, ckv_hbm, wq_hbm, wk_hbm, wv_hbm, wo_hbm, wr_hbm, wg_hbm, wu_hbm, wd_hbm,
                    out_hbm,
                    x_s, xn_s, ckv_s, wq_s, wkv_s, k_s, v_s, ctx_s,
                    wo_s, wr_s, wg_s, wu_s, wd_s, attn_s, h_s, hn_s, out_s, fix_s, unit_s,
                    sem_in, sem_x, sem_q, sem_kv, sem_big, sem_out, sem_reg):

        w_parts = {"q": (wq_hbm, wq_s, NQ, 0, qa), "k": (wk_hbm, wkv_s, NKV, 0, ka), "v": (wv_hbm, wkv_s, NKV, ka, ka)}

        def w_copy(p, names, sem, wait):
            _, buf, nslot, _, _ = w_parts[names[0]]
            slot = p % nslot if isinstance(p, int) else p & (nslot - 1)
            if wait:
                pltpu.make_async_copy(buf.at[slot], buf.at[slot], sem.at[slot]).wait()
                return
            for name in names:
                hbm, _, _, r0, n = w_parts[name]
                for b in range(WB):
                    pltpu.make_async_copy(hbm.at[:, b, p], buf.at[slot, pl.ds(r0, n), pl.ds(2 * b, 2), :],
                                          sem.at[slot]).start()

        def unpack(p, name):
            _, buf, nslot, r0, n = w_parts[name]
            slot = p % nslot if isinstance(p, int) else p & (nslot - 1)
            w = pltpu.bitcast(buf[slot, r0:r0 + n].reshape(n * 2 * WB, D), u32)
            return [pltpu.bitcast(x, f32).astype(bf16) for x in (w << 16, w & jnp.uint32(0xFFFF0000))]

        big_copies = [
            pltpu.make_async_copy(wo_hbm, wo_s.at[:, pl.ds(0, M)], sem_big.at[0]),
            pltpu.make_async_copy(wg_hbm, wg_s, sem_big.at[1]),
            pltpu.make_async_copy(wu_hbm, wu_s, sem_big.at[2]),
            pltpu.make_async_copy(wd_hbm, wd_s.at[:, pl.ds(0, M)], sem_big.at[3]),
            pltpu.make_async_copy(wr_hbm, wr_s, sem_big.at[4]),
        ]

        def rows_at(r0, n, div=1, align=16):
            if isinstance(r0, int):
                return pl.ds(r0 // div, n // div)
            return pl.ds(pl.multiple_of(r0 if div == 1 else r0 >> 1, align // div), n // div)

        def x_copy(i):
            rows = rows_at(i * XC, XC)
            return pltpu.make_async_copy(x_hbm.at[rows, :], x_s.at[rows, :], sem_x.at[i])

        def ckv_copy(i):
            rows = pl.ds(CKV_SPLIT[i], CKV_SPLIT[i + 1] - CKV_SPLIT[i])
            return pltpu.make_async_copy(ckv_hbm.at[rows, :], ckv_s.at[rows, :], sem_in.at[i])

        def layernorm_x(row0, nrows):
            toks = []
            for n in range(nrows // LP):
                r0 = row0 + n * LP
                xf = x_s[rows_at(r0, LP), :].astype(f32)
                if len(toks) >= LCH:
                    xf = jnp.where(toks[-LCH] < 0.0, 0.0, xf)
                elif toks:
                    xf = jnp.where(mu * mu < 0.0, 0.0, xf)
                mu = jnp.sum(xf, axis=1, keepdims=True) * (1.0 / M)
                d = xf - mu
                var = jnp.sum(d * d, axis=1, keepdims=True) * (1.0 / M)
                rs = lax.rsqrt(var + EPS)
                toks.append(rs)
                xn_s[rows_at(r0, LP, 2), :] = pltpu.bitcast((d * rs).astype(bf16), u32)

        def kv_proj(pair, r0, n, names):
            lhs = ckv_s[rows_at(r0, n, 1, 64), :]
            slot = pair % NP if isinstance(pair, int) else pair & (NP - 1)
            for name in names:
                for e, w in enumerate(unpack(pair, name)):
                    y = jnp.dot(lhs, w, preferred_element_type=f32)
                    dst = k_s if name == "k" else v_s
                    dst[2 * slot + e, rows_at(r0, n, 2, 64), :] = pltpu.bitcast(y.astype(bf16), u32)

        with jax.named_scope("prologue"):
            for k, (kind, i) in enumerate(PRO_ORDER):
                if k and kind != PRO_ORDER[k - 1][0]:
                    pl.semaphore_signal(sem_reg, 1)
                    pl.semaphore_wait(sem_reg, 1)
                if kind == "c":
                    ckv_copy(i).start()
                elif kind == "x":
                    x_copy(i).start()
                elif kind == "w":
                    w_copy(i, "kv", sem_kv, False)
                else:
                    w_copy(i, "q", sem_q, False)
            attn_s[...] = jnp.zeros(attn_s.shape, u32)
            w_copy(0, "kv", sem_kv, True)
            for i in range(3):
                ckv_copy(i).wait()
                with jax.named_scope("r%d" % i):
                    kv_proj(0, CKV_SPLIT[i], CKV_SPLIT[i + 1] - CKV_SPLIT[i], "kv")
            ckv_copy(3).wait()

            def pro_body(t, carry):
                @pl.when(t == 1)
                def _():
                    w_copy(1, "kv", sem_kv, True)

                x_copy(2 * t).wait()
                x_copy(2 * t + 1).wait()
                with jax.named_scope("rl"):
                    layernorm_x(2 * t * XC, 2 * XC)
                    kv_proj(jnp.minimum(t, 1), jnp.where(t == 0, S - KR, jnp.minimum((t - 1) * KR, S - KR)), KR, "kv")
                return carry

            lax.fori_loop(0, 4, pro_body, 0)

        row = lax.broadcasted_iota(jnp.int32, (G, T), 0)
        col = lax.broadcasted_iota(jnp.int32, (G, T), 1)

        def pair_step(p):
            w_copy(p, "q", sem_q, True)

            @pl.when(p + 2 < n_pair)
            def _():
                w_copy(p + 2, "kv", sem_kv, True)

            tri = col <= row + (T - G)

            def kv_units(name):
                for i in range(UPS):
                    u = p * UPS + i
                    kv_proj(2 + (u >> 3), (u & 7) * UR, UR, name)

            kv_units("k")
            wq2 = unpack(p, "q")

            hist = []

            def geom(blk):
                _, c, j = blk
                k0 = (c + 1) * G % T
                return k0, A * j + (0 if k0 else 1), [(A * j + a) * T + c * G for a in range(A)]

            def qproj(blk):
                xn = jnp.concatenate([xn_s[r // 2:(r + G) // 2, :] for r in geom(blk)[2]], axis=0)
                return jnp.dot(pltpu.bitcast(xn, bf16), wq2[blk[0]], preferred_element_type=f32) * scale

            def qk(blk, qf):
                k0, n, _ = geom(blk)
                kk = kv(k_s, blk[0])
                if len(hist) >= AQ:
                    qf = jnp.where(jnp.concatenate(hist[-AQ], axis=0) < 0.0, 0.0, qf)
                q = qf.astype(bf16)
                main = head = None
                if n:
                    main = lax.dot_general(q, kk[k0:k0 + n * T, :], NT, preferred_element_type=f32)
                if k0:
                    st = lax.dot_general(kk[0:k0, :], q, NT, preferred_element_type=f32)
                    head = jnp.concatenate([st, jnp.full((T - k0, T), NEG, f32)], axis=0).T
                extra = [lax.dot_general(qf[e * G:].astype(bf16), kk[k0 + (n + e - 1) * T:k0 + (n + e) * T, :], NT,
                                         preferred_element_type=f32) for e in range(1, A)]
                return main, head, extra

            def softmax_pv(blk, sc):
                k0, n, rows = geom(blk)
                vv = kv(v_s, blk[0])
                main, head, extra = sc
                ps, rls = [], []
                for a in range(A):
                    parts = []
                    if n:
                        mm = main[a * G:(a + 1) * G]
                        if a == 0:
                            parts += [mm[:, :(n - 1) * T]] if n > 1 else []
                            parts.append(jnp.where(tri, mm[:, (n - 1) * T:], NEG))
                        else:
                            parts.append(mm)
                    if k0:
                        hd = head[a * G:(a + 1) * G]
                        parts.append(hd if n + a else jnp.where(col <= row + (k0 - G), hd, NEG))
                    for e in range(1, a + 1):
                        ex = extra[e - 1][(a - e) * G:(a - e + 1) * G]
                        parts.append(jnp.where(tri, ex, NEG) if e == a else ex)
                    s = jnp.concatenate(parts, axis=1) if len(parts) > 1 else parts[0]
                    pr = jnp.exp2(s - jnp.max(s, axis=1, keepdims=True))
                    rls.append(_recip(jnp.sum(_rnd(pr), axis=1, keepdims=True)))
                    ps.append(pr)
                hist.append(rls)
                w = ps[0].shape[1]
                vm = [vv[k0:k0 + n * T, :]] if n else []
                vm += [vv[0:T, :]] if k0 else []
                o = jnp.dot(jnp.concatenate([x[:, :w] for x in ps], axis=0).astype(bf16),
                            jnp.concatenate(vm, axis=0) if len(vm) > 1 else vm[0], preferred_element_type=f32)
                outs = [o[a * G:(a + 1) * G] for a in range(A)]
                for e in range(1, A):
                    pe = jnp.concatenate([x[:, w + (e - 1) * T:w + e * T] for x in ps[e:]], axis=0).astype(bf16)
                    oe = jnp.dot(pe, vv[k0 + (n + e - 1) * T:k0 + (n + e) * T, :], preferred_element_type=f32)
                    for a in range(e, A):
                        outs[a] = outs[a] + oe[(a - e) * G:(a - e + 1) * G]
                for a, r in enumerate(rows):
                    ctx_s[2 * p + blk[0], r // 2:(r + G) // 2, :] = pltpu.bitcast((outs[a] * rls[a]).astype(bf16), u32)

            order = [(e, c, j) for e in range(2) for j in range(nb // A - 1, -1, -1) for c in range(A)]
            order = [order[k] for k in ORDER]
            qs, ss, loaded = {}, {}, {}

            def kv(ref, e):
                if (id(ref), e) not in loaded:
                    loaded[id(ref), e] = pltpu.bitcast(ref[2 * (p & (NP - 1)) + e], bf16)
                return loaded[id(ref), e]

            def do_q(n):
                if n < len(order):
                    qs[n] = qproj(order[n])

            def do_qk(n):
                if n < len(order):
                    ss[n] = qk(order[n], qs.pop(n))

            for n in range(AHEAD + QAHEAD):
                do_q(n)
                if n >= QAHEAD:
                    do_qk(n - QAHEAD)
                if n == QAHEAD:
                    kv_units("v")
            for n in range(len(order)):
                do_q(n + AHEAD + QAHEAD)
                do_qk(n + AHEAD)
                softmax_pv(order[n], ss.pop(n))

            @pl.when(p + 2 < n_pair)
            def _():
                w_copy(jnp.minimum(p + 2, n_pair - 1), "q", sem_q, False)

            @pl.when(p + 4 < n_pair)
            def _():
                w_copy(jnp.minimum(p + 4, n_pair - 1), "kv", sem_kv, False)

            for j in range(len(big_copies)):
                @pl.when(p == 2 * j + 1)
                def _():
                    big_copies[j].start()

        def pair_body(p, carry):
            with jax.named_scope("main"):
                pair_step(p)
            return carry

        lax.fori_loop(0, n_pair, pair_body, 0)

        for c in big_copies:
            c.wait()
        wr = wr_s[...].astype(f32).reshape(1, M)

        def out_copy(r0, n):
            rows = rows_at(r0, n)
            return pltpu.make_async_copy(out_s.at[rows, :], out_hbm.at[rows, :], sem_out.at[0])

        def ctx_rows(segs):
            lhs = [jnp.concatenate([ctx_s[j, rows_at(u * (U // 2), n * U // 2, 1, U // 2), :] for j in range(H)], axis=1)
                   for u, n in segs]
            return pltpu.bitcast(jnp.concatenate(lhs, axis=0), bf16)

        def post(segs, attn, top, rs, dist=1, ascending=True):
            for n, r0 in enumerate([u * U + k * PR for u, nu in segs for k in range(nu * U // PR)]):
                rows = rows_at(r0, PR)
                xf = x_s[rows, :].astype(f32)
                if len(rs) >= dist:
                    xf = jnp.where(rs[-dist] * rs[-dist] < 0.0, 0.0, xf)
                elif rs and dist < 4:
                    xf = jnp.where(var < 0.0, 0.0, xf)
                af = pltpu.bitcast(attn[n * PR // 2:(n + 1) * PR // 2, :], bf16).astype(f32)
                h = (xf + af).astype(bf16)
                hf = h.astype(f32)
                mu = jnp.sum(hf, axis=1, keepdims=True) * (1.0 / M)
                dc = hf - mu
                var = jnp.sum(dc * dc, axis=1, keepdims=True) * (1.0 / M)
                den = _rnd(jnp.sqrt(_rnd(_rnd(var) + _rnd(jnp.full((1, 1), EPS, f32)))))
                hn = (_rnd(hf - _rnd(mu)) * (1.0 / den)).astype(bf16)
                hnf = hn.astype(f32)
                h_s[rows, :] = h
                hn_s[rows, :] = hn
                out_s[rows, :] = (hf + hnf).astype(bf16)
                r = _rnd(jnp.sum(hnf * wr, axis=1, keepdims=True))
                rs.append(r)
                m1, i1, m2, i2 = top
                idx = r0 + slot_id
                g1, g2 = r > m1, r > m2
                if not ascending:
                    g1, g2 = g1 | ((r == m1) & (idx < i1)), g2 | ((r == m2) & (idx < i2))
                top = (jnp.where(g1, r, m1), jnp.where(g1, idx, i1),
                       jnp.where(g1, m1, jnp.where(g2, r, m2)), jnp.where(g1, i1, jnp.where(g2, idx, i2)))
            return top

        slot_id = lax.broadcasted_iota(jnp.int32, (PR, 1), 0)
        ninf = jnp.full((PR, 1), -jnp.inf, f32)

        def pick(top):
            val = jnp.concatenate([top[0], top[2]], axis=0)
            pos = jnp.concatenate([top[1], top[3]], axis=0).astype(f32)
            m1 = jnp.max(val, axis=0, keepdims=True)
            p1 = jnp.min(jnp.where(val == m1, pos, float(S)), axis=0, keepdims=True)
            rest = jnp.where(pos == p1, -jnp.inf, val)
            m2 = jnp.max(rest, axis=0, keepdims=True)
            p2 = jnp.min(jnp.where((rest == m2) & (pos != p1), pos, float(S)), axis=0, keepdims=True)
            return m1, m2, [jnp.clip(x.astype(jnp.int32)[0, 0], 0, S - 1) for x in (p1, p2)]

        ut = S // U - 3
        rt = ut * U
        top0 = (ninf, slot_id, ninf, slot_id + PR)
        unit_s[0] = 0

        def hot_unit():
            return jnp.clip(unit_s[0], 0, 2)

        def oproj_body(b, top):
            @pl.when(b == 1)
            def _():
                unit_s[0] = (pick(top)[2][0] - rt) // U

            with jax.named_scope("oloop"):
                prev = jnp.where(b == 0, ut, 3 * (b - 1))
                top = post([(prev, 3)], attn_s, [jnp.where(b == 1, i, t) for i, t in zip(top0, top)], [])
                segs = [(3 * b, 2), (3 * b + 2 + jnp.where(b == n_rb - 1, hot_unit(), 0), 1)]
                o = jnp.dot(ctx_rows(segs), wo_s[:, 0:M], preferred_element_type=f32)
                attn_s[...] = pltpu.bitcast(o.astype(bf16), u32)

                @pl.when(b > 0)
                def _():
                    out_copy(prev * U, RB).start()
            return top

        top = lax.fori_loop(0, n_rb, oproj_body, top0)

        def groups(tok, end=S):
            return [pl.multiple_of(jnp.clip(i >> 3, 0, end // FG - 1) * FG, FG) for i in tok]

        def gather(ref, tok):
            return jnp.concatenate([ref[pl.ds(g, FG), :].astype(f32) for g in groups(tok)], axis=0)

        def swiglu(g, u):
            g, u = _rnd(g), _rnd(u)
            return (_rnd(g * jax.nn.sigmoid(g)) * u).astype(bf16)

        def finish(y, xs, m1, m2, tok):
            rid = lax.broadcasted_iota(jnp.int32, (2 * FG, 1), 0)
            g1, g2 = groups(tok)
            pos = jnp.where(rid < FG, g1 + rid, g2 + rid - FG)
            gate = _rnd(jax.nn.sigmoid(jnp.where(pos == tok[0], m1, m2)))
            upd = jnp.where((pos == tok[0]) | (pos == tok[1]), _rnd(_rnd(y) * gate), 0.0)
            fix_s[...] = (gather(h_s, tok) + _rnd(xs + upd)).astype(bf16)

        with jax.named_scope("tail"):
            unit = hot_unit()
            ua, ub = ut + jnp.where(unit == 0, 1, 0), ut + jnp.where(unit == 2, 1, 2)
            top = post([(ut - 2, 2), (ut + unit, 1)], attn_s, top, [], dist=2)
            out_copy(rt - 2 * U, 2 * U).start()

            m1, m2, tok = pick(top)
            xs = gather(hn_s, tok)
            xb = xs.astype(bf16)
            nc = F // KC
            todo = []
            for c in range(nc + DL):
                todo += [("gu", c, n) for n in range(2 * KC // T)] if c < nc else []
                todo += [("down", c - DL, n) for n in range(M // (2 * T))] if c >= DL else []
            gu, act, y, rs_a = {}, {}, {}, []

            def ffn_step():
                kind, c, n = todo.pop(0)
                if kind == "gu":
                    c0 = c * KC + n // 2 * T
                    gu[c, n] = jnp.dot(xb, (wg_s, wu_s)[n % 2][:, c0:c0 + T], preferred_element_type=f32)
                    return
                if c not in act:
                    g, u = [jnp.concatenate([gu[c, k] for k in range(w, 2 * KC // T, 2)], axis=1) for w in range(2)]
                    if c == AC:
                        u = jnp.where(rs_a[-1] * rs_a[-1] < 0.0, 0.0, u)
                    act[c] = swiglu(g, u)
                d = jnp.dot(act[c], wd_s[c * KC:(c + 1) * KC, n * 2 * T:(n + 1) * 2 * T], preferred_element_type=f32)
                y[n] = d if c == 0 else y[n] + d

            attn_t, host = [], 0
            n_host, n_in = 2 * (M // T) * (H * D // KC), len(todo) - NLEFT
            slots = {LEAD + i * (n_host - LEAD) // n_in for i in range(n_in)}
            for u in (ua, ub):
                lhs = ctx_rows([(u, 1)])
                acc = []
                for i in range(M // T * (H * D // KC)):
                    n, k = divmod(i, H * D // KC)
                    if u is ua:
                        w = wo_s[:, n * T:(n + 1) * T][k * KC:(k + 1) * KC]
                    else:
                        w = wo_s[k * KC:(k + 1) * KC, n * T:(n + 1) * T]
                    d = jnp.dot(lhs[:, k * KC:(k + 1) * KC], w, preferred_element_type=f32)
                    acc = acc + [d] if k == 0 else acc[:-1] + [acc[-1] + d]
                    if host in slots:
                        ffn_step()
                    host += 1
                attn_t.append(pltpu.bitcast(jnp.concatenate(acc, axis=1).astype(bf16), u32))
                if u is ua:
                    top = post([(ua, 1)], attn_t[0], top, rs_a, ascending=False)
                    out_copy(rt, U).start()
            while todo:
                ffn_step()
            finish(jnp.concatenate([y[n] for n in range(M // (2 * T))], axis=1), xs, m1, m2, tok)

            top = post([(ub, 1)], attn_t[1], top, [], dist=4, ascending=False)
            m1, m2, fin = pick(top)

            @pl.when((fin[0] != tok[0]) | (fin[1] != tok[1]))
            def _():
                xs = gather(hn_s, fin)
                xb = xs.astype(bf16)

                def chunk(c, y):
                    cols = pl.ds(pl.multiple_of(c * FC, FC), FC)
                    act = swiglu(jnp.dot(xb, wg_s[:, cols], preferred_element_type=f32),
                                 jnp.dot(xb, wu_s[:, cols], preferred_element_type=f32))
                    return y + jnp.dot(act, wd_s[cols, 0:M], preferred_element_type=f32)

                finish(lax.fori_loop(0, F // FC, chunk, jnp.zeros((2 * FG, M), f32)), xs, m1, m2, fin)

            out_copy(0, rt + U).wait()
            for k, g in enumerate(groups(fin)):
                out_s[pl.ds(g, FG), :] = fix_s[k * FG:(k + 1) * FG, :]
            c1, c2 = [pltpu.make_async_copy(out_s.at[pl.ds(g, FG), :], out_hbm.at[pl.ds(g, FG), :], sem_out.at[1])
                      for g in groups(fin, rt + U)]
            c1.start()
            out_copy(rt + U, 2 * U).start()
            c1.wait()
            c2.start()
            c2.wait()
            out_copy(rt + U, 2 * U).wait()

    scratch = [
        pltpu.VMEM((S, M), bf16),
        pltpu.VMEM((S // 2, M), u32),
        pltpu.VMEM((S, C), bf16),
        pltpu.VMEM((NQ, qa, 2 * WB, D), bf16),
        pltpu.VMEM((NKV, 2 * ka, 2 * WB, D), bf16),
        pltpu.VMEM((2 * NP, S // 2, D), u32),
        pltpu.VMEM((2 * NP, S // 2, D), u32),
        pltpu.VMEM((H, S // 2, D), u32),
        pltpu.VMEM((H * D, M + W_PAD), bf16),
        pltpu.VMEM((M,), bf16),
        pltpu.VMEM((M, F), bf16),
        pltpu.VMEM((M, F), bf16),
        pltpu.VMEM((F, M + W_PAD), bf16),
        pltpu.VMEM((RB // 2, M), u32),
        pltpu.VMEM((S, M), bf16),
        pltpu.VMEM((S, M), bf16),
        pltpu.VMEM((S, M), bf16),
        pltpu.VMEM((2 * FG, M), bf16),
        pltpu.SMEM((1,), jnp.int32),
        pltpu.SemaphoreType.DMA((len(CKV_SPLIT) - 1,)),
        pltpu.SemaphoreType.DMA((n_xc,)),
        pltpu.SemaphoreType.DMA((NQ,)),
        pltpu.SemaphoreType.DMA((NKV,)),
        pltpu.SemaphoreType.DMA((5,)),
        pltpu.SemaphoreType.DMA((2,)),
        pltpu.SemaphoreType.REGULAR,
    ]
    return kernel, scratch


@jax.jit
def pallas_sequential_preLN__compressed_kv_cla__moe_arch_mod__prompt_kernel(
    A_x: jax.Array,
    A_c_kv: jax.Array,
    A_w_q: jax.Array,
    A_w_uk: jax.Array,
    A_w_uv: jax.Array,
    A_w_o: jax.Array,
    B_x: jax.Array,
    B_w_r: jax.Array,
    B_w_gate: jax.Array,
    B_w_up: jax.Array,
    B_w_down: jax.Array,
):
    B, S, M = A_x.shape
    C = A_c_kv.shape[2]
    H, D = A_w_q.shape[1], A_w_q.shape[2]
    F = B_w_gate.shape[1]
    assert B == 1 and A_c_kv.shape[1] == S

    kernel, scratch = _make_kernel(S, M, C, H, D, F)
    any_spec = pl.BlockSpec(memory_space=pl.ANY)
    out = pl.pallas_call(
        kernel,
        grid=(1,),
        in_specs=[any_spec] * 10,
        out_specs=any_spec,
        out_shape=jax.ShapeDtypeStruct((S, M), A_x.dtype),
        scratch_shapes=scratch,
        compiler_params=pltpu.CompilerParams(
            vmem_limit_bytes=120 * 1024 * 1024,
            disable_bounds_checks=True,
            disable_semaphore_checks=True,
        ),
        name="mla_mod_block",
    )(
        A_x.reshape(S, M), A_c_kv.reshape(S, C),
        A_w_q.reshape(M // WB, WB, H // 2, 2, D),
        A_w_uk.reshape(C // WB, WB, H // 2, 2, D),
        A_w_uv.reshape(C // WB, WB, H // 2, 2, D),
        A_w_o.reshape(H * D, M), B_w_r, B_w_gate, B_w_up, B_w_down,
    )
    return out.reshape(B, S, M)
```

```python
import jax
import jax.numpy as jnp
from jax import lax
import jax.experimental.pallas as pl
import jax.experimental.pallas.tpu as pltpu

bf16 = jnp.bfloat16
f32 = jnp.float32
u32 = jnp.uint32

T = 128
G = 32
A = T // G
AHEAD = 3
QAHEAD = 1
AQ = 8
ORDER = (0, 1, 2, 4, 3, 5, 10, 7, 8, 16, 6, 11, 9, 17, 18, 19, 20, 22, 21, 24, 25, 26, 27, 28, 23, 12, 13, 29, 14, 30, 15, 31)
WB = 4
NQ, NKV, NP = 4, 8, 4
UR, UPS = 256, 7
RB = 192
U = 64
FG = 8
KC = 512
LEAD, NLEFT = 51, 11
DL, AC = 2, 4
FC = 896
PR = 16
LP, LCH = 16, 4
XC = 256
CKV_SPLIT = (0, 256, 768, 1344, 2048)
PRO_ORDER = ([("w", 0)] + [("c", i) for i in range(4)] + [("x", i) for i in range(3)] + [("w", 1)]
             + [("x", i) for i in range(3, 8)] + [("w", 2), ("q", 0), ("q", 1), ("w", 3)])
KR = 704
W_PAD = 128
EPS = 1e-5
NEG = -1e30
LOG2E = 1.4426950408889634
NT = (((1,), (1,)), ((), ()))


def _rnd(x):
    return x.astype(bf16).astype(f32)


def _recip(l):
    r = pl.reciprocal(l, approx=True)
    return r * (2.0 - l * r)


def _make_kernel(S, M, C, H, D, F):
    n_pair = H // 2
    nb = S // T
    n_rb = (S - 2 * U) // RB
    assert n_rb * RB + 2 * U == S and RB == 3 * U and FG == 8
    n_xc = S // XC
    qa, ka = M // WB, C // WB
    upp = S // UR
    assert sorted(ORDER) == list(range(2 * nb)) and CKV_SPLIT[-1] == S and CKV_SPLIT[-2] == S - KR
    assert upp == 8 and (n_pair - 2) * upp == n_pair * UPS
    scale = (D ** -0.5) * LOG2E

    def kernel(*refs):
        def once(i, carry):
            kernel_body(*refs)
            return carry

        lax.fori_loop(0, pl.program_id(0) + 1, once, 0)

    def kernel_body(x_hbm, ckv_hbm, wq_hbm, wk_hbm, wv_hbm, wo_hbm, wr_hbm, wg_hbm, wu_hbm, wd_hbm,
                    out_hbm,
                    x_s, xn_s, ckv_s, wq_s, wkv_s, k_s, v_s, ctx_s,
                    wo_s, wr_s, wg_s, wu_s, wd_s, attn_s, h_s, hn_s, out_s, fix_s, unit_s,
                    sem_in, sem_x, sem_q, sem_kv, sem_big, sem_out, sem_reg):

        w_parts = {"q": (wq_hbm, wq_s, NQ, 0, qa), "k": (wk_hbm, wkv_s, NKV, 0, ka), "v": (wv_hbm, wkv_s, NKV, ka, ka)}

        def w_copy(p, names, sem, wait):
            _, buf, nslot, _, _ = w_parts[names[0]]
            slot = p % nslot if isinstance(p, int) else p & (nslot - 1)
            if wait:
                pltpu.make_async_copy(buf.at[slot], buf.at[slot], sem.at[slot]).wait()
                return
            for name in names:
                hbm, _, _, r0, n = w_parts[name]
                for b in range(WB):
                    pltpu.make_async_copy(hbm.at[:, b, p], buf.at[slot, pl.ds(r0, n), pl.ds(2 * b, 2), :],
                                          sem.at[slot]).start()

        def unpack(p, name):
            _, buf, nslot, r0, n = w_parts[name]
            slot = p % nslot if isinstance(p, int) else p & (nslot - 1)
            w = pltpu.bitcast(buf[slot, r0:r0 + n].reshape(n * 2 * WB, D), u32)
            return [pltpu.bitcast(x, f32).astype(bf16) for x in (w << 16, w & jnp.uint32(0xFFFF0000))]

        big_copies = [
            pltpu.make_async_copy(wo_hbm, wo_s.at[:, pl.ds(0, M)], sem_big.at[0]),
            pltpu.make_async_copy(wg_hbm, wg_s.at[:, pl.ds(0, F)], sem_big.at[1]),
            pltpu.make_async_copy(wu_hbm, wu_s.at[:, pl.ds(0, F)], sem_big.at[2]),
            pltpu.make_async_copy(wd_hbm, wd_s.at[:, pl.ds(0, M)], sem_big.at[3]),
            pltpu.make_async_copy(wr_hbm, wr_s, sem_big.at[4]),
        ]

        def rows_at(r0, n, div=1, align=16):
            if isinstance(r0, int):
                return pl.ds(r0 // div, n // div)
            return pl.ds(pl.multiple_of(r0 if div == 1 else r0 >> 1, align // div), n // div)

        def x_copy(i):
            rows = rows_at(i * XC, XC)
            return pltpu.make_async_copy(x_hbm.at[rows, :], x_s.at[rows, :], sem_x.at[i])

        def ckv_copy(i):
            rows = pl.ds(CKV_SPLIT[i], CKV_SPLIT[i + 1] - CKV_SPLIT[i])
            return pltpu.make_async_copy(ckv_hbm.at[rows, :], ckv_s.at[rows, :], sem_in.at[i])

        def layernorm_x(row0, nrows):
            toks = []
            for n in range(nrows // LP):
                r0 = row0 + n * LP
                xf = x_s[rows_at(r0, LP), :].astype(f32)
                if len(toks) >= LCH:
                    xf = jnp.where(toks[-LCH] < 0.0, 0.0, xf)
                elif toks:
                    xf = jnp.where(mu * mu < 0.0, 0.0, xf)
                mu = jnp.sum(xf, axis=1, keepdims=True) * (1.0 / M)
                d = xf - mu
                var = jnp.sum(d * d, axis=1, keepdims=True) * (1.0 / M)
                rs = lax.rsqrt(var + EPS)
                toks.append(rs)
                xn_s[rows_at(r0, LP, 2), :] = pltpu.bitcast((d * rs).astype(bf16), u32)

        def kv_proj(pair, r0, n, names):
            lhs = ckv_s[rows_at(r0, n, 1, 64), :]
            slot = pair % NP if isinstance(pair, int) else pair & (NP - 1)
            for name in names:
                for e, w in enumerate(unpack(pair, name)):
                    y = jnp.dot(lhs, w, preferred_element_type=f32)
                    dst = k_s if name == "k" else v_s
                    dst[2 * slot + e, rows_at(r0, n, 2, 64), :] = pltpu.bitcast(y.astype(bf16), u32)

        with jax.named_scope("prologue"):
            for k, (kind, i) in enumerate(PRO_ORDER):
                if k and kind != PRO_ORDER[k - 1][0]:
                    pl.semaphore_signal(sem_reg, 1)
                    pl.semaphore_wait(sem_reg, 1)
                if kind == "c":
                    ckv_copy(i).start()
                elif kind == "x":
                    x_copy(i).start()
                elif kind == "w":
                    w_copy(i, "kv", sem_kv, False)
                else:
                    w_copy(i, "q", sem_q, False)
            attn_s[...] = jnp.zeros(attn_s.shape, u32)
            w_copy(0, "kv", sem_kv, True)
            for i in range(3):
                ckv_copy(i).wait()
                with jax.named_scope("r%d" % i):
                    kv_proj(0, CKV_SPLIT[i], CKV_SPLIT[i + 1] - CKV_SPLIT[i], "kv")
            ckv_copy(3).wait()

            def pro_body(t, carry):
                @pl.when(t == 1)
                def _():
                    w_copy(1, "kv", sem_kv, True)

                x_copy(2 * t).wait()
                x_copy(2 * t + 1).wait()
                with jax.named_scope("rl"):
                    layernorm_x(2 * t * XC, 2 * XC)
                    kv_proj(jnp.minimum(t, 1), jnp.where(t == 0, S - KR, jnp.minimum((t - 1) * KR, S - KR)), KR, "kv")
                return carry

            lax.fori_loop(0, 4, pro_body, 0)

        row = lax.broadcasted_iota(jnp.int32, (G, T), 0)
        col = lax.broadcasted_iota(jnp.int32, (G, T), 1)

        def pair_step(p):
            w_copy(p, "q", sem_q, True)

            @pl.when(p + 2 < n_pair)
            def _():
                w_copy(p + 2, "kv", sem_kv, True)

            tri = col <= row + (T - G)

            def kv_units(name):
                for i in range(UPS):
                    u = p * UPS + i
                    kv_proj(2 + (u >> 3), (u & 7) * UR, UR, name)

            kv_units("k")
            wq2 = unpack(p, "q")

            hist = []

            def geom(blk):
                _, c, j = blk
                k0 = (c + 1) * G % T
                return k0, A * j + (0 if k0 else 1), [(A * j + a) * T + c * G for a in range(A)]

            def qproj(blk):
                xn = jnp.concatenate([xn_s[r // 2:(r + G) // 2, :] for r in geom(blk)[2]], axis=0)
                return jnp.dot(pltpu.bitcast(xn, bf16), wq2[blk[0]], preferred_element_type=f32) * scale

            def qk(blk, qf):
                k0, n, _ = geom(blk)
                kk = kv(k_s, blk[0])
                if len(hist) >= AQ:
                    qf = jnp.where(jnp.concatenate(hist[-AQ], axis=0) < 0.0, 0.0, qf)
                q = qf.astype(bf16)
                main = head = None
                if n:
                    main = lax.dot_general(q, kk[k0:k0 + n * T, :], NT, preferred_element_type=f32)
                if k0:
                    st = lax.dot_general(kk[0:k0, :], q, NT, preferred_element_type=f32)
                    head = jnp.concatenate([st, jnp.full((T - k0, T), NEG, f32)], axis=0).T
                extra = [lax.dot_general(qf[e * G:].astype(bf16), kk[k0 + (n + e - 1) * T:k0 + (n + e) * T, :], NT,
                                         preferred_element_type=f32) for e in range(1, A)]
                return main, head, extra

            def softmax_pv(blk, sc):
                k0, n, rows = geom(blk)
                vv = kv(v_s, blk[0])
                main, head, extra = sc
                ps, rls = [], []
                for a in range(A):
                    parts = []
                    if n:
                        mm = main[a * G:(a + 1) * G]
                        if a == 0:
                            parts += [mm[:, :(n - 1) * T]] if n > 1 else []
                            parts.append(jnp.where(tri, mm[:, (n - 1) * T:], NEG))
                        else:
                            parts.append(mm)
                    if k0:
                        hd = head[a * G:(a + 1) * G]
                        parts.append(hd if n + a else jnp.where(col <= row + (k0 - G), hd, NEG))
                    for e in range(1, a + 1):
                        ex = extra[e - 1][(a - e) * G:(a - e + 1) * G]
                        parts.append(jnp.where(tri, ex, NEG) if e == a else ex)
                    s = jnp.concatenate(parts, axis=1) if len(parts) > 1 else parts[0]
                    pr = jnp.exp2(s - jnp.max(s, axis=1, keepdims=True))
                    rls.append(_recip(jnp.sum(_rnd(pr), axis=1, keepdims=True)))
                    ps.append(pr)
                hist.append(rls)
                w = ps[0].shape[1]
                vm = [vv[k0:k0 + n * T, :]] if n else []
                vm += [vv[0:T, :]] if k0 else []
                o = jnp.dot(jnp.concatenate([x[:, :w] for x in ps], axis=0).astype(bf16),
                            jnp.concatenate(vm, axis=0) if len(vm) > 1 else vm[0], preferred_element_type=f32)
                outs = [o[a * G:(a + 1) * G] for a in range(A)]
                for e in range(1, A):
                    pe = jnp.concatenate([x[:, w + (e - 1) * T:w + e * T] for x in ps[e:]], axis=0).astype(bf16)
                    oe = jnp.dot(pe, vv[k0 + (n + e - 1) * T:k0 + (n + e) * T, :], preferred_element_type=f32)
                    for a in range(e, A):
                        outs[a] = outs[a] + oe[(a - e) * G:(a - e + 1) * G]
                for a, r in enumerate(rows):
                    ctx_s[2 * p + blk[0], r // 2:(r + G) // 2, :] = pltpu.bitcast((outs[a] * rls[a]).astype(bf16), u32)

            order = [(e, c, j) for e in range(2) for j in range(nb // A - 1, -1, -1) for c in range(A)]
            order = [order[k] for k in ORDER]
            qs, ss, loaded = {}, {}, {}

            def kv(ref, e):
                if (id(ref), e) not in loaded:
                    loaded[id(ref), e] = pltpu.bitcast(ref[2 * (p & (NP - 1)) + e], bf16)
                return loaded[id(ref), e]

            def do_q(n):
                if n < len(order):
                    qs[n] = qproj(order[n])

            def do_qk(n):
                if n < len(order):
                    ss[n] = qk(order[n], qs.pop(n))

            for n in range(AHEAD + QAHEAD):
                do_q(n)
                if n >= QAHEAD:
                    do_qk(n - QAHEAD)
                if n == QAHEAD:
                    kv_units("v")
            for n in range(len(order)):
                do_q(n + AHEAD + QAHEAD)
                do_qk(n + AHEAD)
                softmax_pv(order[n], ss.pop(n))

            @pl.when(p + 2 < n_pair)
            def _():
                w_copy(jnp.minimum(p + 2, n_pair - 1), "q", sem_q, False)

            @pl.when(p + 4 < n_pair)
            def _():
                w_copy(jnp.minimum(p + 4, n_pair - 1), "kv", sem_kv, False)

            for j in range(len(big_copies)):
                @pl.when(p == 2 * j + 1)
                def _():
                    big_copies[j].start()

        def pair_body(p, carry):
            with jax.named_scope("main"):
                pair_step(p)
            return carry

        lax.fori_loop(0, n_pair, pair_body, 0)

        for c in big_copies:
            c.wait()
        wr = wr_s[...].astype(f32).reshape(1, M)

        def out_copy(r0, n):
            rows = rows_at(r0, n)
            return pltpu.make_async_copy(out_s.at[rows, :], out_hbm.at[rows, :], sem_out.at[0])

        def ctx_rows(segs):
            lhs = [jnp.concatenate([ctx_s[j, rows_at(u * (U // 2), n * U // 2, 1, U // 2), :] for j in range(H)], axis=1)
                   for u, n in segs]
            return pltpu.bitcast(jnp.concatenate(lhs, axis=0), bf16)

        def post(segs, attn, top, rs, dist=1, ascending=True):
            for n, r0 in enumerate([u * U + k * PR for u, nu in segs for k in range(nu * U // PR)]):
                rows = rows_at(r0, PR)
                xf = x_s[rows, :].astype(f32)
                if len(rs) >= dist:
                    xf = jnp.where(rs[-dist] * rs[-dist] < 0.0, 0.0, xf)
                elif rs and dist < 4:
                    xf = jnp.where(var < 0.0, 0.0, xf)
                af = pltpu.bitcast(attn[n * PR // 2:(n + 1) * PR // 2, :], bf16).astype(f32)
                h = (xf + af).astype(bf16)
                hf = h.astype(f32)
                mu = jnp.sum(hf, axis=1, keepdims=True) * (1.0 / M)
                dc = hf - mu
                var = jnp.sum(dc * dc, axis=1, keepdims=True) * (1.0 / M)
                den = _rnd(jnp.sqrt(_rnd(_rnd(var) + _rnd(jnp.full((1, 1), EPS, f32)))))
                hn = (_rnd(hf - _rnd(mu)) * (1.0 / den)).astype(bf16)
                hnf = hn.astype(f32)
                h_s[rows, :] = h
                hn_s[rows, :] = hn
                out_s[rows, :] = (hf + hnf).astype(bf16)
                r = _rnd(jnp.sum(hnf * wr, axis=1, keepdims=True))
                rs.append(r)
                m1, i1, m2, i2 = top
                idx = r0 + slot_id
                g1, g2 = r > m1, r > m2
                if not ascending:
                    g1, g2 = g1 | ((r == m1) & (idx < i1)), g2 | ((r == m2) & (idx < i2))
                top = (jnp.where(g1, r, m1), jnp.where(g1, idx, i1),
                       jnp.where(g1, m1, jnp.where(g2, r, m2)), jnp.where(g1, i1, jnp.where(g2, idx, i2)))
            return top

        slot_id = lax.broadcasted_iota(jnp.int32, (PR, 1), 0)
        ninf = jnp.full((PR, 1), -jnp.inf, f32)

        def pick(top):
            val = jnp.concatenate([top[0], top[2]], axis=0)
            pos = jnp.concatenate([top[1], top[3]], axis=0).astype(f32)
            m1 = jnp.max(val, axis=0, keepdims=True)
            p1 = jnp.min(jnp.where(val == m1, pos, float(S)), axis=0, keepdims=True)
            rest = jnp.where(pos == p1, -jnp.inf, val)
            m2 = jnp.max(rest, axis=0, keepdims=True)
            p2 = jnp.min(jnp.where((rest == m2) & (pos != p1), pos, float(S)), axis=0, keepdims=True)
            return m1, m2, [jnp.clip(x.astype(jnp.int32)[0, 0], 0, S - 1) for x in (p1, p2)]

        ut = S // U - 3
        rt = ut * U
        top0 = (ninf, slot_id, ninf, slot_id + PR)
        unit_s[0] = 0

        def hot_unit():
            return jnp.clip(unit_s[0], 0, 2)

        def oproj_body(b, top):
            @pl.when(b == 1)
            def _():
                unit_s[0] = (pick(top)[2][0] - rt) // U

            with jax.named_scope("oloop"):
                prev = jnp.where(b == 0, ut, 3 * (b - 1))
                top = post([(prev, 3)], attn_s, [jnp.where(b == 1, i, t) for i, t in zip(top0, top)], [])
                segs = [(3 * b, 2), (3 * b + 2 + jnp.where(b == n_rb - 1, hot_unit(), 0), 1)]
                o = jnp.dot(ctx_rows(segs), wo_s[:, 0:M], preferred_element_type=f32)
                attn_s[...] = pltpu.bitcast(o.astype(bf16), u32)

                @pl.when(b > 0)
                def _():
                    out_copy(prev * U, RB).start()
            return top

        top = lax.fori_loop(0, n_rb, oproj_body, top0)

        def groups(tok, end=S):
            return [pl.multiple_of(jnp.clip(i >> 3, 0, end // FG - 1) * FG, FG) for i in tok]

        def gather(ref, tok):
            return jnp.concatenate([ref[pl.ds(g, FG), :].astype(f32) for g in groups(tok)], axis=0)

        def swiglu(g, u):
            g, u = _rnd(g), _rnd(u)
            return (_rnd(g * jax.nn.sigmoid(g)) * u).astype(bf16)

        def finish(y, xs, m1, m2, tok):
            rid = lax.broadcasted_iota(jnp.int32, (2 * FG, 1), 0)
            g1, g2 = groups(tok)
            pos = jnp.where(rid < FG, g1 + rid, g2 + rid - FG)
            gate = _rnd(jax.nn.sigmoid(jnp.where(pos == tok[0], m1, m2)))
            upd = jnp.where((pos == tok[0]) | (pos == tok[1]), _rnd(_rnd(y) * gate), 0.0)
            fix_s[...] = (gather(h_s, tok) + _rnd(xs + upd)).astype(bf16)

        with jax.named_scope("tail"):
            unit = hot_unit()
            ua, ub = ut + jnp.where(unit == 0, 1, 0), ut + jnp.where(unit == 2, 1, 2)
            top = post([(ut - 2, 2), (ut + unit, 1)], attn_s, top, [], dist=2)
            out_copy(rt - 2 * U, 2 * U).start()

            m1, m2, tok = pick(top)
            xs = gather(hn_s, tok)
            xb = xs.astype(bf16)
            nc = F // KC
            todo = []
            for c in range(nc + DL):
                todo += [("gu", c, n) for n in range(2 * KC // T)] if c < nc else []
                todo += [("down", c - DL, n) for n in range(M // (2 * T))] if c >= DL else []
            gu, act, y, rs_a = {}, {}, {}, []

            def ffn_step():
                kind, c, n = todo.pop(0)
                if kind == "gu":
                    c0 = c * KC + n // 2 * T
                    gu[c, n] = jnp.dot(xb, (wg_s, wu_s)[n % 2][:, c0:c0 + T], preferred_element_type=f32)
                    return
                if c not in act:
                    g, u = [jnp.concatenate([gu[c, k] for k in range(w, 2 * KC // T, 2)], axis=1) for w in range(2)]
                    if c == AC:
                        u = jnp.where(rs_a[-1] * rs_a[-1] < 0.0, 0.0, u)
                    act[c] = swiglu(g, u)
                d = jnp.dot(act[c], wd_s[c * KC:(c + 1) * KC, n * 2 * T:(n + 1) * 2 * T], preferred_element_type=f32)
                y[n] = d if c == 0 else d + y[n]

            attn_t, host = [], 0
            n_host, n_in = 2 * (M // T) * (H * D // KC), len(todo) - NLEFT
            slots = {LEAD + i * (n_host - LEAD) // n_in for i in range(n_in)}
            for u in (ua, ub):
                lhs = ctx_rows([(u, 1)])
                acc = []
                for i in range(M // T * (H * D // KC)):
                    n, k = divmod(i, H * D // KC)
                    if u is ua:
                        w = wo_s[:, n * T:(n + 1) * T][k * KC:(k + 1) * KC]
                    else:
                        w = wo_s[k * KC:(k + 1) * KC, n * T:(n + 1) * T]
                    d = jnp.dot(lhs[:, k * KC:(k + 1) * KC], w, preferred_element_type=f32)
                    acc = acc + [d] if k == 0 else acc[:-1] + [d + acc[-1]]
                    if host in slots:
                        ffn_step()
                    host += 1
                attn_t.append(pltpu.bitcast(jnp.concatenate(acc, axis=1).astype(bf16), u32))
                if u is ua:
                    top = post([(ua, 1)], attn_t[0], top, rs_a, ascending=False)
                    out_copy(rt, U).start()
            while todo:
                ffn_step()
            finish(jnp.concatenate([y[n] for n in range(M // (2 * T))], axis=1), xs, m1, m2, tok)

            top = post([(ub, 1)], attn_t[1], top, [], dist=4, ascending=False)
            m1, m2, fin = pick(top)

            @pl.when((fin[0] != tok[0]) | (fin[1] != tok[1]))
            def _():
                xs = gather(hn_s, fin)
                xb = xs.astype(bf16)

                def chunk(c, y):
                    cols = pl.ds(pl.multiple_of(c * FC, FC), FC)
                    act = swiglu(jnp.dot(xb, wg_s[:, cols], preferred_element_type=f32),
                                 jnp.dot(xb, wu_s[:, cols], preferred_element_type=f32))
                    return y + jnp.dot(act, wd_s[cols, 0:M], preferred_element_type=f32)

                finish(lax.fori_loop(0, F // FC, chunk, jnp.zeros((2 * FG, M), f32)), xs, m1, m2, fin)

            out_copy(0, rt + U).wait()
            for k, g in enumerate(groups(fin)):
                out_s[pl.ds(g, FG), :] = fix_s[k * FG:(k + 1) * FG, :]
            c1, c2 = [pltpu.make_async_copy(out_s.at[pl.ds(g, FG), :], out_hbm.at[pl.ds(g, FG), :], sem_out.at[1])
                      for g in groups(fin, rt + U)]
            c1.start()
            out_copy(rt + U, 2 * U).start()
            c1.wait()
            c2.start()
            c2.wait()
            out_copy(rt + U, 2 * U).wait()

    scratch = [
        pltpu.VMEM((S, M), bf16),
        pltpu.VMEM((S // 2, M), u32),
        pltpu.VMEM((S, C), bf16),
        pltpu.VMEM((NQ, qa, 2 * WB, D), bf16),
        pltpu.VMEM((NKV, 2 * ka, 2 * WB, D), bf16),
        pltpu.VMEM((2 * NP, S // 2, D), u32),
        pltpu.VMEM((2 * NP, S // 2, D), u32),
        pltpu.VMEM((H, S // 2, D), u32),
        pltpu.VMEM((H * D, M + W_PAD), bf16),
        pltpu.VMEM((M,), bf16),
        pltpu.VMEM((M, F + W_PAD), bf16),
        pltpu.VMEM((M, F + W_PAD), bf16),
        pltpu.VMEM((F, M + W_PAD), bf16),
        pltpu.VMEM((RB // 2, M), u32),
        pltpu.VMEM((S, M), bf16),
        pltpu.VMEM((S, M), bf16),
        pltpu.VMEM((S, M), bf16),
        pltpu.VMEM((2 * FG, M), bf16),
        pltpu.SMEM((1,), jnp.int32),
        pltpu.SemaphoreType.DMA((len(CKV_SPLIT) - 1,)),
        pltpu.SemaphoreType.DMA((n_xc,)),
        pltpu.SemaphoreType.DMA((NQ,)),
        pltpu.SemaphoreType.DMA((NKV,)),
        pltpu.SemaphoreType.DMA((5,)),
        pltpu.SemaphoreType.DMA((2,)),
        pltpu.SemaphoreType.REGULAR,
    ]
    return kernel, scratch


@jax.jit
def pallas_sequential_preLN__compressed_kv_cla__moe_arch_mod__prompt_kernel(
    A_x: jax.Array,
    A_c_kv: jax.Array,
    A_w_q: jax.Array,
    A_w_uk: jax.Array,
    A_w_uv: jax.Array,
    A_w_o: jax.Array,
    B_x: jax.Array,
    B_w_r: jax.Array,
    B_w_gate: jax.Array,
    B_w_up: jax.Array,
    B_w_down: jax.Array,
):
    B, S, M = A_x.shape
    C = A_c_kv.shape[2]
    H, D = A_w_q.shape[1], A_w_q.shape[2]
    F = B_w_gate.shape[1]
    assert B == 1 and A_c_kv.shape[1] == S

    kernel, scratch = _make_kernel(S, M, C, H, D, F)
    any_spec = pl.BlockSpec(memory_space=pl.ANY)
    out = pl.pallas_call(
        kernel,
        grid=(1,),
        in_specs=[any_spec] * 10,
        out_specs=any_spec,
        out_shape=jax.ShapeDtypeStruct((S, M), A_x.dtype),
        scratch_shapes=scratch,
        compiler_params=pltpu.CompilerParams(
            vmem_limit_bytes=120 * 1024 * 1024,
            disable_bounds_checks=True,
            disable_semaphore_checks=True,
        ),
        name="mla_mod_block",
    )(
        A_x.reshape(S, M), A_c_kv.reshape(S, C),
        A_w_q.reshape(M // WB, WB, H // 2, 2, D),
        A_w_uk.reshape(C // WB, WB, H // 2, 2, D),
        A_w_uv.reshape(C // WB, WB, H // 2, 2, D),
        A_w_o.reshape(H * D, M), B_w_r, B_w_gate, B_w_up, B_w_down,
    )
    return out.reshape(B, S, M)
```
